```python
import jax
import jax.numpy as jnp

def _softmax(x, axis=-1):
    return jax.nn.softmax(x, axis=axis)
def _gelu(x):
    return jax.nn.gelu(x, approximate=True)
def _silu(x):
    return jax.nn.silu(x)
def _sigmoid(x):
    return jax.nn.sigmoid(x)
def _layernorm(x, axis=-1, eps=1e-5):
    m = jnp.mean(x, axis=axis, keepdims=True)
    v = jnp.var(x, axis=axis, keepdims=True)
    return (x - m) / jnp.sqrt(v + eps)
def _scatter_add(tgt, idx, src, axis=0):
    return tgt.at[idx].add(src)
def _segment_sum(src, seg, n):
    return jax.ops.segment_sum(src, seg, n)
class _Rng:
    def __init__(self, key):
        self._k = key
    def _next(self):
        self._k, sub = jax.random.split(self._k)
        return sub
    def normal(self, shape):
        return jax.random.normal(self._next(), shape, dtype=jnp.bfloat16)
    def randint(self, lo, hi, shape):
        return jax.random.randint(self._next(), shape, lo, hi, dtype=jnp.int32)
    def uniform(self, shape, lo=0.0, hi=1.0):
        return jax.random.uniform(self._next(), shape, jnp.bfloat16, lo, hi)
    def permutation(self, n):
        return jax.random.permutation(self._next(), n)


kernel_name = 'concat_heads__sliding_local_dilated__compressed_kv_cla__prompt'

def setup_inputs():
    _rng = _Rng(jax.random.key(int.from_bytes(__import__("os").urandom(4), "little")))
    _w = (lambda a: (lambda t: t.astype(jnp.bfloat16) if jnp.issubdtype(t.dtype, jnp.floating) else t)(jnp.asarray(a)))
    def _A_setup():
        B, S, D = 1, 2048, 1024
        return {
            "x": _w((lambda *s: _rng.normal(s) * 0.05)(B, S, D)),
            "wqkv": _w((lambda *s: _rng.normal(s) * 0.05)(D, 3 * D)),
            "wo": _w((lambda *s: _rng.normal(s) * 0.05)(D, D)),
        }
    _A_in = _A_setup()

    def _B_setup():
        B, H, Sq, Sk, D, M = 1, 32, 2048, 2048, 128, 1024
        Dc = 4 * D
        return {
            "x": _w((lambda *s: _rng.normal(s) * 0.05)(B, Sq, M)),
            "c_kv": _w((lambda *s: _rng.normal(s) * 0.05)(B, Sk, Dc)),
            "w_q": _w((lambda *s: _rng.normal(s) * 0.05)(M, H, D) * (M ** -0.5)),
            "w_uk": _w((lambda *s: _rng.normal(s) * 0.05)(Dc, H, D) * (Dc ** -0.5)),
            "w_uv": _w((lambda *s: _rng.normal(s) * 0.05)(Dc, H, D) * (Dc ** -0.5)),
            "w_o": _w((lambda *s: _rng.normal(s) * 0.05)(H, D, M) * ((H * D) ** -0.5)),
        }
    _B_in = _B_setup()

    return {
        "A_x": _A_in["x"],
        "A_wqkv": _A_in["wqkv"],
        "A_wo": _A_in["wo"],
        "B_x": _B_in["x"],
        "B_c_kv": _B_in["c_kv"],
        "B_w_q": _B_in["w_q"],
        "B_w_uk": _B_in["w_uk"],
        "B_w_uv": _B_in["w_uv"],
        "B_w_o": _B_in["w_o"],
    }

def reference(A_x, A_wqkv, A_wo, B_x, B_c_kv, B_w_q, B_w_uk, B_w_uv, B_w_o):
    def _A_ref(x, wqkv, wo):
        B, S, D = x.shape
        H = 32; Dh = D // H
        W, dil = 8, 2
        qkv = (lambda x, *d: x.transpose(*d))((x @ wqkv).reshape(B, S, 3, H, Dh), 2, 0, 3, 1, 4)
        q, k, v = qkv[0], qkv[1], qkv[2]
        scale = Dh ** -0.5
        pos = jnp.arange(S)
        off = jnp.arange(W) * dil
        idx = pos[:, None] - off[None, :]
        mask = idx >= 0
        idx_c = jnp.where(mask, idx, 0).reshape(-1)
        kg = k[:, :, idx_c, :].reshape(B, H, S, W, Dh)
        vg = v[:, :, idx_c, :].reshape(B, H, S, W, Dh)
        logits = jnp.einsum("bhsd,bhswd->bhsw", q, kg) * scale
        logits = jnp.where(mask[None, None, :, :], logits, -1e9)
        attn = _softmax(logits, axis=-1)
        o = jnp.einsum("bhsw,bhswd->bhsd", attn, vg)
        return (lambda x, *d: x.transpose(*d))(o, 0, 2, 1, 3).reshape(B, S, D) @ wo

    def _B_ref(x, c_kv, w_q, w_uk, w_uv, w_o):
        B, Sq, M = x.shape[0], x.shape[1], x.shape[2]
        Sk = c_kv.shape[1]
        H, D = w_q.shape[1], w_q.shape[2]
        q = jnp.einsum("bqm,mhd->bhqd", x, w_q)
        k = jnp.einsum("bkc,chd->bhkd", c_kv, w_uk)
        v = jnp.einsum("bkc,chd->bhkd", c_kv, w_uv)
        scores = jnp.einsum("bhqd,bhkd->bhqk", q, k) * (D ** -0.5)
        off = Sk - Sq
        qi = jnp.arange(Sq)[:, None]
        kj = jnp.arange(Sk)[None, :]
        cmask = kj <= (qi + off)
        scores = jnp.where(cmask[None, None], scores, -1e9)
        p = _softmax(scores, axis=-1)
        ctx = jnp.einsum("bhqk,bhkd->bhqd", p, v)
        return jnp.einsum("bhqd,hdm->bqm", ctx, w_o)

    a = _A_ref(A_x, A_wqkv, A_wo)
    b = _B_ref(B_x, B_c_kv, B_w_q, B_w_uk, B_w_uv, B_w_o)
    return jnp.concatenate([a, b], axis=-1)
```

```python
import functools
import math

import jax
import jax.numpy as jnp
import numpy as np
from jax.experimental import pallas as pl
from jax.experimental.pallas import tpu as pltpu

S = 2048
DM = 1024
HA, DA = 32, 32
WIN, DIL = 8, 2
HB, DB = 32, 128
DC = 512
NEG = -1e9
LOG2E = math.log2(math.e)

F32, BF16, U32 = jnp.float32, jnp.bfloat16, jnp.uint32
NT = (((1,), (1,)), ((), ()))

CFG = dict(bq=128, ra=256, ro=256)


def _dot(a, b):
    return jnp.dot(a, b, preferred_element_type=F32)


def _as_bf16(x32):
    return pltpu.bitcast(x32, BF16)


def _half(w32, hi):
    x = (w32 & jnp.uint32(0xFFFF0000)) if hi else (w32 << 16)
    return pltpu.bitcast(x, F32).astype(BF16)


def _swap_lane_and_chunk_bits(chunks):
    lane = jax.lax.broadcasted_iota(jnp.int32, chunks[0].shape, 1)
    u = (lane >> 1) & 7
    rolled = [x if c == 0 else pltpu.roll(x, 2 * c, 1) for c, x in enumerate(chunks)]
    xs = [rolled[(-i) % 8] for i in range(8)]
    for t in (1, 2, 4):
        m = (u & t) != 0
        xs = [jnp.where(m, xs[(i - t) % 8], xs[i]) for i in range(8)]
    return [x if j == 0 else pltpu.roll(x, 128 - 2 * j, 1) for j, x in enumerate(xs)]


def _kernel(xa_hbm, wqkv_hbm, woa_hbm, xb_hbm, c_hbm, wq_hbm, wuk_hbm, wuv_hbm, wob_hbm,
            out_hbm,
            xb, cc, wq, wk, wv, q0, k0, v0, q1, k1, v1, ctx, wob,
            xa, wqkv, wperm, woa, qa, ka, va, stage0, stage1,
            sem_w, sem_c, sem_x, sem_in, sem_woa, sem_out, *, bq, ra, ro):
    xa32, wqkv32, woa32 = (r.bitcast(U32) for r in (xa_hbm, wqkv_hbm, woa_hbm))
    xb32, c32, wob32 = (r.bitcast(U32) for r in (xb_hbm, c_hbm, wob_hbm))
    wq32, wk32, wv32 = (r.bitcast(U32) for r in (wq_hbm, wuk_hbm, wuv_hbm))

    NCH = 8
    RC = S // NCH

    def cp_wq(p): return pltpu.make_async_copy(wq32.at[:, p, :], wq.at[p], sem_w.at[0, p])
    def cp_wk(p): return pltpu.make_async_copy(wk32.at[:, p, :], wk.at[p], sem_w.at[1, p])
    def cp_wv(p): return pltpu.make_async_copy(wv32.at[:, p, :], wv.at[p], sem_w.at[2, p])
    def cp_c(i):
        r = pl.ds(i * RC // 2, RC // 2)
        return pltpu.make_async_copy(c32.at[r, :], cc.at[r, :], sem_c.at[i])
    def cp_x(i):
        r = pl.ds(i * RC // 2, RC // 2)
        return pltpu.make_async_copy(xb32.at[r, :], xb.at[r, :], sem_x.at[i])
    cp_wqkv = pltpu.make_async_copy(wqkv32, wqkv, sem_in.at[0])
    cp_xa = pltpu.make_async_copy(xa32, xa, sem_in.at[1])
    cp_wob = pltpu.make_async_copy(wob32, wob, sem_in.at[2])
    def cp_woa(n):
        d321, h10, d4 = n >> 3, (n >> 1) & 3, n & 1
        r = h10 * 16 + d4 * 8 + d321
        return pltpu.make_async_copy(woa32.at[:, r, :], woa.at[pl.ds(8 * n, 8), :], sem_woa)

    qscale = DB ** -0.5 * LOG2E

    def proj_kv(p, hi, r0, nr, kd, vd):
        w = jnp.concatenate([_half(wk[p], hi), _half(wv[p], hi)], axis=1)
        kv = _dot(_as_bf16(cc[pl.ds(r0 // 2, nr // 2), :]), w).astype(BF16)
        kd[pl.ds(r0, nr), :] = kv[:, :DB]
        vd[pl.ds(r0, nr), :] = kv[:, DB:]

    def proj_q(p, hi, r0, nr, qd):
        q = _dot(_as_bf16(xb[pl.ds(r0 // 2, nr // 2), :]), _half(wq[p], hi))
        qd[pl.ds(r0, nr), :] = (q * qscale).astype(BF16)

    def attend(h, qs, ks, vs, filler):
        n = S // bq

        def qk(i):
            kv = (i + 1) * bq
            s = jax.lax.dot_general(qs[i * bq:(i + 1) * bq, :], ks[:kv, :], NT,
                                    preferred_element_type=F32)
            row = jax.lax.broadcasted_iota(jnp.int32, (bq, bq), 0)
            col = jax.lax.broadcasted_iota(jnp.int32, (bq, bq), 1)
            sd = jnp.where(col <= row, s[:, kv - bq:], NEG)
            s = jnp.concatenate([s[:, :kv - bq], sd], axis=1) if i else sd
            return s, jnp.max(s, axis=1, keepdims=True)

        def pv(i, s, m):
            kv = (i + 1) * bq
            p = jnp.exp2(s - m)
            l = jnp.sum(p, axis=1, keepdims=True)
            o = _dot(p.astype(BF16), vs[:kv, :])
            ctx[h, i * bq:(i + 1) * bq, :] = (o * (1.0 / l)).astype(BF16)

        prev = qk(0)
        for i in range(n):
            nxt = qk(i + 1) if i + 1 < n else None
            filler(i)
            pv(i, *prev)
            prev = nxt

    cp_wk(0).start()
    cp_wv(0).start()
    for i in range(NCH):
        cp_c(i).start()
    cp_wq(0).start()
    for i in range(NCH):
        cp_x(i).start()
    cp_wk(0).wait()
    cp_wv(0).wait()
    for i in range(NCH):
        cp_c(i).wait()
        proj_kv(0, False, i * RC, RC, k0, v0)
    for cp in (cp_wq(1), cp_wk(1), cp_wv(1)):
        cp.start()
    cp_wq(0).wait()
    for i in range(NCH):
        cp_x(i).wait()
        proj_q(0, False, i * RC, RC, q0)
    cp_wqkv.start()

    def pair_body(p, last):
        @pl.when(p + 2 < HB // 2)
        def _():
            for cp in (cp_wq(p + 2), cp_wk(p + 2), cp_wv(p + 2)):
                cp.start()

        @pl.when(p == 1)
        def _():
            cp_xa.start()

        @pl.when(p == 2)
        def _():
            cp_wob.start()

        @pl.when(p == 3)
        def _():
            for n in range(64):
                cp_woa(n).start()

        if not last:
            for cp in (cp_wq(p + 1), cp_wk(p + 1), cp_wv(p + 1)):
                cp.wait()

        def fill0(i):
            proj_kv(p, True, i * bq, bq, k1, v1)
            proj_q(p, True, i * bq, bq, q1)

        def fill1(i):
            if not last:
                proj_kv(p + 1, False, i * bq, bq, k0, v0)
                proj_q(p + 1, False, i * bq, bq, q0)

        attend(2 * p, q0, k0, v0, fill0)
        attend(2 * p + 1, q1, k1, v1, fill1)

    jax.lax.fori_loop(0, HB // 2 - 1, lambda p, _: pair_body(p, False), None)
    cp_wqkv.wait()
    for g in range(3):
        for r in range(0, 512, 64):
            chunks = [wqkv[r:r + 64, g * DM + c * 128:g * DM + (c + 1) * 128] for c in range(8)]
            for j, x in enumerate(_swap_lane_and_chunk_bits(chunks)):
                wperm[r:r + 64, g * DM + j * 128:g * DM + (j + 1) * 128] = x
    pair_body(HB // 2 - 1, True)

    cp_xa.wait()
    for n in range(64):
        cp_woa(n).wait()
    stages = (stage0, stage1)

    def cp_out(slot, r0, nr, col):
        return pltpu.make_async_copy(stages[slot],
                                     out_hbm.at[pl.ds(r0, nr), pl.ds(col, DM)], sem_out.at[slot])

    ascale = DA ** -0.5 * LOG2E
    ka[:, 0:16, :] = jnp.zeros((8, 16, 128), F32)
    va[:, 0:16, :] = jnp.zeros((8, 16, 128), F32)

    def a_block(i, slot):
        x = _as_bf16(xa[pl.ds(pl.multiple_of(i * (ra // 2), ra // 2), ra // 2), :])
        k = _dot(x, _as_bf16(wperm[:, DM:2 * DM]))
        for j in range(8):
            ka[j, 16:, :] = k[:, j * 128:(j + 1) * 128]
        q = _dot(x, _as_bf16(wperm[:, :DM])) * ascale
        v = _dot(x, _as_bf16(wperm[:, 2 * DM:]))
        for j in range(8):
            va[j, 16:, :] = v[:, j * 128:(j + 1) * 128]
        lane = jax.lax.broadcasted_iota(jnp.int32, (ra, 128), 1)
        pos = jax.lax.broadcasted_iota(jnp.int32, (ra, 128), 0) + i * ra
        logits = []
        for w in range(WIN):
            o = 16 - DIL * w
            t = q[:, 0:128] * ka[0, o:o + ra, :]
            for j in range(1, 8):
                t = t + q[:, j * 128:(j + 1) * 128] * ka[j, o:o + ra, :]
            for b in (16, 1):
                t = t + jnp.where((lane & b) != 0, pltpu.roll(t, b, 1), pltpu.roll(t, 128 - b, 1))
            logits.append(jnp.where(pos >= DIL * w, t, NEG) if w else t)
        m = functools.reduce(jnp.maximum, logits)
        es = [jnp.exp2(t - m) for t in logits]
        inv = 1.0 / functools.reduce(jnp.add, es)
        ps = [e * inv for e in es]
        os = []
        for j in range(8):
            acc = ps[0] * va[j, 16:16 + ra, :]
            for w in range(1, WIN):
                o = 16 - DIL * w
                acc = acc + ps[w] * va[j, o:o + ra, :]
            os.append(acc.astype(BF16))
        y = _dot(jnp.concatenate(os, axis=1), _as_bf16(woa[...]))
        stages[slot][...] = y.astype(BF16)
        ka[:, 0:16, :] = ka[:, ra:ra + 16, :]
        va[:, 0:16, :] = va[:, ra:ra + 16, :]

    def a_pair(t, _):
        for slot in range(2):
            @pl.when(t > 0)
            def _():
                cp_out(slot, 0, ra, 0).wait()
        for slot in range(2):
            a_block(2 * t + slot, slot)
        for slot in range(2):
            cp_out(slot, pl.multiple_of((2 * t + slot) * ra, ra), ra, 0).start()

    jax.lax.fori_loop(0, S // ra // 2, a_pair, None)

    cp_wob.wait()

    def o_pair(t, _):
        for slot in range(2):
            cp_out(slot, 0, ro, 0).wait()
        for slot in range(2):
            r0 = pl.multiple_of((2 * t + slot) * ro, ro)
            lhs = jnp.concatenate([ctx[h, pl.ds(r0, ro), :] for h in range(HB)], axis=1)
            stages[slot][...] = _dot(lhs, _as_bf16(wob[...])).astype(BF16)
        for slot in range(2):
            cp_out(slot, pl.multiple_of((2 * t + slot) * ro, ro), ro, DM).start()

    jax.lax.fori_loop(0, S // ro // 2, o_pair, None)
    for slot in range(2):
        cp_out(slot, 0, ro, 0).wait()


def build(bq, ra, ro):
    assert ra == ro
    vm = pltpu.VMEM
    dma = pltpu.SemaphoreType.DMA
    scratch = [
        vm((S // 2, DM), U32), vm((S // 2, DC), U32),
        vm((HB // 2, DM, DB), U32), vm((HB // 2, DC, DB), U32), vm((HB // 2, DC, DB), U32),
        *[vm((S, DB), BF16) for _ in range(6)],
        vm((HB, S, DB), BF16), vm((HB * DB // 2, DM), U32),
        vm((S // 2, DM), U32), vm((DM // 2, 3 * DM), U32), vm((DM // 2, 3 * DM), U32),
        vm((DM // 2, DM), U32),
        vm((8, ra, 128), F32), vm((8, 16 + ra, 128), F32), vm((8, 16 + ra, 128), F32),
        vm((ra, DM), BF16), vm((ra, DM), BF16),
        dma((3, HB // 2)), dma((8,)), dma((8,)), dma((3,)), dma(()), dma((2,)),
    ]

    @jax.jit
    def run(A_x, A_wqkv, A_wo, B_x, B_c_kv, B_w_q, B_w_uk, B_w_uv, B_w_o):
        out = pl.pallas_call(
            functools.partial(_kernel, bq=bq, ra=ra, ro=ro),
            out_shape=jax.ShapeDtypeStruct((S, 2 * DM), BF16),
            in_specs=[pl.BlockSpec(memory_space=pl.ANY)] * 9,
            out_specs=pl.BlockSpec(memory_space=pl.ANY),
            scratch_shapes=scratch,
            compiler_params=pltpu.CompilerParams(vmem_limit_bytes=120 * 2**20),
            name="fused",
        )(A_x.reshape(S, DM), A_wqkv, A_wo.reshape(8, DM // 8, DM),
          B_x.reshape(S, DM), B_c_kv.reshape(S, DC), B_w_q, B_w_uk, B_w_uv,
          B_w_o.reshape(HB * DB, DM))
        return out.reshape(1, S, 2 * DM)

    return run


@jax.jit
def pallas_concat_heads__sliding_local_dilated__compressed_kv_cla__prompt_kernel(
    A_x: jax.Array,
    A_wqkv: jax.Array,
    A_wo: jax.Array,
    B_x: jax.Array,
    B_c_kv: jax.Array,
    B_w_q: jax.Array,
    B_w_uk: jax.Array,
    B_w_uv: jax.Array,
    B_w_o: jax.Array,
):
    return build(**CFG)(A_x, A_wqkv, A_wo, B_x, B_c_kv, B_w_q, B_w_uk, B_w_uv, B_w_o)
```

```python
import functools
import math

import jax
import jax.numpy as jnp
from jax.experimental import pallas as pl
from jax.experimental.pallas import tpu as pltpu

S = 2048
DM = 1024
HA, DA = 32, 32
WIN, DIL = 8, 2
HB, DB = 32, 128
DC = 512
NEG = -1e9
LOG2E = math.log2(math.e)

GH = 4
NG = HB // GH
SET = S // GH
RO = 256
HALO = 16
NP = 49
TILE = 64

F32, BF16, U32 = jnp.float32, jnp.bfloat16, jnp.uint32
NT = (((1,), (1,)), ((), ()))

CFG = dict(ph="pfhlr", vlag=7, ch=4, lag=8, nx=12, age=6, ager=4, lw=8, lj=8, tail=49, st=0, pin=20, sa=2, run=7)

AT_SLAB = 2 * NP * 4 * TILE
AT_CTX = AT_SLAB + 8 * TILE
RA = RO // 8


def _b16(x32):
    return pltpu.bitcast(x32, BF16)


def _pack2(lo, hi):
    return pltpu.pack_elementwise([lo, hi], packed_dtype=BF16)


def _halves(w):
    return jnp.concatenate([pltpu.unpack_elementwise(w, index=i, packed_dtype=BF16, unpacked_dtype=F32)
                            for i in range(2)], axis=0)


def _words(x):
    n = x.shape[0] // 2
    return _pack2(x[:n], x[n:])


def _shuffled(x):
    parts = [_pack2(x[r:r + 8], x[r + 8:r + 16]) for r in range(0, x.shape[0], 16)]
    return jnp.concatenate(parts, axis=0) if len(parts) > 1 else parts[0]


def _dot(a32, b32):
    return jnp.dot(_b16(a32), _b16(b32), preferred_element_type=F32)


def _recip(x):
    r = pl.reciprocal(x, approx=True)
    return r * (2.0 - x * r)


def _rows(start, size, align=None):
    return pl.ds(start if isinstance(start, int) else pl.multiple_of(start, align or size), size)


def _fold(f, x):
    return functools.reduce(f, [x[:, c:c + 128] for c in range(0, x.shape[1], 128)])


def _quads(x):
    n = len(x) // 2
    return ([r[:n] for r in x[:n]], [r[n:] for r in x[:n]],
            [r[:n] for r in x[n:]], [r[n:] for r in x[n:]])


def _add(x, y):
    return [[a + b for a, b in zip(r, s)] for r, s in zip(x, y)]


def _sub(x, y):
    return [[a - b for a, b in zip(r, s)] for r, s in zip(x, y)]


def _lhs_term(x, i):
    a11, a12, a21, a22 = _quads(x)
    return (lambda: _sub(a12, a22), lambda: _sub(a21, a11), lambda: _add(a11, a22), lambda: a22,
            lambda: a11, lambda: _add(a21, a22), lambda: _add(a11, a12))[i]()


def _rhs_term(x, i):
    b11, b12, b21, b22 = _quads(x)
    return (lambda: _add(b21, b22), lambda: _add(b11, b12), lambda: _add(b11, b22), lambda: _sub(b21, b11),
            lambda: _sub(b12, b22), lambda: b11, lambda: b22)[i]()


def _seven(term, x, i):
    y = term(x, i)
    return [(7 * i + j, term(y, j)[0][0]) for j in range(7)]


def _combine(product, level=2, base=0):
    if level == 0:
        return [[(yield from product(base))]]
    k = 7 ** (level - 1)
    m7 = yield from _combine(product, level - 1, base)
    m6 = yield from _combine(product, level - 1, base + k)
    m1 = yield from _combine(product, level - 1, base + 2 * k)
    c11 = _add(m7, m1)
    c22 = _add(m6, m1)
    m4 = yield from _combine(product, level - 1, base + 3 * k)
    c11 = _add(c11, m4)
    m3 = yield from _combine(product, level - 1, base + 4 * k)
    c22 = _add(c22, m3)
    m2 = yield from _combine(product, level - 1, base + 5 * k)
    c21 = _add(m2, m4)
    c22 = _sub(c22, m2)
    m5 = yield from _combine(product, level - 1, base + 6 * k)
    c11 = _sub(c11, m5)
    c12 = _add(m3, m5)
    return [r + s for r, s in zip(c11, c12)] + [r + s for r, s in zip(c21, c22)]


def _drain(gen):
    while True:
        try:
            next(gen)
        except StopIteration as e:
            return e.value


def _chain(*gens):
    for g in gens:
        yield from g


def _woven(main, count, side, side_count):
    done = 0
    for i in range(count):
        while done < side_count and done * count < (i + 1) * side_count:
            next(side)
            done += 1
        next(main)
        yield
    _drain(side)


class _Pace:
    def __init__(self, zero, age):
        self.zero, self.age, self.recent = zero, age, []

    def note(self, y):
        self.recent.append(y[:, -128:])
        return y

    def after(self):
        if len(self.recent) < self.age:
            return lambda x: x
        bits = pltpu.bitcast(self.recent[-self.age][:8], U32) & self.zero
        return lambda x: pltpu.bitcast(pltpu.bitcast(x, U32) | bits, x.dtype)

    def tied(self, x, y):
        zero = jnp.concatenate([self.zero] * (x.shape[0] // 8), axis=0)
        return pltpu.bitcast(pltpu.bitcast(x, U32) | (pltpu.bitcast(y, U32) & zero), x.dtype)

    def blocks(self, load):
        tie = self.after()
        return [[tie(load(i, j)) if i % 2 == 0 and j % 2 == 0 else load(i, j) for j in range(4)]
                for i in range(4)]


def _swap_lane_and_chunk_bits(chunks):
    lane = jax.lax.broadcasted_iota(jnp.int32, chunks[0].shape, 1)
    u = (lane >> 1) & 7
    rolled = [x if c == 0 else pltpu.roll(x, 2 * c, 1) for c, x in enumerate(chunks)]
    xs = [rolled[(-i) % 8] for i in range(8)]
    for t in (1, 2, 4):
        m = (u & t) != 0
        xs = [jnp.where(m, xs[(i - t) % 8], xs[i]) for i in range(8)]
    return [x if j == 0 else pltpu.roll(x, 128 - 2 * j, 1) for j, x in enumerate(xs)]


def _kernel(xa_hbm, wqkv_hbm, woa_hbm, xb_hbm, c_hbm, wq_hbm, wuk_hbm, wuv_hbm, wob_hbm,
            out_hbm,
            hs, wo, wa, wo_raw, wa_raw,
            sem_wo, sem_wa, *, ph, vlag, ch, lag, nx, age, ager, lw, lj, tail, st, pin, sa, run):
    xa32, wqkv32, woa32 = (r.bitcast(U32) for r in (xa_hbm, wqkv_hbm, woa_hbm))
    xb32, c32, wob32 = (r.bitcast(U32) for r in (xb_hbm, c_hbm, wob_hbm))
    wq32, wk32, wv32 = (r.bitcast(U32) for r in (wq_hbm, wuk_hbm, wuv_hbm))

    def ctx_rows(page, row, n):
        return _rows(AT_CTX + page * (S // 2) + row, n)

    def pace(step, age):
        return _Pace(jnp.full((8, 128), step // S, jnp.int32).astype(U32), age)

    def zero(step, salt):
        return step // (S + salt)

    def cp_wo(g):
        return pltpu.make_async_copy(wob32.at[pl.ds(g * GH, GH)], wo_raw.at[g % 2], sem_wo.at[g % 2])

    def cp_wa(m):
        return pltpu.make_async_copy(wqkv32.at[:, _rows(m * DM, DM)], wa_raw.at[m % 2], sem_wa.at[m % 2])

    def cp_woa(n):
        d321, h10, d4 = n >> 3, (n >> 1) & 3, n & 1
        return pltpu.make_async_copy(woa32.at[:, h10 * 16 + d4 * 8 + d321, :],
                                     wa_raw.at[1, _rows(8 * n, 8), :], sem_wa.at[1])

    def prep_slabs(pc, u, load, store):
        for half in range(2):
            for c in range(2):
                for i in range(7):
                    z = zero(u, i)
                    x = pc.blocks(lambda k, j: load(z, k, half * 8, 2 * j + c))
                    for n, y in _seven(_rhs_term, [[_halves(w) for w in r] for r in x], i):
                        store(n, half * 8, c, _words(y))
                    yield

    def prep_wo(pc, u):
        def store(n, row, c, y):
            wo[n, _rows(u * 16 + row, 8), c * 128:(c + 1) * 128] = y
        return prep_slabs(
            pc, u, lambda z, k, row, c: wo_raw[u // GH % 2 + z, k, _rows(u % GH * 16 + row, 8), c * 128:(c + 1) * 128], store)

    def permute_wa(pc, u):
        for i in range(4):
            for half in range(2):
                tie = pc.after()
                raw = [tie(wa_raw[u // 8 % 2, _rows(i * 128 + u % 8 * 16 + half * 8, 8), c * 128:(c + 1) * 128])
                       for c in range(8)]
                for c, y in enumerate(_swap_lane_and_chunk_bits(raw)):
                    hs[pl.ds(AT_SLAB + c * TILE + i * 16 + half * 8, 8), :] = jnp.where(u < 24, y, raw[c])
                yield

    def prep_wa(pc, u):
        def store(n, row, c, y):
            wa[u // 8, n, _rows(u % 8 * 16 + row, 8), c * 128:(c + 1) * 128] = y
        return prep_slabs(
            pc, u, lambda z, k, row, c: hs[_rows(AT_SLAB + (c + z) * TILE + k * 16 + row, 8), :], store)

    def heads(xc, cc, wq_raw, wkv_raw, qs, ks, vs, sem_w, sem_x):
        def cp_w(g):
            cps = []
            for i in range(2):
                p = 2 * g + i
                cps.append(pltpu.make_async_copy(wk32.at[:, p, :], wkv_raw.at[g % 2, 0, i], sem_w.at[g % 2, 0, i]))
                cps.append(pltpu.make_async_copy(wv32.at[:, p, :], wkv_raw.at[g % 2, 1, i], sem_w.at[g % 2, 1, i]))
            for i in range(2):
                cps.append(pltpu.make_async_copy(wq32.at[:, 2 * g + i, :], wq_raw.at[g % 2, i], sem_w.at[g % 2, 2, i]))
            return cps

        def cp_rows(j):
            r = _rows(j * (SET // 2), SET // 2)
            return [pltpu.make_async_copy(src.at[r, t * 128:(t + 1) * 128],
                                          hs.at[ctx_rows(page + t, j * (SET // 2), SET // 2), :], sem_x.at[j])
                    for page, src in ((0, c32), (4, xb32)) for t in range(src.shape[1] // 128)]

        def prep_rows(pc, page, dst, j, starts=range(0, SET // 8, 8)):
            r, tiles = SET // 8, dst.shape[-1] // 128
            for a in starts:
                for t in range(tiles):
                    for i in range(7):
                        z = zero(j, i)
                        x = pc.blocks(lambda b, k: hs[ctx_rows(page + k * tiles + t + z, j * (SET // 2) + b * r + a, 8), :])
                        for n, y in _seven(_lhs_term, [[_b16(w).astype(F32) for w in row] for row in x], i):
                            dst[n, _rows(j * r + a, 8), t * 128:(t + 1) * 128] = _shuffled(y)
                        yield

        def prep_w(pc, g, j):
            def unit(raw, depth, a, row):
                for i in range(7):
                    z = zero(j, i)
                    x = pc.blocks(lambda k, c: raw[
                        c // 2 + z, pl.ds(k * (depth // 4) + j * (depth // 16) + a + c % 2, 8, stride=2), :])
                    x = [[_halves(w) for w in r] for r in x]
                    x = [[jnp.concatenate([r[c // 2 * 2][c % 2 * 8:c % 2 * 8 + 8],
                                           r[c // 2 * 2 + 1][c % 2 * 8:c % 2 * 8 + 8]], axis=0)
                          for c in range(4)] for r in x]
                    for n, y in _seven(_rhs_term, x, i):
                        hs[_rows((g % 2 * NP + n) * 4 * TILE + row, 8), :] = _words(y)
                    yield

            for a in range(0, DM // 16, 16):
                yield from unit(wq_raw.at[g % 2], DM, a, j * (DM // 32) + a // 2)
            for kind in range(2):
                for a in range(0, DC // 16, 16):
                    yield from unit(wkv_raw.at[g % 2, kind], DC, a, (2 + kind) * TILE + j * (DC // 32) + a // 2)

        def project(pc, g, j):
            r = SET // 8
            rows = _rows(j * r, r)

            def product(lhs, first, last):
                def run(n):
                    y = pc.note(_dot(lhs[n, rows, :], hs[_rows(((g % 2 * NP + n) * 4 + first) * TILE, (last - first) * TILE, TILE), :]))
                    yield
                    return y
                return _combine(run)

            q, k, v = product(xc, 0, 2), product(cc, 2, 3), product(cc, 3, 4)
            for n in range(0, NP, run):
                for gen in (q, k, v):
                    for _ in range(min(run, NP - n)):
                        next(gen)
                        yield
            q, k, v = _drain(q), _drain(k), _drain(v)
            for i in range(4):
                dst = _rows(j * (SET // 2) + i * r, r)
                for h in range(GH):
                    slot = g % 2 * GH + h
                    qs[slot, dst, :] = _shuffled(q[i][h] * (DB ** -0.5 * LOG2E))
                    ks[slot, dst, :] = _shuffled(k[i][h])
                    vs[slot, dst, :] = _shuffled(v[i][h])

        def attend(pc, h, filler, fill_steps):
            slot = h % (2 * GH)
            nb = S // 128
            work = [(i, t, min(t + ch, i + 1)) for i in reversed(range(nb)) for t in range(0, i + 1, ch)]
            s, mx, m, l, o, done, ready = {}, {}, {}, {}, {}, {}, []

            def scores(i, t0, t1):
                x = pc.note(jax.lax.dot_general(_b16(qs[slot, i * TILE:(i + 1) * TILE, :]),
                                                _b16(ks[slot, t0 * TILE:t1 * TILE, :]), NT,
                                                preferred_element_type=F32))
                if t1 == i + 1:
                    row, col = (jax.lax.broadcasted_iota(jnp.int32, (128, 128), d) for d in range(2))
                    row, col = ((u & ~15) | ((u >> 2) & 3) | ((u & 3) << 2) for u in (row, col))
                    diag = jnp.where(col <= row, x[:, -128:], NEG)
                    x = jnp.concatenate([x[:, :-128], diag], axis=1) if t1 - t0 > 1 else diag
                s[i, t0] = x
                mx[i] = jnp.maximum(mx[i], _fold(jnp.maximum, x)) if t0 else _fold(jnp.maximum, x)
                if t1 == i + 1:
                    m[i] = jnp.max(mx[i], axis=1, keepdims=True)

            def values(i, t0, t1):
                p = jnp.exp2(s.pop((i, t0)) - m[i])
                y = pc.note(jnp.dot(p.astype(BF16), _b16(vs[slot, t0 * TILE:t1 * TILE, :]),
                                    preferred_element_type=F32))
                parts = ([l[i]] if t0 else []) + [p[:, c:c + 128] for c in range(0, p.shape[1], 128)]
                l[i] = functools.reduce(jnp.add, [pc.tied(parts[0], pc.recent[-1 - sa])] + parts[1:])
                o[i] = o[i] + y if t0 else y
                if t1 == i + 1:
                    ready.append((clock + pin, i, _shuffled(o[i] * _recip(jnp.sum(l[i], axis=1, keepdims=True)))))

            def finish():
                while ready and ready[0][0] <= clock:
                    _, i, x = ready.pop(0)
                    hs[ctx_rows(h, i * TILE, TILE), :] = x

            total = 2 * sum(t1 - t0 for _, t0, t1 in work)
            clock = attn = filled = qi = pi = turn = 0
            while pi < len(work):
                can = work[pi][0] in done and clock - done[work[pi][0]] >= lag
                if filled < fill_steps and (filled * total <= attn * fill_steps
                                            or (qi == len(work) and not can)):
                    for _ in range(min(vlag, fill_steps - filled)):
                        next(filler)
                        filled += 1
                        clock += 4 / 3
                elif qi < len(work) and (not can or turn == 0):
                    scores(*work[qi])
                    clock += work[qi][2] - work[qi][1]
                    attn += work[qi][2] - work[qi][1]
                    if work[qi][2] == work[qi][0] + 1:
                        done[work[qi][0]] = clock
                    qi, turn = qi + 1, 1
                else:
                    values(*work[pi])
                    clock += work[pi][2] - work[pi][1]
                    attn += work[pi][2] - work[pi][1]
                    pi, turn = pi + 1, 0
                finish()
            for _ in filler or ():
                clock += 4 / 3
                finish()
            clock += pin
            finish()

        for cp in cp_w(0) + cp_rows(0) + cp_rows(1) + cp_w(1) + [cp_wo(0), cp_wa(0)]:
            cp.start()
        for cp in cp_w(0):
            cp.wait()
        if "p" in ph:
            jax.lax.fori_loop(0, GH, lambda j, _: _drain(prep_w(pace(j, 1), 0, j)), None)
        for cp in cp_rows(0):
            cp.wait()

        def first_rows(a, _):
            _drain(prep_rows(pace(a, 1), 0, cc, 0, [a * 8]))
            _drain(prep_rows(pace(a, 1), 4, xc, 0, [a * 8]))
        if "p" in ph:
            jax.lax.fori_loop(0, SET // 64, first_rows, None)
        for cp in cp_w(1):
            cp.wait()

        def later_weights(pc, u):
            @pl.when(u % GH == 0)
            def _():
                @pl.when(u // GH + 1 < NG)
                def _():
                    cp_wo(u // GH + 1).start()
                cp_wo(u // GH).wait()

                @pl.when((u == 0) | (u == 8))
                def _():
                    cp_wa(u // 8 + 1).start()

                @pl.when(u == 16)
                def _():
                    jax.lax.fori_loop(0, 64, lambda n, _: cp_woa(n).start(), None)

                @pl.when((u % 8 == 0) & (u < 24))
                def _():
                    cp_wa(u // 8).wait()

                @pl.when(u == 24)
                def _():
                    jax.lax.fori_loop(0, 64, lambda n, _: cp_woa(n).wait(), None)
            return _chain(_woven(prep_wo(pc, u), 28, permute_wa(pc, u), 8), prep_wa(pc, u))

        def first_group(j, _):
            @pl.when(j + 2 < GH)
            def _():
                for cp in cp_rows(j + 2):
                    cp.start()

            @pl.when(j == 1)
            def _():
                for cp in cp_w(2):
                    cp.start()

            @pl.when(j + 1 < GH)
            def _():
                for cp in cp_rows(j + 1):
                    cp.wait()

            nxt = jnp.minimum(j + 1, GH - 1)
            pc = pace(j, age)
            side = _chain(later_weights(pc, j), prep_rows(pc, 0, cc, nxt), prep_w(pc, 1, j), prep_rows(pc, 4, xc, nxt))
            main = project(pc, 0, j)
            _drain(_woven(main, 3 * NP, side, 280))
            _drain(main)
        if "f" in ph:
            jax.lax.fori_loop(0, GH, first_group, None)

        def head(h, _):
            g, j = h // GH, h % GH

            @pl.when(j == 0)
            def _():
                @pl.when(g + 3 < NG)
                def _():
                    for cp in cp_w(g + 3):
                        cp.start()

                @pl.when(g + 2 < NG)
                def _():
                    for cp in cp_w(g + 2):
                        cp.wait()

            pc = pace(h, age)
            side = _chain(later_weights(pc, h + GH), prep_w(pc, g + 2, j))
            main = project(pc, g + 1, j)
            filler = _woven(main, 3 * NP - st, side, 112)
            attend(pc, h, filler, 3 * NP - tail)
            _drain(main)
        if "h" in ph:
            jax.lax.fori_loop(0, HB - GH, head, None)

        if "l" in ph:
            jax.lax.fori_loop(HB - GH, HB, lambda h, _: attend(pace(h, age), h, None, 0), None)

    vm, dma = pltpu.VMEM, pltpu.SemaphoreType.DMA
    pl.run_scoped(
        heads,
        vm((NP, S // 8, DM // 4), U32), vm((NP, S // 8, DC // 4), U32),
        vm((2, 2, DM, DB), U32), vm((2, 2, 2, DC, DB), U32),
        *[vm((2 * GH, S // 2, DB), U32) for _ in range(3)],
        dma((2, 3, 2)), dma((GH,)))

    def rows_phase(oc, xac, oac, qa, ka, va, ya, xa_raw, stage, sem_xa, sem_out):
        def cp_xa(t):
            return pltpu.make_async_copy(xa32.at[_rows(t * (RO // 2), RO // 2), :],
                                         xa_raw.at[t % 3], sem_xa.at[t % 3])

        def cp_out(t, part):
            at = (_rows(t * RO, RO), pl.ds(part * DM, DM))
            return pltpu.make_async_copy(stage.at[at], out_hbm.at[at], sem_out.at[part, t])

        def prep_ctx(pc, t, i, groups=range(NG)):
            for a in range(0, RA, 8):
                for p in groups:
                    z = zero(t, i)
                    x = pc.blocks(lambda b, k: hs[ctx_rows(p * GH + k + z, t * (RO // 2) + b * RA + a, 8), :])
                    for n, y in _seven(_lhs_term, [[_b16(w).astype(F32) for w in row] for row in x], i):
                        oc[n, a:a + 8, _rows(p * 128, 128)] = _shuffled(y)
                    yield

        def prep_xa(pc, t, i):
            for a in range(0, RA, 8):
                for c in range(2):
                    slot = t % 3 + zero(t, i)
                    x = pc.blocks(lambda b, k: xa_raw[slot, b * RA + a:b * RA + a + 8, (2 * k + c) * 128:(2 * k + c + 1) * 128])
                    for n, y in _seven(_lhs_term, [[_halves(w) for w in row] for row in x], i):
                        xac[n, a:a + 8, c * 128:(c + 1) * 128] = _words(y)
                    yield

        def local_attention(pc, t):
            lane = jax.lax.broadcasted_iota(jnp.int32, (8, 128), 1)
            for a in range(0, RO, 8):
                logits = []
                for w in range(WIN):
                    if w % lw == 0:
                        tie = pc.after()
                        q = [tie(qa[j, a:a + 8, :]) for j in range(8)]
                    b = a + HALO - DIL * w
                    x = q[0] * ka[0, b:b + 8, :]
                    for j in range(1, 8):
                        x = x + q[j] * ka[j, b:b + 8, :]
                    for bit in (16, 1):
                        x = x + jnp.where((lane & bit) != 0, pltpu.roll(x, bit, 1), pltpu.roll(x, 128 - bit, 1))
                    if a < DIL * w:
                        pos = jax.lax.broadcasted_iota(jnp.int32, (8, 128), 0) + (t * RO + a)
                        x = jnp.where(pos >= DIL * w, x, NEG)
                    logits.append(x)
                    if w % lw == lw - 1:
                        yield
                top = functools.reduce(jnp.maximum, logits)
                es = [jnp.exp2(x - top) for x in logits]
                inv = _recip(functools.reduce(jnp.add, es))
                ps = [e * inv for e in es]
                for j in range(8):
                    if j % lj == 0 and lj < 8:
                        tie = pc.after()
                        ps = [tie(p) for p in ps]
                    acc = ps[0] * va[j, a + HALO:a + HALO + 8, :]
                    for w in range(1, WIN):
                        b = a + HALO - DIL * w
                        acc = acc + ps[w] * va[j, b:b + 8, :]
                    ya[j, a:a + 8, :] = acc
                    if j % lj == lj - 1:
                        yield
            ka[:, 0:HALO, :] = ka[:, RO:, :]
            va[:, 0:HALO, :] = va[:, RO:, :]
            for i in range(7):
                for a in range(0, RA, 8):
                    for c in range(2):
                        z = zero(t, i)
                        x = [pc.blocks(lambda b, k: ya[2 * k + c + z, pl.ds(2 * (b * RA + a) + e, 8, stride=2), :])
                             for e in range(2)]
                        x = [[jnp.concatenate(w, axis=0) for w in zip(*rows)] for rows in zip(*x)]
                        for n, y in _seven(_lhs_term, x, i):
                            oac[n, a:a + 8, c * 128:(c + 1) * 128] = _words(y)
                        yield

        def joined(c):
            return jnp.concatenate([jnp.concatenate(row, axis=1) for row in c], axis=0)

        steps = S // RO
        cp_xa(0).start()
        cp_xa(1).start()
        ka[:, 0:HALO, :] = jnp.zeros((8, HALO, 128), F32)
        va[:, 0:HALO, :] = jnp.zeros((8, HALO, 128), F32)

        def first_ctx(p, _):
            for i in range(7):
                _drain(prep_ctx(pace(p, 1), 0, i, [p]))
        if "p" in ph:
            jax.lax.fori_loop(0, NG, first_ctx, None)
        cp_xa(0).wait()
        if "p" in ph:
            for i in range(7):
                _drain(prep_xa(pace(0, 1), 0, i))

        def step(t, _):
            nxt = jnp.minimum(t + 1, steps - 1)
            pc = pace(t, ager)

            @pl.when(t + 2 < steps)
            def _():
                cp_xa(t + 2).start()

            @pl.when(t + 1 < steps)
            def _():
                cp_xa(t + 1).wait()

            def times(lhs, w):
                def run(n):
                    y = None
                    for k in range(lhs.shape[2] // 256):
                        z = pc.note(_dot(lhs[n, :, k * 256:(k + 1) * 256], w[n, k * 128:(k + 1) * 128, :]))
                        y = z if y is None else y + z
                        yield
                    return y
                return _combine(run)

            k = joined(_drain(times(xac, wa.at[1])))
            for j in range(8):
                ka[j, HALO:, :] = k[:, j * 128:(j + 1) * 128]
            q = joined(_drain(times(xac, wa.at[0]))) * (DA ** -0.5 * LOG2E)
            for j in range(8):
                qa[j] = q[:, j * 128:(j + 1) * 128]
            v = times(xac, wa.at[2])
            for i in range(7):
                _drain(_woven(v, 7, prep_xa(pc, nxt, i - 1) if i else iter(()), 8 if i else 0))
            v = joined(_drain(v))
            for j in range(8):
                va[j, HALO:, :] = v[:, j * 128:(j + 1) * 128]

            b = times(oc, wo)
            _drain(_woven(b, nx, prep_xa(pc, nxt, 6), 8))
            rest = _chain(_woven(b, 28 - nx, iter(()), 0),
                          *[_woven(b, 28, prep_ctx(pc, nxt, i - 1), 32) for i in range(1, 7)])
            _drain(_woven(rest, 4 * NP - nx - 6, local_attention(pc, t), 32 * (WIN // lw + 8 // lj) + 56))
            _drain(rest)
            stage[_rows(t * RO, RO), DM:] = joined(_drain(b)).astype(BF16)
            cp_out(t, 1).start()
            y = times(oac, wa.at[3])
            _drain(_woven(y, NP - 7, prep_ctx(pc, nxt, 6), 32))
            stage[_rows(t * RO, RO), 0:DM] = joined(_drain(y)).astype(BF16)
            cp_out(t, 0).start()

        if "r" in ph:
            jax.lax.fori_loop(0, steps, step, None)
        else:
            stage[0:16, 0:128] = _b16(hs[AT_CTX:AT_CTX + 8, :] | wo[0, 0:8, 0:128] | wa[0, 0, 0:8, 0:128])
        for t in range(steps):
            cp_out(t, 1).wait()
            cp_out(t, 0).wait()

    pl.run_scoped(
        rows_phase,
        vm((NP, RA, HB * DB // 4), U32), vm((NP, RA, DM // 4), U32), vm((NP, RA, DM // 4), U32),
        vm((8, RO, 128), F32), vm((8, HALO + RO, 128), F32), vm((8, HALO + RO, 128), F32), vm((8, RO, 128), F32),
        vm((3, RO // 2, DM), U32), vm((S, 2 * DM), BF16),
        dma((3,)), dma((2, S // RO)))


def build(pred=8, **cfg):
    flags = {"XLA_TPU_MAX_INSTS_TO_PREDICATE": pred} if pred is not None else None
    vm, dma = pltpu.VMEM, pltpu.SemaphoreType.DMA
    scratch = [
        vm((AT_CTX + HB * S // 2, 128), U32),
        vm((NP, HB * DB // 8, DM // 4), U32), vm((4, NP, DM // 8, DM // 4), U32),
        vm((2, GH, DB // 2, DM), U32), vm((2, DM // 2, DM), U32),
        dma((2,)), dma((2,)),
    ]

    @jax.jit
    def run(A_x, A_wqkv, A_wo, B_x, B_c_kv, B_w_q, B_w_uk, B_w_uv, B_w_o):
        out = pl.pallas_call(
            functools.partial(_kernel, **cfg),
            out_shape=jax.ShapeDtypeStruct((S, 2 * DM), BF16),
            in_specs=[pl.BlockSpec(memory_space=pl.ANY)] * 9,
            out_specs=pl.BlockSpec(memory_space=pl.ANY),
            scratch_shapes=scratch,
            compiler_params=pltpu.CompilerParams(vmem_limit_bytes=128 * 2**20, flags=flags),
            name="fused",
        )(A_x.reshape(S, DM), A_wqkv, A_wo.reshape(8, DM // 8, DM),
          B_x.reshape(S, DM), B_c_kv.reshape(S, DC), B_w_q, B_w_uk, B_w_uv, B_w_o)
        return out.reshape(1, S, 2 * DM)

    return run


@jax.jit
def pallas_concat_heads__sliding_local_dilated__compressed_kv_cla__prompt_kernel(
    A_x: jax.Array,
    A_wqkv: jax.Array,
    A_wo: jax.Array,
    B_x: jax.Array,
    B_c_kv: jax.Array,
    B_w_q: jax.Array,
    B_w_uk: jax.Array,
    B_w_uv: jax.Array,
    B_w_o: jax.Array,
):
    return build(**CFG)(A_x, A_wqkv, A_wo, B_x, B_c_kv, B_w_q, B_w_uk, B_w_uv, B_w_o)
```

```python
import functools
import math

import jax
import jax.numpy as jnp
from jax.experimental import pallas as pl
from jax.experimental.pallas import tpu as pltpu

S = 2048
DM = 1024
HA, DA = 32, 32
WIN, DIL = 8, 2
HB, DB = 32, 128
DC = 512
NEG = -1e9
LOG2E = math.log2(math.e)

GH = 4
NG = HB // GH
SET = S // GH
RO = 256
HALO = 16
NP = 49
TILE = 64

F32, BF16, U32 = jnp.float32, jnp.bfloat16, jnp.uint32
NT = (((1,), (1,)), ((), ()))

CFG = dict(ph="pfhlr", vlag=7, ch=4, lag=8, nx=6, age=6, ager=6, lw=2, lj=2, tail=49, st=0, pin=20, sa=2, run=7, agel=3, n1=112, n2=6, runf=1, sm=16)

AT_SLAB = 2 * NP * 4 * TILE
AT_CTX = AT_SLAB + 8 * TILE
RA = RO // 8


def _b16(x32):
    return pltpu.bitcast(x32, BF16)


def _pack2(lo, hi):
    return pltpu.pack_elementwise([lo, hi], packed_dtype=BF16)


def _halves(w):
    return jnp.concatenate([pltpu.unpack_elementwise(w, index=i, packed_dtype=BF16, unpacked_dtype=F32)
                            for i in range(2)], axis=0)


def _words(x):
    n = x.shape[0] // 2
    return _pack2(x[:n], x[n:])


def _shuffled(x):
    parts = [_pack2(x[r:r + 8], x[r + 8:r + 16]) for r in range(0, x.shape[0], 16)]
    return jnp.concatenate(parts, axis=0) if len(parts) > 1 else parts[0]


def _dot(a32, b32):
    return jnp.dot(_b16(a32), _b16(b32), preferred_element_type=F32)


def _recip(x):
    r = pl.reciprocal(x, approx=True)
    return r * (2.0 - x * r)


def _rows(start, size, align=None):
    return pl.ds(start if isinstance(start, int) else pl.multiple_of(start, align or size), size)


def _fold(f, x):
    return functools.reduce(f, [x[:, c:c + 128] for c in range(0, x.shape[1], 128)])


def _quads(x):
    n = len(x) // 2
    return ([r[:n] for r in x[:n]], [r[n:] for r in x[:n]],
            [r[:n] for r in x[n:]], [r[n:] for r in x[n:]])


def _add(x, y):
    return [[a + b for a, b in zip(r, s)] for r, s in zip(x, y)]


def _sub(x, y):
    return [[a - b for a, b in zip(r, s)] for r, s in zip(x, y)]


def _lhs_term(x, i):
    a11, a12, a21, a22 = _quads(x)
    return (lambda: _sub(a12, a22), lambda: _sub(a21, a11), lambda: _add(a11, a22), lambda: a22,
            lambda: a11, lambda: _add(a21, a22), lambda: _add(a11, a12))[i]()


def _rhs_term(x, i):
    b11, b12, b21, b22 = _quads(x)
    return (lambda: _add(b21, b22), lambda: _add(b11, b12), lambda: _add(b11, b22), lambda: _sub(b21, b11),
            lambda: _sub(b12, b22), lambda: b11, lambda: b22)[i]()


def _seven(term, x, i):
    y = term(x, i)
    return [(7 * i + j, term(y, j)[0][0]) for j in range(7)]


def _combine(product, level=2, base=0):
    if level == 0:
        return [[(yield from product(base))]]
    k = 7 ** (level - 1)
    m7 = yield from _combine(product, level - 1, base)
    m6 = yield from _combine(product, level - 1, base + k)
    m1 = yield from _combine(product, level - 1, base + 2 * k)
    c11 = _add(m7, m1)
    c22 = _add(m6, m1)
    m4 = yield from _combine(product, level - 1, base + 3 * k)
    c11 = _add(c11, m4)
    m3 = yield from _combine(product, level - 1, base + 4 * k)
    c22 = _add(c22, m3)
    m2 = yield from _combine(product, level - 1, base + 5 * k)
    c21 = _add(m2, m4)
    c22 = _sub(c22, m2)
    m5 = yield from _combine(product, level - 1, base + 6 * k)
    c11 = _sub(c11, m5)
    c12 = _add(m3, m5)
    return [r + s for r, s in zip(c11, c12)] + [r + s for r, s in zip(c21, c22)]


def _drain(gen):
    while True:
        try:
            next(gen)
        except StopIteration as e:
            return e.value


def _chain(*gens):
    for g in gens:
        yield from g


def _woven(main, count, side, side_count):
    done = 0
    for i in range(count):
        while done < side_count and done * count < (i + 1) * side_count:
            next(side)
            done += 1
        next(main)
        yield
    _drain(side)


class _Pace:
    def __init__(self, zero, age):
        self.zero, self.age, self.recent = zero, age, []

    def note(self, y):
        self.recent.append(y[:, -128:])
        return y

    def after(self):
        if len(self.recent) < self.age:
            return lambda x: x
        bits = pltpu.bitcast(self.recent[-self.age][:8], U32) & self.zero
        return lambda x: pltpu.bitcast(pltpu.bitcast(x, U32) | bits, x.dtype)

    def tied(self, x, y):
        zero = jnp.concatenate([self.zero] * (x.shape[0] // 8), axis=0)
        return pltpu.bitcast(pltpu.bitcast(x, U32) | (pltpu.bitcast(y, U32) & zero), x.dtype)

    def blocks(self, load):
        tie = self.after()
        return [[tie(load(i, j)) if i % 2 == 0 and j % 2 == 0 else load(i, j) for j in range(4)]
                for i in range(4)]


def _swap_lane_and_chunk_bits(chunks):
    lane = jax.lax.broadcasted_iota(jnp.int32, chunks[0].shape, 1)
    u = (lane >> 1) & 7
    rolled = [x if c == 0 else pltpu.roll(x, 2 * c, 1) for c, x in enumerate(chunks)]
    xs = [rolled[(-i) % 8] for i in range(8)]
    for t in (1, 2, 4):
        m = (u & t) != 0
        xs = [jnp.where(m, xs[(i - t) % 8], xs[i]) for i in range(8)]
    return [x if j == 0 else pltpu.roll(x, 128 - 2 * j, 1) for j, x in enumerate(xs)]


def _kernel(xa_hbm, wqkv_hbm, woa_hbm, xb_hbm, c_hbm, wq_hbm, wuk_hbm, wuv_hbm, wob_hbm,
            out_hbm,
            hs, wo, wa, wo_raw, wa_raw,
            sem_wo, sem_wa, *, ph, vlag, ch, lag, nx, age, ager, lw, lj, tail, st, pin, sa, run, agel, n1, n2, runf, sm):
    xa32, wqkv32, woa32 = (r.bitcast(U32) for r in (xa_hbm, wqkv_hbm, woa_hbm))
    xb32, c32, wob32 = (r.bitcast(U32) for r in (xb_hbm, c_hbm, wob_hbm))
    wq32, wk32, wv32 = (r.bitcast(U32) for r in (wq_hbm, wuk_hbm, wuv_hbm))

    def ctx_rows(page, row, n):
        return _rows(AT_CTX + page * (S // 2) + row, n)

    def pace(step, age):
        return _Pace(jnp.full((8, 128), step // S, jnp.int32).astype(U32), age)

    def zero(step, salt):
        return step // (S + salt)

    def cp_wo(g):
        return pltpu.make_async_copy(wob32.at[pl.ds(g * GH, GH)], wo_raw.at[g % 2], sem_wo.at[g % 2])

    def cp_wa(m):
        return pltpu.make_async_copy(wqkv32.at[:, _rows(m * DM, DM)], wa_raw.at[m % 2], sem_wa.at[m % 2])

    def cp_woa(n):
        d321, h10, d4 = n >> 3, (n >> 1) & 3, n & 1
        return pltpu.make_async_copy(woa32.at[:, h10 * 16 + d4 * 8 + d321, :],
                                     wa_raw.at[1, _rows(8 * n, 8), :], sem_wa.at[1])

    def prep_slabs(pc, u, load, store):
        for half in range(2):
            for c in range(2):
                for i in range(7):
                    z = zero(u, i)
                    x = pc.blocks(lambda k, j: load(z, k, half * 8, 2 * j + c))
                    for n, y in _seven(_rhs_term, [[_halves(w) for w in r] for r in x], i):
                        store(n, half * 8, c, _words(y))
                    yield

    def prep_wo(pc, u):
        def store(n, row, c, y):
            wo[n, _rows(u * 16 + row, 8), c * 128:(c + 1) * 128] = y
        return prep_slabs(
            pc, u, lambda z, k, row, c: wo_raw[u // GH % 2 + z, k, _rows(u % GH * 16 + row, 8), c * 128:(c + 1) * 128], store)

    def permute_wa(pc, u):
        for i in range(4):
            for half in range(2):
                tie = pc.after()
                raw = [tie(wa_raw[u // 8 % 2, _rows(i * 128 + u % 8 * 16 + half * 8, 8), c * 128:(c + 1) * 128])
                       for c in range(8)]
                for c, y in enumerate(_swap_lane_and_chunk_bits(raw)):
                    hs[pl.ds(AT_SLAB + c * TILE + i * 16 + half * 8, 8), :] = jnp.where(u < 24, y, raw[c])
                yield

    def prep_wa(pc, u, permuted):
        def load(z, k, row, c):
            if permuted:
                return hs[_rows(AT_SLAB + (c + z) * TILE + k * 16 + row, 8), :]
            return wa_raw[1 + z, _rows(k * 128 + u % 8 * 16 + row, 8), c * 128:(c + 1) * 128]

        def store(n, row, c, y):
            wa[u // 8, n, _rows(u % 8 * 16 + row, 8), c * 128:(c + 1) * 128] = y
        return prep_slabs(pc, u, load, store)

    def heads(xc, cc, wq_raw, wkv_raw, qs, ks, vs, sem_w, sem_x):
        def cp_w(g):
            cps = []
            for i in range(2):
                p = 2 * g + i
                cps.append(pltpu.make_async_copy(wk32.at[:, p, :], wkv_raw.at[g % 2, 0, i], sem_w.at[g % 2, 0, i]))
                cps.append(pltpu.make_async_copy(wv32.at[:, p, :], wkv_raw.at[g % 2, 1, i], sem_w.at[g % 2, 1, i]))
            for i in range(2):
                cps.append(pltpu.make_async_copy(wq32.at[:, 2 * g + i, :], wq_raw.at[g % 2, i], sem_w.at[g % 2, 2, i]))
            return cps

        def cp_rows(j):
            r = _rows(j * (SET // 2), SET // 2)
            return [pltpu.make_async_copy(src.at[r, t * 128:(t + 1) * 128],
                                          hs.at[ctx_rows(page + t, j * (SET // 2), SET // 2), :], sem_x.at[j])
                    for page, src in ((0, c32), (4, xb32)) for t in range(src.shape[1] // 128)]

        def prep_rows(pc, page, dst, j, starts=range(0, SET // 8, 8)):
            r, tiles = SET // 8, dst.shape[-1] // 128
            for a in starts:
                for t in range(tiles):
                    for i in range(7):
                        z = zero(j, i)
                        x = pc.blocks(lambda b, k: hs[ctx_rows(page + k * tiles + t + z, j * (SET // 2) + b * r + a, 8), :])
                        for n, y in _seven(_lhs_term, [[_b16(w).astype(F32) for w in row] for row in x], i):
                            dst[n, _rows(j * r + a, 8), t * 128:(t + 1) * 128] = _shuffled(y)
                        yield

        def prep_w(pc, g, j):
            def unit(raw, depth, a, row):
                for i in range(7):
                    z = zero(j, i)
                    x = pc.blocks(lambda k, c: raw[
                        c // 2 + z, pl.ds(k * (depth // 4) + j * (depth // 16) + a + c % 2, 8, stride=2), :])
                    x = [[_halves(w) for w in r] for r in x]
                    x = [[jnp.concatenate([r[c // 2 * 2][c % 2 * 8:c % 2 * 8 + 8],
                                           r[c // 2 * 2 + 1][c % 2 * 8:c % 2 * 8 + 8]], axis=0)
                          for c in range(4)] for r in x]
                    for n, y in _seven(_rhs_term, x, i):
                        hs[_rows((g % 2 * NP + n) * 4 * TILE + row, 8), :] = _words(y)
                    yield

            for a in range(0, DM // 16, 16):
                yield from unit(wq_raw.at[g % 2], DM, a, j * (DM // 32) + a // 2)
            for kind in range(2):
                for a in range(0, DC // 16, 16):
                    yield from unit(wkv_raw.at[g % 2, kind], DC, a, (2 + kind) * TILE + j * (DC // 32) + a // 2)

        def project(pc, g, j, run):
            r = SET // 8
            rows = _rows(j * r, r)

            def product(lhs, first, last):
                def run(n):
                    y = pc.note(_dot(lhs[n, rows, :], hs[_rows(((g % 2 * NP + n) * 4 + first) * TILE, (last - first) * TILE, TILE), :]))
                    yield
                    return y
                return _combine(run)

            q, k, v = product(xc, 0, 2), product(cc, 2, 3), product(cc, 3, 4)
            for n in range(0, NP, run):
                for gen in (q, k, v):
                    for _ in range(min(run, NP - n)):
                        next(gen)
                        yield
            q, k, v = _drain(q), _drain(k), _drain(v)
            for i in range(4):
                dst = _rows(j * (SET // 2) + i * r, r)
                for h in range(GH):
                    slot = g % 2 * GH + h
                    qs[slot, dst, :] = _shuffled(q[i][h] * (DB ** -0.5 * LOG2E))
                    ks[slot, dst, :] = _shuffled(k[i][h])
                    vs[slot, dst, :] = _shuffled(v[i][h])

        def attend(pc, h, filler, fill_steps, run, cost):
            slot = h % (2 * GH)
            nb = S // 128
            work = [(i, t, min(t + ch, i + 1)) for i in reversed(range(nb)) for t in range(0, i + 1, ch)]
            s, mx, m, l, o, done, ready = {}, {}, {}, {}, {}, {}, []

            def scores(i, t0, t1):
                x = pc.note(jax.lax.dot_general(_b16(qs[slot, i * TILE:(i + 1) * TILE, :]),
                                                _b16(ks[slot, t0 * TILE:t1 * TILE, :]), NT,
                                                preferred_element_type=F32))
                if t1 == i + 1:
                    row, col = (jax.lax.broadcasted_iota(jnp.int32, (128, 128), d) for d in range(2))
                    row, col = ((u & ~15) | ((u >> 2) & 3) | ((u & 3) << 2) for u in (row, col))
                    diag = jnp.where(col <= row, x[:, -128:], NEG)
                    x = jnp.concatenate([x[:, :-128], diag], axis=1) if t1 - t0 > 1 else diag
                s[i, t0] = x
                mx[i] = jnp.maximum(mx[i], _fold(jnp.maximum, x)) if t0 else _fold(jnp.maximum, x)
                if t1 == i + 1:
                    m[i] = jnp.max(mx[i], axis=1, keepdims=True)

            def values(i, t0, t1):
                p = jnp.exp2(s.pop((i, t0)) - m[i])
                y = pc.note(jnp.dot(p.astype(BF16), _b16(vs[slot, t0 * TILE:t1 * TILE, :]),
                                    preferred_element_type=F32))
                parts = ([l[i]] if t0 else []) + [p[:, c:c + 128] for c in range(0, p.shape[1], 128)]
                l[i] = functools.reduce(jnp.add, [pc.tied(parts[0], pc.recent[-1 - sa])] + parts[1:])
                o[i] = o[i] + y if t0 else y
                if t1 == i + 1:
                    ready.append((clock + pin, i, _shuffled(o[i] * _recip(jnp.sum(l[i], axis=1, keepdims=True)))))

            def finish():
                while ready and ready[0][0] <= clock:
                    _, i, x = ready.pop(0)
                    hs[ctx_rows(h, i * TILE, TILE), :] = x

            total = 2 * sum(t1 - t0 for _, t0, t1 in work)
            clock = attn = filled = qi = pi = turn = 0
            while pi < len(work):
                can = work[pi][0] in done and clock - done[work[pi][0]] >= lag
                if filled < fill_steps and (filled * total <= attn * fill_steps
                                            or (qi == len(work) and not can)):
                    for _ in range(min(run, fill_steps - filled)):
                        next(filler)
                        filled += 1
                        clock += cost
                elif qi < len(work) and (not can or turn == 0):
                    scores(*work[qi])
                    clock += work[qi][2] - work[qi][1]
                    attn += work[qi][2] - work[qi][1]
                    if work[qi][2] == work[qi][0] + 1:
                        done[work[qi][0]] = clock
                    qi, turn = qi + 1, 1
                else:
                    values(*work[pi])
                    clock += work[pi][2] - work[pi][1]
                    attn += work[pi][2] - work[pi][1]
                    pi, turn = pi + 1, 0
                finish()
            for _ in filler:
                clock += cost
                finish()
            clock += pin
            finish()

        for cp in cp_w(0) + cp_rows(0) + cp_rows(1) + cp_w(1):
            cp.start()
        for cp in cp_w(0):
            cp.wait()
        if "p" in ph:
            jax.lax.fori_loop(0, GH, lambda j, _: _drain(prep_w(pace(j, 1), 0, j)), None)
        for cp in cp_rows(0):
            cp.wait()

        def first_rows(a, _):
            _drain(prep_rows(pace(a, 1), 0, cc, 0, [a * 8]))
            _drain(prep_rows(pace(a, 1), 4, xc, 0, [a * 8]))
        if "p" in ph:
            jax.lax.fori_loop(0, SET // 64, first_rows, None)
        for cp in cp_w(1):
            cp.wait()

        def fetch_later_weights(u):
            @pl.when(u % GH == 0)
            def _():
                @pl.when(u // GH + 1 < NG)
                def _():
                    cp_wo(u // GH + 1).start()
                cp_wo(u // GH).wait()

                @pl.when((u == 0) | (u == 8))
                def _():
                    cp_wa(u // 8 + 1).start()

                @pl.when(u == 16)
                def _():
                    jax.lax.fori_loop(0, 64, lambda n, _: cp_woa(n).start(), None)

                @pl.when((u % 8 == 0) & (u < 24))
                def _():
                    cp_wa(u // 8).wait()

                @pl.when(u == 24)
                def _():
                    jax.lax.fori_loop(0, 64, lambda n, _: cp_woa(n).wait(), None)

        def first_group(j, _):
            @pl.when(j + 2 < GH)
            def _():
                for cp in cp_rows(j + 2):
                    cp.start()

            @pl.when(j == 1)
            def _():
                for cp in cp_w(2) + [cp_wo(0), cp_wa(0)]:
                    cp.start()

            @pl.when(j + 1 < GH)
            def _():
                for cp in cp_rows(j + 1):
                    cp.wait()

            nxt = jnp.minimum(j + 1, GH - 1)
            pc = pace(j, age)
            side = _chain(prep_rows(pc, 0, cc, nxt), prep_rows(pc, 4, xc, nxt), prep_w(pc, 1, j))
            main = project(pc, 0, j, runf)
            _drain(_woven(main, 3 * NP, side, 224))
            _drain(main)
        if "f" in ph:
            jax.lax.fori_loop(0, GH, first_group, None)

        def head(h, _):
            g, j = h // GH, h % GH

            @pl.when(j == 0)
            def _():
                @pl.when(g + 3 < NG)
                def _():
                    for cp in cp_w(g + 3):
                        cp.start()

                @pl.when(g + 2 < NG)
                def _():
                    for cp in cp_w(g + 2):
                        cp.wait()

            pc = pace(h, age)
            fetch_later_weights(h)
            side = _chain(_woven(prep_wo(pc, h), 28, permute_wa(pc, h), 8), prep_wa(pc, h, True), prep_w(pc, g + 2, j))
            main = project(pc, g + 1, j, run)
            filler = _woven(main, 3 * NP - st, side, 112)
            attend(pc, h, filler, 3 * NP - tail, vlag, 4 / 3)
            _drain(main)
        if "h" in ph:
            jax.lax.fori_loop(0, HB - GH, head, None)

        def last_head(h, _):
            pc = pace(h, agel)
            fetch_later_weights(h)
            attend(pc, h, _chain(prep_wo(pc, h), prep_wa(pc, h, False)), 56, 1, 0)
        if "l" in ph:
            jax.lax.fori_loop(HB - GH, HB, last_head, None)

    vm, dma = pltpu.VMEM, pltpu.SemaphoreType.DMA
    pl.run_scoped(
        heads,
        vm((NP, S // 8, DM // 4), U32), vm((NP, S // 8, DC // 4), U32),
        vm((2, 2, DM, DB), U32), vm((2, 2, 2, DC, DB), U32),
        *[vm((2 * GH, S // 2, DB), U32) for _ in range(3)],
        dma((2, 3, 2)), dma((GH,)))

    def rows_phase(oc, xac, oac, qa, ka, va, ya, pa, xa_raw, stage, sem_xa, sem_out):
        def cp_xa(t):
            return pltpu.make_async_copy(xa32.at[_rows(t * (RO // 2), RO // 2), :],
                                         xa_raw.at[t % 3], sem_xa.at[t % 3])

        def cp_out(t, part):
            at = (_rows(t * RO, RO), pl.ds(part * DM, DM))
            return pltpu.make_async_copy(stage.at[at], out_hbm.at[at], sem_out.at[part, t])

        def prep_ctx(pc, t, i, groups=range(NG)):
            for a in range(0, RA, 8):
                for p in groups:
                    z = zero(t, i)
                    x = pc.blocks(lambda b, k: hs[ctx_rows(p * GH + k + z, t * (RO // 2) + b * RA + a, 8), :])
                    for n, y in _seven(_lhs_term, [[_b16(w).astype(F32) for w in row] for row in x], i):
                        oc[n, a:a + 8, _rows(p * 128, 128)] = _shuffled(y)
                    yield

        def prep_xa(pc, t, i):
            for a in range(0, RA, 8):
                for c in range(2):
                    slot = t % 3 + zero(t, i)
                    x = pc.blocks(lambda b, k: xa_raw[slot, b * RA + a:b * RA + a + 8, (2 * k + c) * 128:(2 * k + c + 1) * 128])
                    for n, y in _seven(_lhs_term, [[_halves(w) for w in row] for row in x], i):
                        xac[n, a:a + 8, c * 128:(c + 1) * 128] = _words(y)
                    yield

        def window_weights(pc, t):
            lane = jax.lax.broadcasted_iota(jnp.int32, (sm, 128), 1)

            def softmax(a):
                tie = pc.after()
                logits = []
                for w in range(WIN):
                    x = jnp.concatenate([tie(pa[w + zero(t, 1), b:b + 8, :]) for b in range(a, a + sm, 8)], axis=0)
                    for bit in (16, 1):
                        x = x + jnp.where((lane & bit) != 0, pltpu.roll(x, bit, 1), pltpu.roll(x, 128 - bit, 1))
                    if a < DIL * w:
                        pos = jax.lax.broadcasted_iota(jnp.int32, (sm, 128), 0) + (t * RO + a)
                        x = jnp.where(pos >= DIL * w, x, NEG)
                    logits.append(x)
                top = functools.reduce(jnp.maximum, logits)
                es = [jnp.exp2(x - top) for x in logits]
                inv = _recip(functools.reduce(jnp.add, es))
                for w, e in enumerate(es):
                    pa[w, a:a + sm, :] = e * inv

            for a in range(0, RO, 8):
                for w in range(WIN):
                    if w % lw == 0:
                        tie = pc.after()
                        q = [tie(qa[j, a:a + 8, :]) for j in range(8)]
                    b = a + HALO - DIL * w
                    x = q[0] * ka[0, b:b + 8, :]
                    for j in range(1, 8):
                        x = x + q[j] * ka[j, b:b + 8, :]
                    pa[w, a:a + 8, :] = x
                    if w % lw == lw - 1:
                        yield
                if (a + 8) % sm == 0:
                    softmax(a + 8 - sm)
                    yield
            ka[:, 0:HALO, :] = ka[:, RO:, :]

        def window_mix(pc, t):
            for a in range(0, RO, 8):
                for j in range(8):
                    if j % lj == 0:
                        tie = pc.after()
                        ps = [tie(pa[w + zero(t, 0), a:a + 8, :]) for w in range(WIN)]
                    acc = ps[0] * va[j, a + HALO:a + HALO + 8, :]
                    for w in range(1, WIN):
                        b = a + HALO - DIL * w
                        acc = acc + ps[w] * va[j, b:b + 8, :]
                    ya[j, a:a + 8, :] = acc
                    if j % lj == lj - 1:
                        yield
            va[:, 0:HALO, :] = va[:, RO:, :]
            for i in range(7):
                for a in range(0, RA, 8):
                    for c in range(2):
                        z = zero(t, i)
                        x = [pc.blocks(lambda b, k: ya[2 * k + c + z, pl.ds(2 * (b * RA + a) + e, 8, stride=2), :])
                             for e in range(2)]
                        x = [[jnp.concatenate(w, axis=0) for w in zip(*rows)] for rows in zip(*x)]
                        for n, y in _seven(_lhs_term, x, i):
                            oac[n, a:a + 8, c * 128:(c + 1) * 128] = _words(y)
                        yield

        def joined(c):
            return jnp.concatenate([jnp.concatenate(row, axis=1) for row in c], axis=0)

        steps = S // RO
        cp_xa(0).start()
        cp_xa(1).start()
        ka[:, 0:HALO, :] = jnp.zeros((8, HALO, 128), F32)
        va[:, 0:HALO, :] = jnp.zeros((8, HALO, 128), F32)

        def first_ctx(p, _):
            for i in range(7):
                _drain(prep_ctx(pace(p, 1), 0, i, [p]))
        if "p" in ph:
            jax.lax.fori_loop(0, NG, first_ctx, None)
        cp_xa(0).wait()
        if "p" in ph:
            for i in range(7):
                _drain(prep_xa(pace(0, 1), 0, i))

        def step(t, _):
            nxt = jnp.minimum(t + 1, steps - 1)
            pc = pace(t, ager)

            @pl.when(t + 2 < steps)
            def _():
                cp_xa(t + 2).start()

            @pl.when(t + 1 < steps)
            def _():
                cp_xa(t + 1).wait()

            def times(lhs, w):
                def run(n):
                    y = None
                    for k in range(lhs.shape[2] // 256):
                        z = pc.note(_dot(lhs[n, :, k * 256:(k + 1) * 256], w[n, k * 128:(k + 1) * 128, :]))
                        y = z if y is None else y + z
                        yield
                    return y
                return _combine(run)

            k = joined(_drain(times(xac, wa.at[1])))
            for j in range(8):
                ka[j, HALO:, :] = k[:, j * 128:(j + 1) * 128]
            q = joined(_drain(times(xac, wa.at[0]))) * (DA ** -0.5 * LOG2E)
            for j in range(8):
                qa[j] = q[:, j * 128:(j + 1) * 128]
            v, b = times(xac, wa.at[2]), times(oc, wo)

            def later():
                for i in range(7):
                    yield from _woven(v, 7, prep_xa(pc, nxt, i - 1) if i else iter(()), 8 if i else 0)
                y = joined(_drain(v))
                for j in range(8):
                    va[j, HALO:, :] = y[:, j * 128:(j + 1) * 128]
                yield from _woven(b, 28, prep_xa(pc, nxt, 6), 8)
                for i in range(1, 7):
                    yield from _woven(b, 28, prep_ctx(pc, nxt, i - 1), 32)

            rest = later()
            _drain(_woven(rest, nx, iter(()), 0))
            _drain(_woven(rest, n1, window_weights(pc, t), 32 * (WIN // lw) + RO // sm))
            _drain(_woven(rest, 5 * NP - nx - n1 - n2, window_mix(pc, t), 32 * (8 // lj) + 56))
            _drain(rest)
            stage[_rows(t * RO, RO), DM:] = joined(_drain(b)).astype(BF16)
            cp_out(t, 1).start()
            y = times(oac, wa.at[3])
            _drain(_woven(y, NP - 7, prep_ctx(pc, nxt, 6), 32))
            stage[_rows(t * RO, RO), 0:DM] = joined(_drain(y)).astype(BF16)
            cp_out(t, 0).start()

        if "r" in ph:
            jax.lax.fori_loop(0, steps, step, None)
        else:
            stage[0:16, 0:128] = _b16(hs[AT_CTX:AT_CTX + 8, :] | wo[0, 0:8, 0:128] | wa[0, 0, 0:8, 0:128])
        for t in range(steps):
            cp_out(t, 1).wait()
            cp_out(t, 0).wait()

    pl.run_scoped(
        rows_phase,
        vm((NP, RA, HB * DB // 4), U32), vm((NP, RA, DM // 4), U32), vm((NP, RA, DM // 4), U32),
        vm((8, RO, 128), F32), vm((8, HALO + RO, 128), F32), vm((8, HALO + RO, 128), F32), vm((8, RO, 128), F32),
        vm((WIN, RO, 128), F32),
        vm((3, RO // 2, DM), U32), vm((S, 2 * DM), BF16),
        dma((3,)), dma((2, S // RO)))


def build(pred=8, **cfg):
    flags = {"XLA_TPU_MAX_INSTS_TO_PREDICATE": pred} if pred is not None else None
    vm, dma = pltpu.VMEM, pltpu.SemaphoreType.DMA
    scratch = [
        vm((AT_CTX + HB * S // 2, 128), U32),
        vm((NP, HB * DB // 8, DM // 4), U32), vm((4, NP, DM // 8, DM // 4), U32),
        vm((2, GH, DB // 2, DM), U32), vm((2, DM // 2, DM), U32),
        dma((2,)), dma((2,)),
    ]

    @jax.jit
    def run(A_x, A_wqkv, A_wo, B_x, B_c_kv, B_w_q, B_w_uk, B_w_uv, B_w_o):
        out = pl.pallas_call(
            functools.partial(_kernel, **cfg),
            out_shape=jax.ShapeDtypeStruct((S, 2 * DM), BF16),
            in_specs=[pl.BlockSpec(memory_space=pl.ANY)] * 9,
            out_specs=pl.BlockSpec(memory_space=pl.ANY),
            scratch_shapes=scratch,
            compiler_params=pltpu.CompilerParams(vmem_limit_bytes=128 * 2**20, flags=flags),
            name="fused",
        )(A_x.reshape(S, DM), A_wqkv, A_wo.reshape(8, DM // 8, DM),
          B_x.reshape(S, DM), B_c_kv.reshape(S, DC), B_w_q, B_w_uk, B_w_uv, B_w_o)
        return out.reshape(1, S, 2 * DM)

    return run


@jax.jit
def pallas_concat_heads__sliding_local_dilated__compressed_kv_cla__prompt_kernel(
    A_x: jax.Array,
    A_wqkv: jax.Array,
    A_wo: jax.Array,
    B_x: jax.Array,
    B_c_kv: jax.Array,
    B_w_q: jax.Array,
    B_w_uk: jax.Array,
    B_w_uv: jax.Array,
    B_w_o: jax.Array,
):
    return build(**CFG)(A_x, A_wqkv, A_wo, B_x, B_c_kv, B_w_q, B_w_uk, B_w_uv, B_w_o)
```

```python
import functools
import math

import jax
import jax.numpy as jnp
from jax.experimental import pallas as pl
from jax.experimental.pallas import tpu as pltpu

S = 2048
DM = 1024
HA, DA = 32, 32
WIN, DIL = 8, 2
HB, DB = 32, 128
DC = 512
NEG = -1e9
LOG2E = math.log2(math.e)

GH = 4
NG = HB // GH
SET = S // GH
RO = 256
HALO = 16
NP = 49
TILE = 64

F32, BF16, U32 = jnp.float32, jnp.bfloat16, jnp.uint32
NT = (((1,), (1,)), ((), ()))

CFG = dict(ph="pjar", ch=4, lag=8, nx=6, agep=6, agea=3, ager=6, lw=2, lj=2, sa=2, n1=112, n2=6, sm=16,
           hp=2, sp=2, pin=12, agex=12, order='qkv', tailp=14)

RA = RO // 8


def _b16(x32):
    return pltpu.bitcast(x32, BF16)


def _pack2(lo, hi):
    return pltpu.pack_elementwise([lo, hi], packed_dtype=BF16)


def _halves(w):
    return jnp.concatenate([pltpu.unpack_elementwise(w, index=i, packed_dtype=BF16, unpacked_dtype=F32)
                            for i in range(2)], axis=0)


def _words(x):
    n = x.shape[0] // 2
    return _pack2(x[:n], x[n:])


def _shuffled(x):
    parts = [_pack2(x[r:r + 8], x[r + 8:r + 16]) for r in range(0, x.shape[0], 16)]
    return jnp.concatenate(parts, axis=0) if len(parts) > 1 else parts[0]


def _dot(a32, b32):
    return jnp.dot(_b16(a32), _b16(b32), preferred_element_type=F32)


def _recip(x):
    r = pl.reciprocal(x, approx=True)
    return r * (2.0 - x * r)


def _rows(start, size, align=None):
    return pl.ds(start if isinstance(start, int) else pl.multiple_of(start, align or size), size)


def _fold(f, x):
    return functools.reduce(f, [x[:, c:c + 128] for c in range(0, x.shape[1], 128)])


def _quads(x):
    n = len(x) // 2
    return ([r[:n] for r in x[:n]], [r[n:] for r in x[:n]],
            [r[:n] for r in x[n:]], [r[n:] for r in x[n:]])


def _add(x, y):
    return [[a + b for a, b in zip(r, s)] for r, s in zip(x, y)]


def _sub(x, y):
    return [[a - b for a, b in zip(r, s)] for r, s in zip(x, y)]


def _lhs_term(x, i):
    a11, a12, a21, a22 = _quads(x)
    return (lambda: _sub(a12, a22), lambda: _sub(a21, a11), lambda: _add(a11, a22), lambda: a22,
            lambda: a11, lambda: _add(a21, a22), lambda: _add(a11, a12))[i]()


def _rhs_term(x, i):
    b11, b12, b21, b22 = _quads(x)
    return (lambda: _add(b21, b22), lambda: _add(b11, b12), lambda: _add(b11, b22), lambda: _sub(b21, b11),
            lambda: _sub(b12, b22), lambda: b11, lambda: b22)[i]()


def _seven(term, x, i):
    y = term(x, i)
    return [(7 * i + j, term(y, j)[0][0]) for j in range(7)]


def _combine(product, level=2, base=0):
    if level == 0:
        return [[(yield from product(base))]]
    k = 7 ** (level - 1)
    m7 = yield from _combine(product, level - 1, base)
    m6 = yield from _combine(product, level - 1, base + k)
    m1 = yield from _combine(product, level - 1, base + 2 * k)
    c11 = _add(m7, m1)
    c22 = _add(m6, m1)
    m4 = yield from _combine(product, level - 1, base + 3 * k)
    c11 = _add(c11, m4)
    m3 = yield from _combine(product, level - 1, base + 4 * k)
    c22 = _add(c22, m3)
    m2 = yield from _combine(product, level - 1, base + 5 * k)
    c21 = _add(m2, m4)
    c22 = _sub(c22, m2)
    m5 = yield from _combine(product, level - 1, base + 6 * k)
    c11 = _sub(c11, m5)
    c12 = _add(m3, m5)
    return [r + s for r, s in zip(c11, c12)] + [r + s for r, s in zip(c21, c22)]


def _drain(gen):
    while True:
        try:
            next(gen)
        except StopIteration as e:
            return e.value


def _chain(*gens):
    for g in gens:
        yield from g


def _woven(main, count, side, side_count, skip=0):
    done = 0
    for _ in range(skip):
        next(main)
        yield
    count -= skip
    for i in range(count):
        while done < side_count and done * count < (i + 1) * side_count:
            next(side)
            done += 1
        next(main)
        yield
    _drain(side)


class _Pace:
    def __init__(self, zero, age):
        self.zero, self.age, self.recent = zero, age, []

    def note(self, y):
        self.recent.append(y[:, -128:])
        return y

    def after(self, age=None):
        age = age or self.age
        if len(self.recent) < age:
            return lambda x: x
        bits = pltpu.bitcast(self.recent[-age][:8], U32) & self.zero
        return lambda x: pltpu.bitcast(pltpu.bitcast(x, U32) | bits, x.dtype)

    def tied(self, x, y):
        zero = jnp.concatenate([self.zero] * (x.shape[0] // 8), axis=0)
        return pltpu.bitcast(pltpu.bitcast(x, U32) | (pltpu.bitcast(y, U32) & zero), x.dtype)

    def blocks(self, load):
        tie = self.after()
        return [[tie(load(i, j)) if i % 2 == 0 and j % 2 == 0 else load(i, j) for j in range(4)]
                for i in range(4)]


def _swap_lane_and_chunk_bits(chunks):
    lane = jax.lax.broadcasted_iota(jnp.int32, chunks[0].shape, 1)
    u = (lane >> 1) & 7
    rolled = [x if c == 0 else pltpu.roll(x, 2 * c, 1) for c, x in enumerate(chunks)]
    xs = [rolled[(-i) % 8] for i in range(8)]
    for t in (1, 2, 4):
        m = (u & t) != 0
        xs = [jnp.where(m, xs[(i - t) % 8], xs[i]) for i in range(8)]
    return [x if j == 0 else pltpu.roll(x, 128 - 2 * j, 1) for j, x in enumerate(xs)]


def _kernel(xa_hbm, wqkv_hbm, woa_hbm, xb_hbm, c_hbm, wq_hbm, wuk_hbm, wuv_hbm, wob_hbm,
            out_hbm,
            ctx, wo, wa, wo_raw, wa_raw, xc, cc, wb, wq_raw, wkv_raw, ks, vs,
            qa, ka, va, ya, pa, xa_raw, stage,
            sem_wo, sem_wa, sem_w, sem_x, sem_xa, sem_out, *,
            ph, ch, lag, nx, agep, agea, ager, lw, lj, sa, n1, n2, sm, hp, sp, pin, agex, order, tailp):
    xa32, wqkv32, woa32 = (r.bitcast(U32) for r in (xa_hbm, wqkv_hbm, woa_hbm))
    xb32, c32, wob32 = (r.bitcast(U32) for r in (xb_hbm, c_hbm, wob_hbm))
    wq32, wk32, wv32 = (r.bitcast(U32) for r in (wq_hbm, wuk_hbm, wuv_hbm))

    def pace(step, age):
        return _Pace(jnp.full((8, 128), step // S, jnp.int32).astype(U32), age)

    def zero(step, salt):
        return step // (S + salt)

    def start_slabs(i):
        u, n = i * sp, 16 * sp
        for k in range(4):
            pltpu.make_async_copy(wob32.at[u // GH * GH + k, _rows(u % GH * 16, n), :],
                                  wo_raw.at[i % 2, k], sem_wo.at[i % 2]).start()

        @pl.when(u < 24)
        def _():
            for k in range(4):
                pltpu.make_async_copy(wqkv32.at[_rows(k * 128 + u % 8 * 16, n), _rows(u // 8 * DM, DM)],
                                      wa_raw.at[i % 2, k], sem_wa.at[i % 2]).start()

        @pl.when(u >= 24)
        def _():
            for k in range(4):
                for e in range(n // 8):
                    m = k * 16 + u % 8 * 2 + e
                    pltpu.make_async_copy(woa32.at[:, ((m >> 1) & 3) * 16 + (m & 1) * 8 + (m >> 3), :],
                                          wa_raw.at[i % 2, k, pl.ds(8 * e, 8), :], sem_wa.at[i % 2]).start()

    def wait_slabs(i):
        for raw, sem in ((wo_raw, sem_wo), (wa_raw, sem_wa)):
            pltpu.make_async_copy(raw.at[i % 2], raw.at[i % 2], sem.at[i % 2]).wait()

    def prep_slabs(pc, u, load, store):
        for half in range(2):
            for c in range(2):
                for i in range(7):
                    z = zero(u, i)
                    x = pc.blocks(lambda k, j: load(z, k, half * 8, 2 * j + c))
                    for n, y in _seven(_rhs_term, [[_halves(w) for w in r] for r in x], i):
                        store(n, half * 8, c, _words(y))
                    yield

    def prep_wo(pc, u, at):
        def store(n, row, c, y):
            wo[n, _rows(u * 16 + row, 8), c * 128:(c + 1) * 128] = y
        return prep_slabs(
            pc, u, lambda z, k, row, c: wo_raw[u // sp % 2 + z, k, pl.ds(at + row, 8), c * 128:(c + 1) * 128], store)

    def permute_wa(pc, u, at):
        for i in range(4):
            for half in range(2):
                tie = pc.after(agex)
                raw = [tie(wa_raw[u // sp % 2, i, pl.ds(at + half * 8, 8), c * 128:(c + 1) * 128])
                       for c in range(8)]
                for c, y in enumerate(_swap_lane_and_chunk_bits(raw)):
                    wb[NP + c, pl.ds(i * 16 + half * 8, 8), :] = jnp.where(u < 24, y, raw[c])
                yield

    def prep_wa(pc, u):
        def store(n, row, c, y):
            wa[u // 8, n, _rows(u % 8 * 16 + row, 8), c * 128:(c + 1) * 128] = y
        return prep_slabs(pc, u, lambda z, k, row, c: wb[NP + c + z, k * 16 + row:k * 16 + row + 8, :], store)

    def heads():
        def cp_w(g):
            return [pltpu.make_async_copy(src.at[:, 2 * g + i, :], dst.at[i], sem_w.at[g % 2, kind, i])
                    for kind, (src, dst) in enumerate(((wk32, wkv_raw.at[g % 2, 0]), (wv32, wkv_raw.at[g % 2, 1]),
                                                       (wq32, wq_raw.at[g % 2])))
                    for i in range(2)]

        def cp_rows(j):
            r = _rows(j * (SET // 2), SET // 2)
            return [pltpu.make_async_copy(src.at[r, t * 128:(t + 1) * 128], ctx.at[page + t, r, :], sem_x.at[j])
                    for page, src in ((0, c32), (4, xb32)) for t in range(src.shape[1] // 128)]

        def prep_rows(pc, page, dst, j, a):
            r, tiles = SET // 8, dst.shape[-1] // 128
            for t in range(tiles):
                x = [[_b16(ctx[page + k * tiles + t, _rows(j * (SET // 2) + b * r + a, 8), :]).astype(F32)
                      for k in range(4)] for b in range(4)]
                for i in range(7):
                    for n, y in _seven(_lhs_term, x, i):
                        dst[n, _rows(j * r + a, 8), t * 128:(t + 1) * 128] = _shuffled(y)
                    yield

        def prep_w(pc, g, j):
            def unit(raw, depth, a, row):
                for i in range(7):
                    z = zero(j, i)
                    x = pc.blocks(lambda k, c: raw[
                        c // 2 + z, pl.ds(k * (depth // 4) + j * (depth // 16) + a + c % 2, 8, stride=2), :])
                    x = [[_halves(w) for w in r] for r in x]
                    x = [[jnp.concatenate([r[c // 2 * 2][c % 2 * 8:c % 2 * 8 + 8],
                                           r[c // 2 * 2 + 1][c % 2 * 8:c % 2 * 8 + 8]], axis=0)
                          for c in range(4)] for r in x]
                    for n, y in _seven(_rhs_term, x, i):
                        wb[n, _rows(row, 8), :] = _words(y)
                    yield

            for a in range(0, DM // 16, 16):
                yield from unit(wq_raw.at[g % 2], DM, a, j * (DM // 32) + a // 2)
            for kind in range(2):
                for a in range(0, DC // 16, 16):
                    yield from unit(wkv_raw.at[g % 2, kind], DC, a, (2 + kind) * TILE + j * (DC // 32) + a // 2)

        def project(pc, j):
            r = SET // 8
            rows = _rows(j * r, r)

            def product(lhs, first, last):
                def run(n):
                    y = pc.note(_dot(lhs[n, rows, :], wb[n + zero(j, 0), first * TILE:last * TILE, :]))
                    yield
                    return y
                return _combine(run)

            parts = dict(q=(ctx, HB, DB ** -0.5 * LOG2E, product(xc, 0, 2)),
                         k=(ks, 0, None, product(cc, 2, 3)), v=(vs, 0, None, product(cc, 3, 4)))
            for dst, page, scale, gen in (parts[c] for c in order):
                y = yield from gen
                for i in range(4):
                    for h in range(GH):
                        dst[page + h, _rows(j * (SET // 2) + i * r, r), :] = _shuffled(
                            y[i][h] * scale if scale else y[i][h])

        def attend(pc, g, first, side, side_steps):
            nb = S // 128
            work = [(first + h, i, t, min(t + ch, i + 1))
                    for h in range(hp) for i in reversed(range(nb)) for t in range(0, i + 1, ch)]
            key = [h * nb + i for h in range(hp) for i in reversed(range(nb)) for t in range(0, i + 1, ch)]
            s, mx, m, l, o, done, ready, due = {}, {}, {}, {}, {}, {}, [], []

            def scores(b, h, i, t0, t1):
                x = pc.note(jax.lax.dot_general(_b16(ctx[HB + h, i * TILE:(i + 1) * TILE, :]),
                                                _b16(ks[h, t0 * TILE:t1 * TILE, :]), NT,
                                                preferred_element_type=F32))
                if t1 == i + 1:
                    row, col = (jax.lax.broadcasted_iota(jnp.int32, (128, 128), d) for d in range(2))
                    row, col = ((u & ~15) | ((u >> 2) & 3) | ((u & 3) << 2) for u in (row, col))
                    diag = jnp.where(col <= row, x[:, -128:], NEG)
                    x = jnp.concatenate([x[:, :-128], diag], axis=1) if t1 - t0 > 1 else diag
                s[b, t0] = x
                mx[b] = jnp.maximum(mx[b], _fold(jnp.maximum, x)) if t0 else _fold(jnp.maximum, x)
                if t1 == i + 1:
                    m[b] = jnp.max(mx[b], axis=1, keepdims=True)

            def values(b, h, i, t0, t1):
                p = jnp.exp2(s.pop((b, t0)) - m[b])
                y = pc.note(jnp.dot(p.astype(BF16), _b16(vs[h, t0 * TILE:t1 * TILE, :]),
                                    preferred_element_type=F32))
                parts = ([l[b]] if t0 else []) + [p[:, c:c + 128] for c in range(0, p.shape[1], 128)]
                l[b] = functools.reduce(jnp.add, [pc.tied(parts[0], pc.recent[-1 - sa])] + parts[1:])
                o[b] = o[b] + y if t0 else y
                if t1 == i + 1:
                    ready.append((h, i, _shuffled(o[b] * _recip(jnp.sum(l[b], axis=1, keepdims=True)))))

            def products():
                clock = qi = pi = turn = 0
                while pi < len(work):
                    can = key[pi] in done and clock - done[key[pi]] >= lag
                    if qi < len(work) and (not can or turn == 0):
                        scores(key[qi], *work[qi])
                        clock += work[qi][3] - work[qi][2]
                        if work[qi][3] == work[qi][1] + 1:
                            done[key[qi]] = clock
                        qi, turn = qi + 1, 1
                    else:
                        values(key[pi], *work[pi])
                        clock += work[pi][3] - work[pi][2]
                        if len(due) < len(ready):
                            due.append(clock + pin)
                        pi, turn = pi + 1, 0
                    while due and (due[0] <= clock or pi == len(work)):
                        due.pop(0)
                        h, i, x = ready.pop(0)
                        ctx[g * GH + h, i * TILE:(i + 1) * TILE, :] = x
                    yield

            main = products()
            _drain(_woven(main, 2 * len(work) - 16, side, side_steps, agea))
            _drain(main)

        for cp in cp_w(0) + cp_rows(0) + cp_rows(1):
            cp.start()
        start_slabs(jnp.int32(0))
        for cp in cp_w(0):
            cp.wait()
        jax.lax.fori_loop(0, GH, lambda j, _: _drain(prep_w(pace(j, 1), 0, j)), None)

        def group(g, _):
            def rows(jj, _):
                @pl.when(g == 0)
                def _():
                    for j in [jj * sp + i for i in range(sp)]:
                        @pl.when(j + 2 < GH)
                        def _():
                            for cp in cp_rows(j + 2):
                                cp.start()
                        for cp in cp_rows(j):
                            cp.wait()

                        def first_rows(a, _):
                            _drain(prep_rows(None, 0, cc, j, a * 8))
                            _drain(prep_rows(None, 4, xc, j, a * 8))
                        jax.lax.fori_loop(0, SET // 64, first_rows, None)

                @pl.when((jj == GH // sp - 1) & (g + 1 < NG))
                def _():
                    for cp in cp_w(g + 1):
                        cp.start()

                i = g * (GH // sp) + jj

                @pl.when(i + 1 < HB // sp)
                def _():
                    start_slabs(i + 1)
                wait_slabs(i)
                pc = pace(g, agep)
                for n in range(sp):
                    j = jj * sp + n
                    u = g * GH + j
                    side = _chain(_woven(prep_wo(pc, u, 16 * n), 28, permute_wa(pc, u, 16 * n), 8), prep_wa(pc, u))
                    main = project(pc, j)
                    _drain(_woven(main, 3 * NP - tailp, side, 56, 0 if pc.recent else agex))
                    _drain(main)
            if "j" in ph:
                jax.lax.fori_loop(0, GH // sp, rows, None)

            @pl.when(g + 1 < NG)
            def _():
                for cp in cp_w(g + 1):
                    cp.wait()

            def attention(hh, _):
                pc = pace(g, agea)
                nxt = jnp.minimum(g + 1, NG - 1)
                attend(pc, g, hh * hp, _chain(*[prep_w(pc, nxt, hh * hp + i) for i in range(hp)]), 56 * hp)
            if "a" in ph:
                jax.lax.fori_loop(0, GH // hp, attention, None)
            else:
                ctx[0, 0:8, :] = ks[0, 0:8, :] | vs[0, 0:8, :]

        jax.lax.fori_loop(0, NG, group, None)

    heads()

    def rows_phase():
        def cp_xa(t):
            return pltpu.make_async_copy(xa32.at[_rows(t * (RO // 2), RO // 2), :],
                                         xa_raw.at[t % 3], sem_xa.at[t % 3])

        def cp_out(t, part):
            at = (_rows(t * RO, RO), pl.ds(part * DM, DM))
            return pltpu.make_async_copy(stage.at[at], out_hbm.at[at], sem_out.at[part, t])

        def prep_ctx(pc, t, i, groups=range(NG)):
            for a in range(0, RA, 8):
                for p in groups:
                    z = zero(t, i)
                    x = pc.blocks(lambda b, k: ctx[p * GH + k + z, _rows(t * (RO // 2) + b * RA + a, 8), :])
                    for n, y in _seven(_lhs_term, [[_b16(w).astype(F32) for w in row] for row in x], i):
                        xc[n, _rows(p // 2 * RA + a, 8), _rows(p % 2 * 128, 128)] = _shuffled(y)
                    yield

        def prep_xa(pc, t, i):
            for a in range(0, RA, 8):
                for c in range(2):
                    slot = t % 3 + zero(t, i)
                    x = pc.blocks(lambda b, k: xa_raw[slot, b * RA + a:b * RA + a + 8, (2 * k + c) * 128:(2 * k + c + 1) * 128])
                    for n, y in _seven(_lhs_term, [[_halves(w) for w in row] for row in x], i):
                        xc[n, pl.ds(4 * RA + a, 8), c * 128:(c + 1) * 128] = _words(y)
                    yield

        def window_weights(pc, t):
            lane = jax.lax.broadcasted_iota(jnp.int32, (sm, 128), 1)

            def softmax(a):
                tie = pc.after()
                logits = []
                for w in range(WIN):
                    x = jnp.concatenate([tie(pa[w + zero(t, 1), b:b + 8, :]) for b in range(a, a + sm, 8)], axis=0)
                    for bit in (16, 1):
                        x = x + jnp.where((lane & bit) != 0, pltpu.roll(x, bit, 1), pltpu.roll(x, 128 - bit, 1))
                    if a < DIL * w:
                        pos = jax.lax.broadcasted_iota(jnp.int32, (sm, 128), 0) + (t * RO + a)
                        x = jnp.where(pos >= DIL * w, x, NEG)
                    logits.append(x)
                top = functools.reduce(jnp.maximum, logits)
                es = [jnp.exp2(x - top) for x in logits]
                inv = _recip(functools.reduce(jnp.add, es))
                for w, e in enumerate(es):
                    pa[w, a:a + sm, :] = e * inv

            for a in range(0, RO, 8):
                for w in range(WIN):
                    if w % lw == 0:
                        tie = pc.after()
                        q = [tie(qa[j, a:a + 8, :]) for j in range(8)]
                    b = a + HALO - DIL * w
                    x = q[0] * ka[0, b:b + 8, :]
                    for j in range(1, 8):
                        x = x + q[j] * ka[j, b:b + 8, :]
                    pa[w, a:a + 8, :] = x
                    if w % lw == lw - 1:
                        yield
                if (a + 8) % sm == 0:
                    softmax(a + 8 - sm)
                    yield
            ka[:, 0:HALO, :] = ka[:, RO:, :]

        def window_mix(pc, t):
            for a in range(0, RO, 8):
                for j in range(8):
                    if j % lj == 0:
                        tie = pc.after()
                        ps = [tie(pa[w + zero(t, 0), a:a + 8, :]) for w in range(WIN)]
                    acc = ps[0] * va[j, a + HALO:a + HALO + 8, :]
                    for w in range(1, WIN):
                        b = a + HALO - DIL * w
                        acc = acc + ps[w] * va[j, b:b + 8, :]
                    ya[j, a:a + 8, :] = acc
                    if j % lj == lj - 1:
                        yield
            va[:, 0:HALO, :] = va[:, RO:, :]
            for i in range(7):
                for a in range(0, RA, 8):
                    for c in range(2):
                        z = zero(t, i)
                        x = [pc.blocks(lambda b, k: ya[2 * k + c + z, pl.ds(2 * (b * RA + a) + e, 8, stride=2), :])
                             for e in range(2)]
                        x = [[jnp.concatenate(w, axis=0) for w in zip(*rows)] for rows in zip(*x)]
                        for n, y in _seven(_lhs_term, x, i):
                            xc[n, pl.ds(5 * RA + a, 8), c * 128:(c + 1) * 128] = _words(y)
                        yield

        def joined(c):
            return jnp.concatenate([jnp.concatenate(row, axis=1) for row in c], axis=0)

        steps = S // RO
        cp_xa(0).start()
        cp_xa(1).start()
        ka[:, 0:HALO, :] = jnp.zeros((8, HALO, 128), F32)
        va[:, 0:HALO, :] = jnp.zeros((8, HALO, 128), F32)

        def first_ctx(p, _):
            for i in range(7):
                _drain(prep_ctx(pace(p, 1), 0, i, [p]))
        if "p" in ph:
            jax.lax.fori_loop(0, NG, first_ctx, None)
        cp_xa(0).wait()
        if "p" in ph:
            for i in range(7):
                _drain(prep_xa(pace(0, 1), 0, i))

        def step(t, _):
            nxt = jnp.minimum(t + 1, steps - 1)
            pc = pace(t, ager)

            @pl.when(t + 2 < steps)
            def _():
                cp_xa(t + 2).start()

            @pl.when(t + 1 < steps)
            def _():
                cp_xa(t + 1).wait()

            def times(first, w):
                def run(n):
                    y = None
                    for k in range(w.shape[1] // 128):
                        z = pc.note(_dot(xc[n, pl.ds((first + k) * RA, RA), :], w[n, k * 128:(k + 1) * 128, :]))
                        y = z if y is None else y + z
                        yield
                    return y
                return _combine(run)

            k = joined(_drain(times(4, wa.at[1])))
            for j in range(8):
                ka[j, HALO:, :] = k[:, j * 128:(j + 1) * 128]
            q = joined(_drain(times(4, wa.at[0]))) * (DA ** -0.5 * LOG2E)
            for j in range(8):
                qa[j] = q[:, j * 128:(j + 1) * 128]
            v, b = times(4, wa.at[2]), times(0, wo)

            def later():
                for i in range(7):
                    yield from _woven(v, 7, prep_xa(pc, nxt, i - 1) if i else iter(()), 8 if i else 0)
                y = joined(_drain(v))
                for j in range(8):
                    va[j, HALO:, :] = y[:, j * 128:(j + 1) * 128]
                yield from _woven(b, 28, prep_xa(pc, nxt, 6), 8)
                for i in range(1, 7):
                    yield from _woven(b, 28, prep_ctx(pc, nxt, i - 1), 32)

            rest = later()
            _drain(_woven(rest, nx, iter(()), 0))
            _drain(_woven(rest, n1, window_weights(pc, t), 32 * (WIN // lw) + RO // sm))
            _drain(_woven(rest, 5 * NP - nx - n1 - n2, window_mix(pc, t), 32 * (8 // lj) + 56))
            _drain(rest)
            stage[_rows(t * RO, RO), DM:] = joined(_drain(b)).astype(BF16)
            cp_out(t, 1).start()
            y = times(5, wa.at[3])
            _drain(_woven(y, NP - 7, prep_ctx(pc, nxt, 6), 32))
            stage[_rows(t * RO, RO), 0:DM] = joined(_drain(y)).astype(BF16)
            cp_out(t, 0).start()

        if "r" in ph:
            jax.lax.fori_loop(0, steps, step, None)
        else:
            stage[0:16, 0:128] = _b16(ctx[0, 0:8, :] | wo[0, 0:8, 0:128] | wa[0, 0, 0:8, 0:128])
        for t in range(steps):
            cp_out(t, 1).wait()
            cp_out(t, 0).wait()

    rows_phase()


def build(pred=8, **cfg):
    flags = {"XLA_TPU_MAX_INSTS_TO_PREDICATE": pred} if pred is not None else None
    vm, dma = pltpu.VMEM, pltpu.SemaphoreType.DMA
    scratch = [
        vm((HB + GH, S // 2, DB), U32),
        vm((NP, HB * DB // 8, DM // 4), U32), vm((4, NP, DM // 8, DM // 4), U32),
        vm((2, 4, 16 * cfg["sp"], DM), U32), vm((2, 4, 16 * cfg["sp"], DM), U32),
        vm((NP, S // 8, DM // 4), U32), vm((NP, S // 8, DC // 4), U32), vm((NP + 8, 4 * TILE, DB), U32),
        vm((2, 2, DM, DB), U32), vm((2, 2, 2, DC, DB), U32),
        vm((GH, S // 2, DB), U32), vm((GH, S // 2, DB), U32),
        vm((8, RO, 128), F32), vm((8, HALO + RO, 128), F32), vm((8, HALO + RO, 128), F32),
        vm((8, RO, 128), F32), vm((WIN, RO, 128), F32),
        vm((3, RO // 2, DM), U32), vm((S, 2 * DM), BF16),
        dma((2,)), dma((2,)), dma((2, 3, 2)), dma((GH,)), dma((3,)), dma((2, S // RO)),
    ]

    @jax.jit
    def run(A_x, A_wqkv, A_wo, B_x, B_c_kv, B_w_q, B_w_uk, B_w_uv, B_w_o):
        out = pl.pallas_call(
            functools.partial(_kernel, **cfg),
            out_shape=jax.ShapeDtypeStruct((S, 2 * DM), BF16),
            in_specs=[pl.BlockSpec(memory_space=pl.ANY)] * 9,
            out_specs=pl.BlockSpec(memory_space=pl.ANY),
            scratch_shapes=scratch,
            compiler_params=pltpu.CompilerParams(vmem_limit_bytes=128 * 2**20, flags=flags),
            name="fused",
        )(A_x.reshape(S, DM), A_wqkv, A_wo.reshape(8, DM // 8, DM),
          B_x.reshape(S, DM), B_c_kv.reshape(S, DC), B_w_q, B_w_uk, B_w_uv, B_w_o)
        return out.reshape(1, S, 2 * DM)

    return run


@jax.jit
def pallas_concat_heads__sliding_local_dilated__compressed_kv_cla__prompt_kernel(
    A_x: jax.Array,
    A_wqkv: jax.Array,
    A_wo: jax.Array,
    B_x: jax.Array,
    B_c_kv: jax.Array,
    B_w_q: jax.Array,
    B_w_uk: jax.Array,
    B_w_uv: jax.Array,
    B_w_o: jax.Array,
):
    return build(**CFG)(A_x, A_wqkv, A_wo, B_x, B_c_kv, B_w_q, B_w_uk, B_w_uv, B_w_o)
```

```python
import functools
import math

import jax
import jax.numpy as jnp
from jax.experimental import pallas as pl
from jax.experimental.pallas import tpu as pltpu

S = 2048
DM = 1024
HA, DA = 32, 32
WIN, DIL = 8, 2
HB, DB = 32, 128
DC = 512
NEG = -1e9
LOG2E = math.log2(math.e)

GH = 4
NG = HB // GH
SET = S // GH
RO = 256
HALO = 16
NP = 49
TILE = 64

F32, BF16, U32 = jnp.float32, jnp.bfloat16, jnp.uint32
NT = (((1,), (1,)), ((), ()))

CFG = dict(ph="pjar", ch=4, lag=12, nx=6, agep=6, agea=3, ager=6, lw=2, lj=2, sa=3, n1=112, n2=6, sm=16,
           hp=2, sp=2, pin=16, agex=12, order='qkv', tailp=14)

RA = RO // 8


def _b16(x32):
    return pltpu.bitcast(x32, BF16)


def _pack2(lo, hi):
    return pltpu.pack_elementwise([lo, hi], packed_dtype=BF16)


def _halves(w):
    return jnp.concatenate([pltpu.unpack_elementwise(w, index=i, packed_dtype=BF16, unpacked_dtype=F32)
                            for i in range(2)], axis=0)


def _words(x):
    n = x.shape[0] // 2
    return _pack2(x[:n], x[n:])


def _shuffled(x):
    parts = [_pack2(x[r:r + 8], x[r + 8:r + 16]) for r in range(0, x.shape[0], 16)]
    return jnp.concatenate(parts, axis=0) if len(parts) > 1 else parts[0]


def _dot(a32, b32):
    return jnp.dot(_b16(a32), _b16(b32), preferred_element_type=F32)


def _recip(x):
    r = pl.reciprocal(x, approx=True)
    return r * (2.0 - x * r)


def _rows(start, size, align=None):
    return pl.ds(start if isinstance(start, int) else pl.multiple_of(start, align or size), size)


def _fold(f, x):
    return functools.reduce(f, [x[:, c:c + 128] for c in range(0, x.shape[1], 128)])


def _quads(x):
    n = len(x) // 2
    return ([r[:n] for r in x[:n]], [r[n:] for r in x[:n]],
            [r[:n] for r in x[n:]], [r[n:] for r in x[n:]])


def _add(x, y):
    return [[a + b for a, b in zip(r, s)] for r, s in zip(x, y)]


def _sub(x, y):
    return [[a - b for a, b in zip(r, s)] for r, s in zip(x, y)]


def _lhs_term(x, i):
    a11, a12, a21, a22 = _quads(x)
    return (lambda: a11, lambda: _add(a11, a12), lambda: _add(a21, a22), lambda: a22,
            lambda: _add(a11, a22), lambda: _sub(a12, a22), lambda: _sub(a21, a11))[i]()


def _rhs_term(x, i):
    b11, b12, b21, b22 = _quads(x)
    return (lambda: _sub(b12, b22), lambda: b22, lambda: b11, lambda: _sub(b21, b11),
            lambda: _add(b11, b22), lambda: _add(b21, b22), lambda: _add(b11, b12))[i]()


def _seven(term, x, i):
    y = term(x, i)
    return [(7 * i + j, term(y, j)[0][0]) for j in range(7)]


def _combine(product, level=2, base=0):
    if level == 0:
        return [[(yield from product(base))]]
    k = 7 ** (level - 1)
    m3 = yield from _combine(product, level - 1, base)
    m5 = yield from _combine(product, level - 1, base + k)
    c12 = _add(m3, m5)
    m2 = yield from _combine(product, level - 1, base + 2 * k)
    c22 = _sub(m3, m2)
    m4 = yield from _combine(product, level - 1, base + 3 * k)
    c21 = _add(m2, m4)
    c11 = _sub(m4, m5)
    m1 = yield from _combine(product, level - 1, base + 4 * k)
    c11 = _add(c11, m1)
    c22 = _add(c22, m1)
    c11 = _add(c11, (yield from _combine(product, level - 1, base + 5 * k)))
    c22 = _add(c22, (yield from _combine(product, level - 1, base + 6 * k)))
    return [r + s for r, s in zip(c11, c12)] + [r + s for r, s in zip(c21, c22)]


def _drain(gen):
    while True:
        try:
            next(gen)
        except StopIteration as e:
            return e.value


def _chain(*gens):
    for g in gens:
        yield from g


def _woven(main, count, side, side_count, skip=0):
    done = 0
    for _ in range(skip):
        next(main)
        yield
    count -= skip
    for i in range(count):
        while done < side_count and done * count < (i + 1) * side_count:
            next(side)
            done += 1
        next(main)
        yield
    _drain(side)


class _Pace:
    def __init__(self, zero, age):
        self.zero, self.age, self.recent = zero, age, []

    def note(self, y):
        self.recent.append(y[:, -128:])
        return y

    def after(self, age=None):
        age = age or self.age
        if len(self.recent) < age:
            return lambda x: x
        bits = pltpu.bitcast(self.recent[-age][:8], U32) & self.zero
        return lambda x: pltpu.bitcast(pltpu.bitcast(x, U32) | bits, x.dtype)

    def tied(self, x, y):
        zero = jnp.concatenate([self.zero] * (x.shape[0] // 8), axis=0)
        return pltpu.bitcast(pltpu.bitcast(x, U32) | (pltpu.bitcast(y, U32) & zero), x.dtype)

    def blocks(self, load):
        tie = self.after()
        return [[tie(load(i, j)) if i % 2 == 0 and j % 2 == 0 else load(i, j) for j in range(4)]
                for i in range(4)]


def _swap_lane_and_chunk_bits(chunks):
    lane = jax.lax.broadcasted_iota(jnp.int32, chunks[0].shape, 1)
    u = (lane >> 1) & 7
    rolled = [x if c == 0 else pltpu.roll(x, 2 * c, 1) for c, x in enumerate(chunks)]
    xs = [rolled[(-i) % 8] for i in range(8)]
    for t in (1, 2, 4):
        m = (u & t) != 0
        xs = [jnp.where(m, xs[(i - t) % 8], xs[i]) for i in range(8)]
    return [x if j == 0 else pltpu.roll(x, 128 - 2 * j, 1) for j, x in enumerate(xs)]


def _kernel(xa_hbm, wqkv_hbm, woa_hbm, xb_hbm, c_hbm, wq_hbm, wuk_hbm, wuv_hbm, wob_hbm,
            out_hbm,
            ctx, wo, wa, wo_raw, wa_raw, xc, cc, wb, wq_raw, wkv_raw, ks, vs,
            qa, ka, va, ya, pa, xa_raw, stage,
            sem_wo, sem_wa, sem_w, sem_x, sem_xa, sem_out, *,
            ph, ch, lag, nx, agep, agea, ager, lw, lj, sa, n1, n2, sm, hp, sp, pin, agex, order, tailp):
    xa32, wqkv32, woa32 = (r.bitcast(U32) for r in (xa_hbm, wqkv_hbm, woa_hbm))
    xb32, c32, wob32 = (r.bitcast(U32) for r in (xb_hbm, c_hbm, wob_hbm))
    wq32, wk32, wv32 = (r.bitcast(U32) for r in (wq_hbm, wuk_hbm, wuv_hbm))

    def pace(step, age):
        return _Pace(jnp.full((8, 128), step // S, jnp.int32).astype(U32), age)

    def zero(step, salt):
        return step // (S + salt)

    def start_slabs(i):
        u, n = i * sp, 16 * sp
        for k in range(4):
            pltpu.make_async_copy(wob32.at[u // GH * GH + k, _rows(u % GH * 16, n), :],
                                  wo_raw.at[i % 2, k], sem_wo.at[i % 2]).start()

        @pl.when(u < 24)
        def _():
            for k in range(4):
                pltpu.make_async_copy(wqkv32.at[_rows(k * 128 + u % 8 * 16, n), _rows(u // 8 * DM, DM)],
                                      wa_raw.at[i % 2, k], sem_wa.at[i % 2]).start()

        @pl.when(u >= 24)
        def _():
            for k in range(4):
                for e in range(n // 8):
                    m = k * 16 + u % 8 * 2 + e
                    pltpu.make_async_copy(woa32.at[:, ((m >> 1) & 3) * 16 + (m & 1) * 8 + (m >> 3), :],
                                          wa_raw.at[i % 2, k, pl.ds(8 * e, 8), :], sem_wa.at[i % 2]).start()

    def wait_slabs(i):
        for raw, sem in ((wo_raw, sem_wo), (wa_raw, sem_wa)):
            pltpu.make_async_copy(raw.at[i % 2], raw.at[i % 2], sem.at[i % 2]).wait()

    def prep_slabs(pc, u, load, store):
        for half in range(2):
            for c in range(2):
                for i in range(7):
                    z = zero(u, i)
                    x = pc.blocks(lambda k, j: load(z, k, half * 8, 2 * j + c))
                    for n, y in _seven(_rhs_term, [[_halves(w) for w in r] for r in x], i):
                        store(n, half * 8, c, _words(y))
                    yield

    def prep_wo(pc, u, at):
        def store(n, row, c, y):
            wo[n, _rows(u * 16 + row, 8), c * 128:(c + 1) * 128] = y
        return prep_slabs(
            pc, u, lambda z, k, row, c: wo_raw[u // sp % 2 + z, k, pl.ds(at + row, 8), c * 128:(c + 1) * 128], store)

    def permute_wa(pc, u, at):
        for i in range(4):
            for half in range(2):
                tie = pc.after(agex)
                raw = [tie(wa_raw[u // sp % 2, i, pl.ds(at + half * 8, 8), c * 128:(c + 1) * 128])
                       for c in range(8)]
                for c, y in enumerate(_swap_lane_and_chunk_bits(raw)):
                    wb[NP + c, pl.ds(i * 16 + half * 8, 8), :] = jnp.where(u < 24, y, raw[c])
                yield

    def prep_wa(pc, u):
        def store(n, row, c, y):
            wa[u // 8, n, _rows(u % 8 * 16 + row, 8), c * 128:(c + 1) * 128] = y
        return prep_slabs(pc, u, lambda z, k, row, c: wb[NP + c + z, k * 16 + row:k * 16 + row + 8, :], store)

    def heads():
        def cp_w(g):
            return [pltpu.make_async_copy(src.at[:, 2 * g + i, :], dst.at[i], sem_w.at[g % 2, kind, i])
                    for kind, (src, dst) in enumerate(((wk32, wkv_raw.at[g % 2, 0]), (wv32, wkv_raw.at[g % 2, 1]),
                                                       (wq32, wq_raw.at[g % 2])))
                    for i in range(2)]

        def cp_rows(j):
            r = _rows(j * (SET // 2), SET // 2)
            return [pltpu.make_async_copy(src.at[r, t * 128:(t + 1) * 128], ctx.at[page + t, r, :], sem_x.at[j])
                    for page, src in ((0, c32), (4, xb32)) for t in range(src.shape[1] // 128)]

        def prep_rows(pc, page, dst, j, a):
            r, tiles = SET // 8, dst.shape[-1] // 128
            for t in range(tiles):
                x = [[_b16(ctx[page + k * tiles + t, _rows(j * (SET // 2) + b * r + a, 8), :]).astype(F32)
                      for k in range(4)] for b in range(4)]
                for i in range(7):
                    for n, y in _seven(_lhs_term, x, i):
                        dst[n, _rows(j * r + a, 8), t * 128:(t + 1) * 128] = _shuffled(y)
                    yield

        def prep_w(pc, g, j):
            def unit(raw, depth, a, row):
                for i in range(7):
                    z = zero(j, i)
                    x = pc.blocks(lambda k, c: raw[
                        c // 2 + z, pl.ds(k * (depth // 4) + j * (depth // 16) + a + c % 2, 8, stride=2), :])
                    x = [[_halves(w) for w in r] for r in x]
                    x = [[jnp.concatenate([r[c // 2 * 2][c % 2 * 8:c % 2 * 8 + 8],
                                           r[c // 2 * 2 + 1][c % 2 * 8:c % 2 * 8 + 8]], axis=0)
                          for c in range(4)] for r in x]
                    for n, y in _seven(_rhs_term, x, i):
                        wb[n, _rows(row, 8), :] = _words(y)
                    yield

            for a in range(0, DM // 16, 16):
                yield from unit(wq_raw.at[g % 2], DM, a, j * (DM // 32) + a // 2)
            for kind in range(2):
                for a in range(0, DC // 16, 16):
                    yield from unit(wkv_raw.at[g % 2, kind], DC, a, (2 + kind) * TILE + j * (DC // 32) + a // 2)

        def project(pc, j):
            r = SET // 8
            rows = _rows(j * r, r)

            def product(lhs, first, last):
                def run(n):
                    y = pc.note(_dot(lhs[n, rows, :], wb[n + zero(j, 0), first * TILE:last * TILE, :]))
                    yield
                    return y
                return _combine(run)

            parts = dict(q=(ctx, HB, DB ** -0.5 * LOG2E, product(xc, 0, 2)),
                         k=(ks, 0, None, product(cc, 2, 3)), v=(vs, 0, None, product(cc, 3, 4)))
            for dst, page, scale, gen in (parts[c] for c in order):
                y = yield from gen
                for i in range(4):
                    for h in range(GH):
                        dst[page + h, _rows(j * (SET // 2) + i * r, r), :] = _shuffled(
                            y[i][h] * scale if scale else y[i][h])

        def attend(pc, g, first, side, side_steps):
            nb = S // 128
            work = [(first + h, i, t, min(t + ch, i + 1))
                    for h in range(hp) for i in reversed(range(nb)) for t in range(0, i + 1, ch)]
            key = [h * nb + i for h in range(hp) for i in reversed(range(nb)) for t in range(0, i + 1, ch)]
            s, mx, m, l, o, done, ready, due = {}, {}, {}, {}, {}, {}, [], []

            def scores(b, h, i, t0, t1):
                x = pc.note(jax.lax.dot_general(_b16(ctx[HB + h, i * TILE:(i + 1) * TILE, :]),
                                                _b16(ks[h, t0 * TILE:t1 * TILE, :]), NT,
                                                preferred_element_type=F32))
                if t1 == i + 1:
                    row, col = (jax.lax.broadcasted_iota(jnp.int32, (128, 128), d) for d in range(2))
                    row, col = ((u & ~15) | ((u >> 2) & 3) | ((u & 3) << 2) for u in (row, col))
                    diag = jnp.where(col <= row, x[:, -128:], NEG)
                    x = jnp.concatenate([x[:, :-128], diag], axis=1) if t1 - t0 > 1 else diag
                s[b, t0] = x
                mx[b] = jnp.maximum(mx[b], _fold(jnp.maximum, x)) if t0 else _fold(jnp.maximum, x)
                if t1 == i + 1:
                    m[b] = jnp.max(mx[b], axis=1, keepdims=True)

            def values(b, h, i, t0, t1):
                p = jnp.exp2(s.pop((b, t0)) - m[b])
                y = pc.note(jnp.dot(p.astype(BF16), _b16(vs[h, t0 * TILE:t1 * TILE, :]),
                                    preferred_element_type=F32))
                parts = ([l[b]] if t0 else []) + [p[:, c:c + 128] for c in range(0, p.shape[1], 128)]
                l[b] = functools.reduce(jnp.add, [pc.tied(parts[0], pc.recent[-1 - sa])] + parts[1:])
                o[b] = o[b] + y if t0 else y
                if t1 == i + 1:
                    ready.append((h, i, _shuffled(o[b] * _recip(jnp.sum(l[b], axis=1, keepdims=True)))))

            def products():
                clock = qi = pi = turn = 0
                while pi < len(work):
                    can = key[pi] in done and clock - done[key[pi]] >= lag
                    if qi < len(work) and (not can or turn == 0):
                        scores(key[qi], *work[qi])
                        clock += work[qi][3] - work[qi][2]
                        if work[qi][3] == work[qi][1] + 1:
                            done[key[qi]] = clock
                        qi, turn = qi + 1, 1
                    else:
                        values(key[pi], *work[pi])
                        clock += work[pi][3] - work[pi][2]
                        if len(due) < len(ready):
                            due.append(clock + pin)
                        pi, turn = pi + 1, 0
                    while due and (due[0] <= clock or pi == len(work)):
                        due.pop(0)
                        h, i, x = ready.pop(0)
                        ctx[g * GH + h, i * TILE:(i + 1) * TILE, :] = x
                    yield

            main = products()
            _drain(_woven(main, 2 * len(work) - 16, side, side_steps, agea))
            _drain(main)

        for cp in cp_w(0) + cp_rows(0) + cp_rows(1):
            cp.start()
        start_slabs(jnp.int32(0))
        for cp in cp_w(0):
            cp.wait()
        jax.lax.fori_loop(0, GH, lambda j, _: _drain(prep_w(pace(j, 1), 0, j)), None)

        def group(g, _):
            def rows(jj, _):
                @pl.when(g == 0)
                def _():
                    for j in [jj * sp + i for i in range(sp)]:
                        @pl.when(j + 2 < GH)
                        def _():
                            for cp in cp_rows(j + 2):
                                cp.start()
                        for cp in cp_rows(j):
                            cp.wait()

                        @pl.when(j == GH - 1)
                        def _():
                            for cp in cp_w(1):
                                cp.start()

                        def first_rows(a, _):
                            _drain(prep_rows(None, 0, cc, j, a * 8))
                            _drain(prep_rows(None, 4, xc, j, a * 8))
                        jax.lax.fori_loop(0, SET // 64, first_rows, None)


                i = g * (GH // sp) + jj

                @pl.when(i + 1 < HB // sp)
                def _():
                    start_slabs(i + 1)
                wait_slabs(i)
                pc = pace(g, agep)
                for n in range(sp):
                    j = jj * sp + n
                    u = g * GH + j
                    side = _chain(_woven(prep_wo(pc, u, 16 * n), 28, permute_wa(pc, u, 16 * n), 8), prep_wa(pc, u))
                    main = project(pc, j)
                    _drain(_woven(main, 3 * NP - tailp, side, 56, 0 if pc.recent else agex))
                    _drain(main)
            @pl.when((g > 0) & (g + 1 < NG))
            def _():
                for cp in cp_w(g + 1):
                    cp.start()
            if "j" in ph:
                jax.lax.fori_loop(0, GH // sp, rows, None)

            @pl.when(g + 1 < NG)
            def _():
                for cp in cp_w(g + 1):
                    cp.wait()

            def attention(hh, _):
                pc = pace(g, agea)
                nxt = jnp.minimum(g + 1, NG - 1)
                attend(pc, g, hh * hp, _chain(*[prep_w(pc, nxt, hh * hp + i) for i in range(hp)]), 56 * hp)
            if "a" in ph:
                jax.lax.fori_loop(0, GH // hp, attention, None)
            else:
                ctx[0, 0:8, :] = ks[0, 0:8, :] | vs[0, 0:8, :]

        jax.lax.fori_loop(0, NG, group, None)

    heads()

    def rows_phase():
        def cp_xa(t):
            return pltpu.make_async_copy(xa32.at[_rows(jnp.minimum(t, S // RO - 1) * (RO // 2), RO // 2), :],
                                         xa_raw.at[t % 3], sem_xa.at[t % 3])

        def cp_out(t, part):
            at = (_rows(t * RO, RO), pl.ds(part * DM, DM))
            return pltpu.make_async_copy(stage.at[at], out_hbm.at[at], sem_out.at[part, t])

        def prep_ctx(pc, t, i, groups=range(NG)):
            for a in range(0, RA, 8):
                for p in groups:
                    z = zero(t, i)
                    x = pc.blocks(lambda b, k: ctx[p * GH + k + z, _rows(t * (RO // 2) + b * RA + a, 8), :])
                    for n, y in _seven(_lhs_term, [[_b16(w).astype(F32) for w in row] for row in x], i):
                        xc[n, _rows(p // 2 * RA + a, 8), _rows(p % 2 * 128, 128)] = _shuffled(y)
                    yield

        def prep_xa(pc, t, i):
            for a in range(0, RA, 8):
                for c in range(2):
                    slot = t % 3 + zero(t, i)
                    x = pc.blocks(lambda b, k: xa_raw[slot, b * RA + a:b * RA + a + 8, (2 * k + c) * 128:(2 * k + c + 1) * 128])
                    for n, y in _seven(_lhs_term, [[_halves(w) for w in row] for row in x], i):
                        xc[n, pl.ds(4 * RA + a, 8), c * 128:(c + 1) * 128] = _words(y)
                    yield

        def window_weights(pc, t):
            lane = jax.lax.broadcasted_iota(jnp.int32, (sm, 128), 1)

            def softmax(a):
                tie = pc.after()
                logits = []
                for w in range(WIN):
                    x = jnp.concatenate([tie(pa[w + zero(t, 1), b:b + 8, :]) for b in range(a, a + sm, 8)], axis=0)
                    for bit in (16, 1):
                        x = x + jnp.where((lane & bit) != 0, pltpu.roll(x, bit, 1), pltpu.roll(x, 128 - bit, 1))
                    if a < DIL * w:
                        pos = jax.lax.broadcasted_iota(jnp.int32, (sm, 128), 0) + (t * RO + a)
                        x = jnp.where(pos >= DIL * w, x, NEG)
                    logits.append(x)
                top = functools.reduce(jnp.maximum, logits)
                es = [jnp.exp2(x - top) for x in logits]
                inv = _recip(functools.reduce(jnp.add, es))
                for w, e in enumerate(es):
                    pa[w, a:a + sm, :] = e * inv

            for a in range(0, RO, 8):
                for w in range(WIN):
                    if w % lw == 0:
                        tie = pc.after()
                        q = [tie(qa[j, a:a + 8, :]) for j in range(8)]
                    b = a + HALO - DIL * w
                    x = q[0] * ka[0, b:b + 8, :]
                    for j in range(1, 8):
                        x = x + q[j] * ka[j, b:b + 8, :]
                    pa[w, a:a + 8, :] = x
                    if w % lw == lw - 1:
                        yield
                if (a + 8) % sm == 0:
                    softmax(a + 8 - sm)
                    yield
            ka[:, 0:HALO, :] = ka[:, RO:, :]

        def window_mix(pc, t):
            for a in range(0, RO, 8):
                for j in range(8):
                    if j % lj == 0:
                        tie = pc.after()
                        ps = [tie(pa[w + zero(t, 0), a:a + 8, :]) for w in range(WIN)]
                    acc = ps[0] * va[j, a + HALO:a + HALO + 8, :]
                    for w in range(1, WIN):
                        b = a + HALO - DIL * w
                        acc = acc + ps[w] * va[j, b:b + 8, :]
                    ya[j, a:a + 8, :] = acc
                    if j % lj == lj - 1:
                        yield
            va[:, 0:HALO, :] = va[:, RO:, :]
            for i in range(7):
                for a in range(0, RA, 8):
                    for c in range(2):
                        z = zero(t, i)
                        x = [pc.blocks(lambda b, k: ya[2 * k + c + z, pl.ds(2 * (b * RA + a) + e, 8, stride=2), :])
                             for e in range(2)]
                        x = [[jnp.concatenate(w, axis=0) for w in zip(*rows)] for rows in zip(*x)]
                        for n, y in _seven(_lhs_term, x, i):
                            xc[n, pl.ds(5 * RA + a, 8), c * 128:(c + 1) * 128] = _words(y)
                        yield

        def joined(c):
            return jnp.concatenate([jnp.concatenate(row, axis=1) for row in c], axis=0)

        steps = S // RO
        cp_xa(0).start()
        cp_xa(1).start()
        ka[:, 0:HALO, :] = jnp.zeros((8, HALO, 128), F32)
        va[:, 0:HALO, :] = jnp.zeros((8, HALO, 128), F32)

        def first_ctx(p, _):
            for i in range(7):
                _drain(prep_ctx(pace(p, 1), 0, i, [p]))
        if "p" in ph:
            jax.lax.fori_loop(0, NG, first_ctx, None)
        cp_xa(0).wait()
        if "p" in ph:
            for i in range(7):
                _drain(prep_xa(pace(0, 1), 0, i))

        def step(t, _):
            nxt = jnp.minimum(t + 1, steps - 1)
            pc = pace(t, ager)

            cp_xa(t + 2).start()
            cp_xa(t + 1).wait()

            def times(first, w):
                def run(n):
                    y = None
                    for k in range(w.shape[1] // 128):
                        z = pc.note(_dot(xc[n, pl.ds((first + k) * RA, RA), :], w[n, k * 128:(k + 1) * 128, :]))
                        y = z if y is None else y + z
                        yield
                    return y
                return _combine(run)

            k = joined(_drain(times(4, wa.at[1])))
            for j in range(8):
                ka[j, HALO:, :] = k[:, j * 128:(j + 1) * 128]
            q = joined(_drain(times(4, wa.at[0]))) * (DA ** -0.5 * LOG2E)
            for j in range(8):
                qa[j] = q[:, j * 128:(j + 1) * 128]
            v, b = times(4, wa.at[2]), times(0, wo)

            def later():
                for i in range(7):
                    yield from _woven(v, 7, prep_xa(pc, t + 1, i - 1) if i else iter(()), 8 if i else 0)
                y = joined(_drain(v))
                for j in range(8):
                    va[j, HALO:, :] = y[:, j * 128:(j + 1) * 128]
                yield from _woven(b, 28, prep_xa(pc, t + 1, 6), 8)
                for i in range(1, 7):
                    yield from _woven(b, 28, prep_ctx(pc, nxt, i - 1), 32)

            rest = later()
            _drain(_woven(rest, nx, iter(()), 0))
            _drain(_woven(rest, n1, window_weights(pc, t), 32 * (WIN // lw) + RO // sm))
            _drain(_woven(rest, 5 * NP - nx - n1 - n2, window_mix(pc, t), 32 * (8 // lj) + 56))
            _drain(rest)
            stage[_rows(t * RO, RO), DM:] = joined(_drain(b)).astype(BF16)
            cp_out(t, 1).start()
            y = times(5, wa.at[3])
            _drain(_woven(y, NP - 7, prep_ctx(pc, nxt, 6), 32))
            stage[_rows(t * RO, RO), 0:DM] = joined(_drain(y)).astype(BF16)
            cp_out(t, 0).start()

        if "r" in ph:
            jax.lax.fori_loop(0, steps, step, None)
        else:
            stage[0:16, 0:128] = _b16(ctx[0, 0:8, :] | wo[0, 0:8, 0:128] | wa[0, 0, 0:8, 0:128])
        cp_xa(steps + 1).wait()
        for t in range(steps):
            cp_out(t, 1).wait()
            cp_out(t, 0).wait()

    rows_phase()


def build(pred=8, **cfg):
    flags = {"XLA_TPU_MAX_INSTS_TO_PREDICATE": pred} if pred is not None else None
    vm, dma = pltpu.VMEM, pltpu.SemaphoreType.DMA
    scratch = [
        vm((HB + GH, S // 2, DB), U32),
        vm((NP, HB * DB // 8, DM // 4), U32), vm((4, NP, DM // 8, DM // 4), U32),
        vm((2, 4, 16 * cfg["sp"], DM), U32), vm((2, 4, 16 * cfg["sp"], DM), U32),
        vm((NP, S // 8, DM // 4), U32), vm((NP, S // 8, DC // 4), U32), vm((NP + 8, 4 * TILE, DB), U32),
        vm((2, 2, DM, DB), U32), vm((2, 2, 2, DC, DB), U32),
        vm((GH, S // 2, DB), U32), vm((GH, S // 2, DB), U32),
        vm((8, RO, 128), F32), vm((8, HALO + RO, 128), F32), vm((8, HALO + RO, 128), F32),
        vm((8, RO, 128), F32), vm((WIN, RO, 128), F32),
        vm((3, RO // 2, DM), U32), vm((S, 2 * DM), BF16),
        dma((2,)), dma((2,)), dma((2, 3, 2)), dma((GH,)), dma((3,)), dma((2, S // RO)),
    ]

    @jax.jit
    def run(A_x, A_wqkv, A_wo, B_x, B_c_kv, B_w_q, B_w_uk, B_w_uv, B_w_o):
        out = pl.pallas_call(
            functools.partial(_kernel, **cfg),
            out_shape=jax.ShapeDtypeStruct((S, 2 * DM), BF16),
            in_specs=[pl.BlockSpec(memory_space=pl.ANY)] * 9,
            out_specs=pl.BlockSpec(memory_space=pl.ANY),
            scratch_shapes=scratch,
            compiler_params=pltpu.CompilerParams(vmem_limit_bytes=128 * 2**20, flags=flags),
            name="fused",
        )(A_x.reshape(S, DM), A_wqkv, A_wo.reshape(8, DM // 8, DM),
          B_x.reshape(S, DM), B_c_kv.reshape(S, DC), B_w_q, B_w_uk, B_w_uv, B_w_o)
        return out.reshape(1, S, 2 * DM)

    return run


@jax.jit
def pallas_concat_heads__sliding_local_dilated__compressed_kv_cla__prompt_kernel(
    A_x: jax.Array,
    A_wqkv: jax.Array,
    A_wo: jax.Array,
    B_x: jax.Array,
    B_c_kv: jax.Array,
    B_w_q: jax.Array,
    B_w_uk: jax.Array,
    B_w_uv: jax.Array,
    B_w_o: jax.Array,
):
    return build(**CFG)(A_x, A_wqkv, A_wo, B_x, B_c_kv, B_w_q, B_w_uk, B_w_uv, B_w_o)
```

```python
import functools
import math

import jax
import jax.numpy as jnp
from jax.experimental import pallas as pl
from jax.experimental.pallas import tpu as pltpu

S = 2048
DM = 1024
HA, DA = 32, 32
WIN, DIL = 8, 2
HB, DB = 32, 128
DC = 512
NEG = -1e9
LOG2E = math.log2(math.e)

GH = 4
NG = HB // GH
SET = S // GH
RO = 256
HALO = 16
NP = 49
TILE = 64

F32, BF16, U32 = jnp.float32, jnp.bfloat16, jnp.uint32
NT = (((1,), (1,)), ((), ()))

CFG = dict(ph="pjar", ch=4, lag=12, n0=150, early=1, agep=6, agea=3, ager=8, lw=2, lj=2, sa=3, n1=110, n2=6, sm=16,
           hp=2, sp=2, pin=16, agex=12, order='qkv', tailp=14)

RA = RO // 8


def _b16(x32):
    return pltpu.bitcast(x32, BF16)


def _pack2(lo, hi):
    return pltpu.pack_elementwise([lo, hi], packed_dtype=BF16)


def _halves(w):
    return jnp.concatenate([pltpu.unpack_elementwise(w, index=i, packed_dtype=BF16, unpacked_dtype=F32)
                            for i in range(2)], axis=0)


def _words(x):
    n = x.shape[0] // 2
    return _pack2(x[:n], x[n:])


def _shuffled(x):
    parts = [_pack2(x[r:r + 8], x[r + 8:r + 16]) for r in range(0, x.shape[0], 16)]
    return jnp.concatenate(parts, axis=0) if len(parts) > 1 else parts[0]


def _dot(a32, b32):
    return jnp.dot(_b16(a32), _b16(b32), preferred_element_type=F32)


def _recip(x):
    r = pl.reciprocal(x, approx=True)
    return r * (2.0 - x * r)


def _rows(start, size, align=None):
    return pl.ds(start if isinstance(start, int) else pl.multiple_of(start, align or size), size)


def _fold(f, x):
    return functools.reduce(f, [x[:, c:c + 128] for c in range(0, x.shape[1], 128)])


def _quads(x):
    n = len(x) // 2
    return ([r[:n] for r in x[:n]], [r[n:] for r in x[:n]],
            [r[:n] for r in x[n:]], [r[n:] for r in x[n:]])


def _add(x, y):
    return [[a + b for a, b in zip(r, s)] for r, s in zip(x, y)]


def _sub(x, y):
    return [[a - b for a, b in zip(r, s)] for r, s in zip(x, y)]


def _lhs_term(x, i):
    a11, a12, a21, a22 = _quads(x)
    return (lambda: a11, lambda: _add(a11, a12), lambda: _add(a21, a22), lambda: a22,
            lambda: _add(a11, a22), lambda: _sub(a12, a22), lambda: _sub(a21, a11))[i]()


def _rhs_term(x, i):
    b11, b12, b21, b22 = _quads(x)
    return (lambda: _sub(b12, b22), lambda: b22, lambda: b11, lambda: _sub(b21, b11),
            lambda: _add(b11, b22), lambda: _add(b21, b22), lambda: _add(b11, b12))[i]()


def _seven(term, x, i):
    y = term(x, i)
    return [(7 * i + j, term(y, j)[0][0]) for j in range(7)]


def _combine(product, level=2, base=0):
    if level == 0:
        return [[(yield from product(base))]]
    k = 7 ** (level - 1)
    m3 = yield from _combine(product, level - 1, base)
    m5 = yield from _combine(product, level - 1, base + k)
    c12 = _add(m3, m5)
    m2 = yield from _combine(product, level - 1, base + 2 * k)
    c22 = _sub(m3, m2)
    m4 = yield from _combine(product, level - 1, base + 3 * k)
    c21 = _add(m2, m4)
    c11 = _sub(m4, m5)
    m1 = yield from _combine(product, level - 1, base + 4 * k)
    c11 = _add(c11, m1)
    c22 = _add(c22, m1)
    c11 = _add(c11, (yield from _combine(product, level - 1, base + 5 * k)))
    c22 = _add(c22, (yield from _combine(product, level - 1, base + 6 * k)))
    return [r + s for r, s in zip(c11, c12)] + [r + s for r, s in zip(c21, c22)]


def _drain(gen):
    while True:
        try:
            next(gen)
        except StopIteration as e:
            return e.value


def _chain(*gens):
    for g in gens:
        yield from g


def _woven(main, count, side, side_count, skip=0):
    done = 0
    for _ in range(skip):
        next(main)
        yield
    count -= skip
    for i in range(count):
        while done < side_count and done * count < (i + 1) * side_count:
            next(side)
            done += 1
        next(main)
        yield
    _drain(side)


class _Pace:
    def __init__(self, zero, age):
        self.zero, self.age, self.recent = zero, age, []

    def note(self, y):
        self.recent.append(y[:, -128:])
        return y

    def after(self, age=None):
        age = age or self.age
        if len(self.recent) < age:
            return lambda x: x
        bits = pltpu.bitcast(self.recent[-age][:8], U32) & self.zero
        return lambda x: pltpu.bitcast(pltpu.bitcast(x, U32) | bits, x.dtype)

    def tied(self, x, y):
        zero = jnp.concatenate([self.zero] * (x.shape[0] // 8), axis=0)
        return pltpu.bitcast(pltpu.bitcast(x, U32) | (pltpu.bitcast(y, U32) & zero), x.dtype)

    def blocks(self, load):
        tie = self.after()
        return [[tie(load(i, j)) if i % 2 == 0 and j % 2 == 0 else load(i, j) for j in range(4)]
                for i in range(4)]


def _swap_lane_and_chunk_bits(chunks):
    lane = jax.lax.broadcasted_iota(jnp.int32, chunks[0].shape, 1)
    u = (lane >> 1) & 7
    rolled = [x if c == 0 else pltpu.roll(x, 2 * c, 1) for c, x in enumerate(chunks)]
    xs = [rolled[(-i) % 8] for i in range(8)]
    for t in (1, 2, 4):
        m = (u & t) != 0
        xs = [jnp.where(m, xs[(i - t) % 8], xs[i]) for i in range(8)]
    return [x if j == 0 else pltpu.roll(x, 128 - 2 * j, 1) for j, x in enumerate(xs)]


def _kernel(xa_hbm, wqkv_hbm, woa_hbm, xb_hbm, c_hbm, wq_hbm, wuk_hbm, wuv_hbm, wob_hbm,
            out_hbm,
            ctx, wo, wa, wo_raw, wa_raw, xc, cc, wb, wq_raw, wkv_raw, ks, vs,
            qa, ka, va, ya, pa, xa_raw, stage,
            sem_wo, sem_wa, sem_w, sem_x, sem_xa, sem_out, *,
            ph, ch, lag, n0, early, agep, agea, ager, lw, lj, sa, n1, n2, sm, hp, sp, pin, agex, order, tailp):
    xa32, wqkv32, woa32 = (r.bitcast(U32) for r in (xa_hbm, wqkv_hbm, woa_hbm))
    xb32, c32, wob32 = (r.bitcast(U32) for r in (xb_hbm, c_hbm, wob_hbm))
    wq32, wk32, wv32 = (r.bitcast(U32) for r in (wq_hbm, wuk_hbm, wuv_hbm))

    def pace(step, age):
        return _Pace(jnp.full((8, 128), step // S, jnp.int32).astype(U32), age)

    def zero(step, salt):
        return step // (S + salt)

    def start_slabs(i):
        u, n = i * sp, 16 * sp
        for k in range(4):
            pltpu.make_async_copy(wob32.at[u // GH * GH + k, _rows(u % GH * 16, n), :],
                                  wo_raw.at[i % 2, k], sem_wo.at[i % 2]).start()

        @pl.when(u < 24)
        def _():
            for k in range(4):
                pltpu.make_async_copy(wqkv32.at[_rows(k * 128 + u % 8 * 16, n), _rows(u // 8 * DM, DM)],
                                      wa_raw.at[i % 2, k], sem_wa.at[i % 2]).start()

        @pl.when(u >= 24)
        def _():
            for k in range(4):
                for e in range(n // 8):
                    m = k * 16 + u % 8 * 2 + e
                    pltpu.make_async_copy(woa32.at[:, ((m >> 1) & 3) * 16 + (m & 1) * 8 + (m >> 3), :],
                                          wa_raw.at[i % 2, k, pl.ds(8 * e, 8), :], sem_wa.at[i % 2]).start()

    def wait_slabs(i):
        for raw, sem in ((wo_raw, sem_wo), (wa_raw, sem_wa)):
            pltpu.make_async_copy(raw.at[i % 2], raw.at[i % 2], sem.at[i % 2]).wait()

    def prep_slabs(pc, u, load, store):
        for half in range(2):
            for c in range(2):
                for i in range(7):
                    z = zero(u, i)
                    x = pc.blocks(lambda k, j: load(z, k, half * 8, 2 * j + c))
                    for n, y in _seven(_rhs_term, [[_halves(w) for w in r] for r in x], i):
                        store(n, half * 8, c, _words(y))
                    yield

    def prep_wo(pc, u, at):
        def store(n, row, c, y):
            wo[n, _rows(u * 16 + row, 8), c * 128:(c + 1) * 128] = y
        return prep_slabs(
            pc, u, lambda z, k, row, c: wo_raw[u // sp % 2 + z, k, pl.ds(at + row, 8), c * 128:(c + 1) * 128], store)

    def permute_wa(pc, u, at):
        for i in range(4):
            for half in range(2):
                tie = pc.after(agex)
                raw = [tie(wa_raw[u // sp % 2, i, pl.ds(at + half * 8, 8), c * 128:(c + 1) * 128])
                       for c in range(8)]
                for c, y in enumerate(_swap_lane_and_chunk_bits(raw)):
                    wb[NP + c, pl.ds(i * 16 + half * 8, 8), :] = jnp.where(u < 24, y, raw[c])
                yield

    def prep_wa(pc, u):
        def store(n, row, c, y):
            wa[u // 8, n, _rows(u % 8 * 16 + row, 8), c * 128:(c + 1) * 128] = y
        return prep_slabs(pc, u, lambda z, k, row, c: wb[NP + c + z, k * 16 + row:k * 16 + row + 8, :], store)

    def heads():
        def cp_w(g):
            return [pltpu.make_async_copy(src.at[:, 2 * g + i, :], dst.at[i], sem_w.at[g % 2, kind, i])
                    for kind, (src, dst) in enumerate(((wk32, wkv_raw.at[g % 2, 0]), (wv32, wkv_raw.at[g % 2, 1]),
                                                       (wq32, wq_raw.at[g % 2])))
                    for i in range(2)]

        def cp_rows(j):
            r = _rows(j * (SET // 2), SET // 2)
            return [pltpu.make_async_copy(src.at[r, t * 128:(t + 1) * 128], ctx.at[page + t, r, :], sem_x.at[j])
                    for page, src in ((0, c32), (4, xb32)) for t in range(src.shape[1] // 128)]

        def prep_rows(pc, page, dst, j, a):
            r, tiles = SET // 8, dst.shape[-1] // 128
            for t in range(tiles):
                x = [[_b16(ctx[page + k * tiles + t, _rows(j * (SET // 2) + b * r + a, 8), :]).astype(F32)
                      for k in range(4)] for b in range(4)]
                for i in range(7):
                    for n, y in _seven(_lhs_term, x, i):
                        dst[n, _rows(j * r + a, 8), t * 128:(t + 1) * 128] = _shuffled(y)
                    yield

        def prep_w(pc, g, j):
            def unit(raw, depth, a, row):
                for i in range(7):
                    z = zero(j, i)
                    x = pc.blocks(lambda k, c: raw[
                        c // 2 + z, pl.ds(k * (depth // 4) + j * (depth // 16) + a + c % 2, 8, stride=2), :])
                    x = [[_halves(w) for w in r] for r in x]
                    x = [[jnp.concatenate([r[c // 2 * 2][c % 2 * 8:c % 2 * 8 + 8],
                                           r[c // 2 * 2 + 1][c % 2 * 8:c % 2 * 8 + 8]], axis=0)
                          for c in range(4)] for r in x]
                    for n, y in _seven(_rhs_term, x, i):
                        wb[n, _rows(row, 8), :] = _words(y)
                    yield

            for a in range(0, DM // 16, 16):
                yield from unit(wq_raw.at[g % 2], DM, a, j * (DM // 32) + a // 2)
            for kind in range(2):
                for a in range(0, DC // 16, 16):
                    yield from unit(wkv_raw.at[g % 2, kind], DC, a, (2 + kind) * TILE + j * (DC // 32) + a // 2)

        def project(pc, j):
            r = SET // 8
            rows = _rows(j * r, r)

            def product(lhs, first, last):
                def run(n):
                    y = pc.note(_dot(lhs[n, rows, :], wb[n + zero(j, 0), first * TILE:last * TILE, :]))
                    yield
                    return y
                return _combine(run)

            parts = dict(q=(ctx, HB, DB ** -0.5 * LOG2E, product(xc, 0, 2)),
                         k=(ks, 0, None, product(cc, 2, 3)), v=(vs, 0, None, product(cc, 3, 4)))
            for dst, page, scale, gen in (parts[c] for c in order):
                y = yield from gen
                for i in range(4):
                    for h in range(GH):
                        dst[page + h, _rows(j * (SET // 2) + i * r, r), :] = _shuffled(
                            y[i][h] * scale if scale else y[i][h])

        def attend(pc, g, first, side, side_steps):
            nb = S // 128
            work = [(first + h, i, t, min(t + ch, i + 1))
                    for h in range(hp) for i in reversed(range(nb)) for t in range(0, i + 1, ch)]
            key = [h * nb + i for h in range(hp) for i in reversed(range(nb)) for t in range(0, i + 1, ch)]
            s, mx, m, l, o, done, ready, due = {}, {}, {}, {}, {}, {}, [], []

            def scores(b, h, i, t0, t1):
                x = pc.note(jax.lax.dot_general(_b16(ctx[HB + h, i * TILE:(i + 1) * TILE, :]),
                                                _b16(ks[h, t0 * TILE:t1 * TILE, :]), NT,
                                                preferred_element_type=F32))
                if t1 == i + 1:
                    row, col = (jax.lax.broadcasted_iota(jnp.int32, (128, 128), d) for d in range(2))
                    row, col = ((u & ~15) | ((u >> 2) & 3) | ((u & 3) << 2) for u in (row, col))
                    diag = jnp.where(col <= row, x[:, -128:], NEG)
                    x = jnp.concatenate([x[:, :-128], diag], axis=1) if t1 - t0 > 1 else diag
                s[b, t0] = x
                mx[b] = jnp.maximum(mx[b], _fold(jnp.maximum, x)) if t0 else _fold(jnp.maximum, x)
                if t1 == i + 1:
                    m[b] = jnp.max(mx[b], axis=1, keepdims=True)

            def values(b, h, i, t0, t1):
                p = jnp.exp2(s.pop((b, t0)) - m[b])
                y = pc.note(jnp.dot(p.astype(BF16), _b16(vs[h, t0 * TILE:t1 * TILE, :]),
                                    preferred_element_type=F32))
                parts = ([l[b]] if t0 else []) + [p[:, c:c + 128] for c in range(0, p.shape[1], 128)]
                l[b] = functools.reduce(jnp.add, [pc.tied(parts[0], pc.recent[-1 - sa])] + parts[1:])
                o[b] = o[b] + y if t0 else y
                if t1 == i + 1:
                    ready.append((h, i, _shuffled(o[b] * _recip(jnp.sum(l[b], axis=1, keepdims=True)))))

            def products():
                clock = qi = pi = turn = 0
                while pi < len(work):
                    can = key[pi] in done and clock - done[key[pi]] >= lag
                    if qi < len(work) and (not can or turn == 0):
                        scores(key[qi], *work[qi])
                        clock += work[qi][3] - work[qi][2]
                        if work[qi][3] == work[qi][1] + 1:
                            done[key[qi]] = clock
                        qi, turn = qi + 1, 1
                    else:
                        values(key[pi], *work[pi])
                        clock += work[pi][3] - work[pi][2]
                        if len(due) < len(ready):
                            due.append(clock + pin)
                        pi, turn = pi + 1, 0
                    while due and (due[0] <= clock or pi == len(work)):
                        due.pop(0)
                        h, i, x = ready.pop(0)
                        ctx[g * GH + h, i * TILE:(i + 1) * TILE, :] = x
                    yield

            main = products()
            _drain(_woven(main, 2 * len(work) - 16, side, side_steps, agea))
            _drain(main)

        for cp in cp_w(0) + cp_rows(0) + cp_rows(1):
            cp.start()
        start_slabs(jnp.int32(0))
        for cp in cp_w(0):
            cp.wait()
        jax.lax.fori_loop(0, GH, lambda j, _: _drain(prep_w(pace(j, 1), 0, j)), None)

        def group(g, _):
            def rows(jj, _):
                @pl.when(g == 0)
                def _():
                    for j in [jj * sp + i for i in range(sp)]:
                        @pl.when(j + 2 < GH)
                        def _():
                            for cp in cp_rows(j + 2):
                                cp.start()
                        for cp in cp_rows(j):
                            cp.wait()

                        @pl.when(j == GH - 1)
                        def _():
                            for cp in cp_w(1):
                                cp.start()

                        def first_rows(a, _):
                            _drain(prep_rows(None, 0, cc, j, a * 8))
                            _drain(prep_rows(None, 4, xc, j, a * 8))
                        jax.lax.fori_loop(0, SET // 64, first_rows, None)


                i = g * (GH // sp) + jj

                @pl.when(i + 1 < HB // sp)
                def _():
                    start_slabs(i + 1)
                wait_slabs(i)
                pc = pace(g, agep)
                for n in range(sp):
                    j = jj * sp + n
                    u = g * GH + j
                    side = _chain(_woven(prep_wo(pc, u, 16 * n), 28, permute_wa(pc, u, 16 * n), 8), prep_wa(pc, u))
                    main = project(pc, j)
                    _drain(_woven(main, 3 * NP - tailp, side, 56, 0 if pc.recent else agex))
                    _drain(main)
            @pl.when((g > 0) & (g + 1 < NG))
            def _():
                for cp in cp_w(g + 1):
                    cp.start()
            if "j" in ph:
                jax.lax.fori_loop(0, GH // sp, rows, None)

            @pl.when(g + 1 < NG)
            def _():
                for cp in cp_w(g + 1):
                    cp.wait()

            def attention(hh, _):
                pc = pace(g, agea)
                nxt = jnp.minimum(g + 1, NG - 1)
                attend(pc, g, hh * hp, _chain(*[prep_w(pc, nxt, hh * hp + i) for i in range(hp)]), 56 * hp)
            if "a" in ph:
                jax.lax.fori_loop(0, GH // hp, attention, None)
            else:
                ctx[0, 0:8, :] = ks[0, 0:8, :] | vs[0, 0:8, :]

        jax.lax.fori_loop(0, NG, group, None)

    heads()

    def rows_phase():
        def cp_xa(t):
            return pltpu.make_async_copy(xa32.at[_rows(jnp.minimum(t, S // RO - 1) * (RO // 2), RO // 2), :],
                                         xa_raw.at[t % 3], sem_xa.at[t % 3])

        def cp_out(t, part):
            at = (_rows(t * RO, RO), pl.ds(part * DM, DM))
            return pltpu.make_async_copy(stage.at[at], out_hbm.at[at], sem_out.at[part, t])

        def prep_ctx(pc, t, i):
            for a in range(0, RA, 8):
                for p in range(NG):
                    z = zero(t, i)
                    x = pc.blocks(lambda b, k: ctx[p * GH + k + z, _rows(t * (RO // 2) + b * RA + a, 8), :])
                    for n, y in _seven(_lhs_term, [[_b16(w).astype(F32) for w in row] for row in x], i):
                        xc[n, _rows(p // 2 * RA + a, 8), _rows(p % 2 * 128, 128)] = _shuffled(y)
                    yield

        def prep_xa(pc, t, i):
            for a in range(0, RA, 8):
                for c in range(2):
                    slot = t % 3 + zero(t, i)
                    x = pc.blocks(lambda b, k: xa_raw[slot, b * RA + a:b * RA + a + 8, (2 * k + c) * 128:(2 * k + c + 1) * 128])
                    for n, y in _seven(_lhs_term, [[_halves(w) for w in row] for row in x], i):
                        xc[n, pl.ds(4 * RA + a, 8), c * 128:(c + 1) * 128] = _words(y)
                    yield

        def window_weights(pc, t):
            lane = jax.lax.broadcasted_iota(jnp.int32, (sm, 128), 1)

            def softmax(a):
                tie = pc.after()
                logits = []
                for w in range(WIN):
                    x = jnp.concatenate([tie(pa[w + zero(t, 1), b:b + 8, :]) for b in range(a, a + sm, 8)], axis=0)
                    for bit in (16, 1):
                        x = x + jnp.where((lane & bit) != 0, pltpu.roll(x, bit, 1), pltpu.roll(x, 128 - bit, 1))
                    if a < DIL * w:
                        pos = jax.lax.broadcasted_iota(jnp.int32, (sm, 128), 0) + (t * RO + a)
                        x = jnp.where(pos >= DIL * w, x, NEG)
                    logits.append(x)
                top = functools.reduce(jnp.maximum, logits)
                es = [jnp.exp2(x - top) for x in logits]
                inv = _recip(functools.reduce(jnp.add, es))
                for w, e in enumerate(es):
                    pa[w, a:a + sm, :] = e * inv

            for a in range(0, RO, 8):
                for w in range(WIN):
                    if w % lw == 0:
                        tie = pc.after()
                        q = [tie(qa[j, a:a + 8, :]) for j in range(8)]
                    b = a + HALO - DIL * w
                    x = q[0] * ka[0, b:b + 8, :]
                    for j in range(1, 8):
                        x = x + q[j] * ka[j, b:b + 8, :]
                    pa[w, a:a + 8, :] = x
                    if w % lw == lw - 1:
                        yield
                if (a + 8) % sm == 0:
                    softmax(a + 8 - sm)
                    yield
            ka[:, 0:HALO, :] = ka[:, RO:, :]

        def window_mix(pc, t):
            for a in range(0, RO, 8):
                for j in range(8):
                    if j % lj == 0:
                        tie = pc.after()
                        ps = [tie(pa[w + zero(t, 0), a:a + 8, :]) for w in range(WIN)]
                    acc = ps[0] * va[j, a + HALO:a + HALO + 8, :]
                    for w in range(1, WIN):
                        b = a + HALO - DIL * w
                        acc = acc + ps[w] * va[j, b:b + 8, :]
                    ya[j, a:a + 8, :] = acc
                    if j % lj == lj - 1:
                        yield
            va[:, 0:HALO, :] = va[:, RO:, :]
            for i in range(7):
                for a in range(0, RA, 8):
                    for c in range(2):
                        z = zero(t, i)
                        x = [pc.blocks(lambda b, k: ya[2 * k + c + z, pl.ds(2 * (b * RA + a) + e, 8, stride=2), :])
                             for e in range(2)]
                        x = [[jnp.concatenate(w, axis=0) for w in zip(*rows)] for rows in zip(*x)]
                        for n, y in _seven(_lhs_term, x, i):
                            xc[n, pl.ds(5 * RA + a, 8), c * 128:(c + 1) * 128] = _words(y)
                        yield

        def joined(c):
            return jnp.concatenate([jnp.concatenate(row, axis=1) for row in c], axis=0)

        steps = S // RO
        cp_xa(0).start()
        cp_xa(1).start()
        ka[:, 0:HALO, :] = jnp.zeros((8, HALO, 128), F32)
        va[:, 0:HALO, :] = jnp.zeros((8, HALO, 128), F32)

        cp_xa(0).wait()
        if "p" in ph:
            for i in range(7):
                _drain(prep_xa(pace(0, 1), 0, i))

        def step(t, _):
            pc = pace(t, ager)

            cp_xa(t + 2).start()
            cp_xa(t + 1).wait()

            def times(first, w):
                def run(n):
                    y = None
                    for k in range(w.shape[1] // 128):
                        z = pc.note(_dot(xc[n, pl.ds((first + k) * RA, RA), :], w[n, k * 128:(k + 1) * 128, :]))
                        y = z if y is None else y + z
                        yield
                    return y
                return _combine(run)

            b = times(0, wo)

            def products():
                y = joined((yield from times(4, wa.at[1])))
                for j in range(8):
                    ka[j, HALO:, :] = y[:, j * 128:(j + 1) * 128]
                y = joined((yield from times(4, wa.at[0]))) * (DA ** -0.5 * LOG2E)
                for j in range(8):
                    qa[j] = y[:, j * 128:(j + 1) * 128]
                v = times(4, wa.at[2])
                for i in range(7):
                    yield from _woven(v, 7, prep_xa(pc, t + 1, i - 1) if i else iter(()), 8 if i else 0)
                y = joined(_drain(v))
                for j in range(8):
                    va[j, HALO:, :] = y[:, j * 128:(j + 1) * 128]
                yield from _woven(b, 28, prep_xa(pc, t + 1, 6), 8)
                return (yield from b)

            rest = products()
            _drain(_woven(rest, n0, _chain(*[prep_ctx(pc, t, i) for i in range(7)]), 224, ager))
            _drain(_woven(rest, n1, window_weights(pc, t), 32 * (WIN // lw) + RO // sm))
            _drain(_woven(rest, 7 * NP - n0 - n1 - n2, window_mix(pc, t), 32 * (8 // lj) + 56))
            stage[_rows(t * RO, RO), DM:] = joined(_drain(rest)).astype(BF16)
            if early:
                cp_out(t, 1).start()
            stage[_rows(t * RO, RO), 0:DM] = joined(_drain(times(5, wa.at[3]))).astype(BF16)
            if not early:
                cp_out(t, 1).start()
            cp_out(t, 0).start()

        if "r" in ph:
            jax.lax.fori_loop(0, steps, step, None)
        else:
            stage[0:16, 0:128] = _b16(ctx[0, 0:8, :] | wo[0, 0:8, 0:128] | wa[0, 0, 0:8, 0:128])
        cp_xa(steps + 1).wait()
        for t in range(steps):
            cp_out(t, 1).wait()
            cp_out(t, 0).wait()

    rows_phase()


def build(pred=8, **cfg):
    flags = {"XLA_TPU_MAX_INSTS_TO_PREDICATE": pred} if pred is not None else None
    vm, dma = pltpu.VMEM, pltpu.SemaphoreType.DMA
    scratch = [
        vm((HB + GH, S // 2, DB), U32),
        vm((NP, HB * DB // 8, DM // 4), U32), vm((4, NP, DM // 8, DM // 4), U32),
        vm((2, 4, 16 * cfg["sp"], DM), U32), vm((2, 4, 16 * cfg["sp"], DM), U32),
        vm((NP, S // 8, DM // 4), U32), vm((NP, S // 8, DC // 4), U32), vm((NP + 8, 4 * TILE, DB), U32),
        vm((2, 2, DM, DB), U32), vm((2, 2, 2, DC, DB), U32),
        vm((GH, S // 2, DB), U32), vm((GH, S // 2, DB), U32),
        vm((8, RO, 128), F32), vm((8, HALO + RO, 128), F32), vm((8, HALO + RO, 128), F32),
        vm((8, RO, 128), F32), vm((WIN, RO, 128), F32),
        vm((3, RO // 2, DM), U32), vm((S, 2 * DM), BF16),
        dma((2,)), dma((2,)), dma((2, 3, 2)), dma((GH,)), dma((3,)), dma((2, S // RO)),
    ]

    @jax.jit
    def run(A_x, A_wqkv, A_wo, B_x, B_c_kv, B_w_q, B_w_uk, B_w_uv, B_w_o):
        out = pl.pallas_call(
            functools.partial(_kernel, **cfg),
            out_shape=jax.ShapeDtypeStruct((S, 2 * DM), BF16),
            in_specs=[pl.BlockSpec(memory_space=pl.ANY)] * 9,
            out_specs=pl.BlockSpec(memory_space=pl.ANY),
            scratch_shapes=scratch,
            compiler_params=pltpu.CompilerParams(vmem_limit_bytes=128 * 2**20, flags=flags),
            name="fused",
        )(A_x.reshape(S, DM), A_wqkv, A_wo.reshape(8, DM // 8, DM),
          B_x.reshape(S, DM), B_c_kv.reshape(S, DC), B_w_q, B_w_uk, B_w_uv, B_w_o)
        return out.reshape(1, S, 2 * DM)

    return run


@jax.jit
def pallas_concat_heads__sliding_local_dilated__compressed_kv_cla__prompt_kernel(
    A_x: jax.Array,
    A_wqkv: jax.Array,
    A_wo: jax.Array,
    B_x: jax.Array,
    B_c_kv: jax.Array,
    B_w_q: jax.Array,
    B_w_uk: jax.Array,
    B_w_uv: jax.Array,
    B_w_o: jax.Array,
):
    return build(**CFG)(A_x, A_wqkv, A_wo, B_x, B_c_kv, B_w_q, B_w_uk, B_w_uv, B_w_o)
```

```python
import functools
import math

import jax
import jax.numpy as jnp
from jax.experimental import pallas as pl
from jax.experimental.pallas import tpu as pltpu

S = 2048
DM = 1024
HA, DA = 32, 32
WIN, DIL = 8, 2
HB, DB = 32, 128
DC = 512
NEG = -1e9
LOG2E = math.log2(math.e)

GH = 4
NG = HB // GH
SET = S // GH
RO = 256
HALO = 16
NP = 49
TILE = 64

F32, BF16, U32 = jnp.float32, jnp.bfloat16, jnp.uint32
NT = (((1,), (1,)), ((), ()))

CFG = dict(ph="pjar", ch=4, lag=12, n0=150, early=1, agep=8, agea=3, ager=8, lw=2, lj=2, sa=3, n1=110, n2=6, sm=16,
           hp=2, sp=2, pin=16, agex=14, order='vqk', tailp=18)

RA = RO // 8


def _b16(x32):
    return pltpu.bitcast(x32, BF16)


def _f32(x32):
    return _b16(x32).astype(F32)


def _wide(load, tiles):
    return jnp.concatenate([load(t) for t in range(tiles)], axis=1) if tiles > 1 else load(0)


def _dot(a32, b32):
    return jnp.dot(_b16(a32), _b16(b32), preferred_element_type=F32)


def _recip(x):
    r = pl.reciprocal(x, approx=True)
    return r * (2.0 - x * r)


def _rows(start, size, align=None):
    return pl.ds(start if isinstance(start, int) else pl.multiple_of(start, align or size), size)


def _fold(f, x):
    return functools.reduce(f, [x[:, c:c + 128] for c in range(0, x.shape[1], 128)])


def _quads(x):
    n = len(x) // 2
    return ([r[:n] for r in x[:n]], [r[n:] for r in x[:n]],
            [r[:n] for r in x[n:]], [r[n:] for r in x[n:]])


def _add(x, y):
    return [[a + b for a, b in zip(r, s)] for r, s in zip(x, y)]


def _sub(x, y):
    return [[a - b for a, b in zip(r, s)] for r, s in zip(x, y)]


def _lhs_term(x, i):
    a11, a12, a21, a22 = _quads(x)
    return (lambda: a11, lambda: _add(a11, a12), lambda: _add(a21, a22), lambda: a22,
            lambda: _add(a11, a22), lambda: _sub(a12, a22), lambda: _sub(a21, a11))[i]()


def _rhs_term(x, i):
    b11, b12, b21, b22 = _quads(x)
    return (lambda: _sub(b12, b22), lambda: b22, lambda: b11, lambda: _sub(b21, b11),
            lambda: _add(b11, b22), lambda: _add(b21, b22), lambda: _add(b11, b12))[i]()


def _seven(term, x, i):
    y = term(x, i)
    return [(7 * i + j, term(y, j)[0][0]) for j in range(7)]


def _combine(product, level=2, base=0):
    if level == 0:
        return [[(yield from product(base))]]
    k = 7 ** (level - 1)
    m3 = yield from _combine(product, level - 1, base)
    m5 = yield from _combine(product, level - 1, base + k)
    c12 = _add(m3, m5)
    m2 = yield from _combine(product, level - 1, base + 2 * k)
    c22 = _sub(m3, m2)
    m4 = yield from _combine(product, level - 1, base + 3 * k)
    c21 = _add(m2, m4)
    c11 = _sub(m4, m5)
    m1 = yield from _combine(product, level - 1, base + 4 * k)
    c11 = _add(c11, m1)
    c22 = _add(c22, m1)
    c11 = _add(c11, (yield from _combine(product, level - 1, base + 5 * k)))
    c22 = _add(c22, (yield from _combine(product, level - 1, base + 6 * k)))
    return [r + s for r, s in zip(c11, c12)] + [r + s for r, s in zip(c21, c22)]


def _drain(gen):
    while True:
        try:
            next(gen)
        except StopIteration as e:
            return e.value


def _chain(*gens):
    for g in gens:
        yield from g


def _woven(main, count, side, side_count, skip=0):
    done = 0
    for _ in range(skip):
        next(main)
        yield
    count -= skip
    for i in range(count):
        while done < side_count and done * count < (i + 1) * side_count:
            next(side)
            done += 1
        next(main)
        yield
    _drain(side)


class _Pace:
    def __init__(self, zero, age):
        self.zero, self.age, self.recent = zero, age, []

    def note(self, y):
        self.recent.append(y[:, -128:])
        return y

    def after(self, age=None):
        age = age or self.age
        if len(self.recent) < age:
            return lambda x: x
        bits = pltpu.bitcast(self.recent[-age][:8], U32) & self.zero
        return lambda x: pltpu.bitcast(
            pltpu.bitcast(x, U32) | jnp.concatenate([bits] * (x.shape[0] // 8), axis=0), x.dtype)

    def tied(self, x, y):
        zero = jnp.concatenate([self.zero] * (x.shape[0] // 8), axis=0)
        return pltpu.bitcast(pltpu.bitcast(x, U32) | (pltpu.bitcast(y, U32) & zero), x.dtype)

    def blocks(self, load):
        tie = self.after()
        return [[tie(load(i, j)) if i % 2 == 0 and j % 2 == 0 else load(i, j) for j in range(4)]
                for i in range(4)]


def _swap_lane_and_chunk_bits(chunks):
    lane = jax.lax.broadcasted_iota(jnp.int32, chunks[0].shape, 1)
    u = (lane >> 1) & 7
    rolled = [x if c == 0 else pltpu.roll(x, 2 * c, 1) for c, x in enumerate(chunks)]
    xs = [rolled[(-i) % 8] for i in range(8)]
    for t in (1, 2, 4):
        m = (u & t) != 0
        xs = [jnp.where(m, xs[(i - t) % 8], xs[i]) for i in range(8)]
    return [x if j == 0 else pltpu.roll(x, 128 - 2 * j, 1) for j, x in enumerate(xs)]


def _kernel(xa_hbm, wqkv_hbm, woa_hbm, xb_hbm, c_hbm, wq_hbm, wuk_hbm, wuv_hbm, wob_hbm,
            out_hbm,
            ctx, wo, wa, wo_raw, wa_raw, xc, cc, wb, wq_raw, wkv_raw, ks, vs,
            qa, ka, va, ya, pa, xa_raw, stage,
            sem_wo, sem_wa, sem_w, sem_x, sem_xa, sem_out, *,
            ph, ch, lag, n0, early, agep, agea, ager, lw, lj, sa, n1, n2, sm, hp, sp, pin, agex, order, tailp):
    xa32, wqkv32, woa32 = (r.bitcast(U32) for r in (xa_hbm, wqkv_hbm, woa_hbm))
    wob32 = wob_hbm.bitcast(U32)
    wq32, wk32, wv32 = (r.bitcast(U32) for r in (wq_hbm, wuk_hbm, wuv_hbm))

    ctx32, wo32, wa32, xc32, cc32, wb32, ks32, vs32 = (
        r.bitcast(U32) for r in (ctx, wo, wa, xc, cc, wb, ks, vs))

    def pace(step, age):
        return _Pace(jnp.full((8, 128), step // S, jnp.int32).astype(U32), age)

    def zero(step, salt):
        return step // (S + salt)

    def start_slabs(i):
        u, n = i * sp, 16 * sp
        for k in range(4):
            pltpu.make_async_copy(wob32.at[u // GH * GH + k, _rows(u % GH * 16, n), :],
                                  wo_raw.at[i % 2, k], sem_wo.at[i % 2]).start()

        @pl.when(u < 24)
        def _():
            for k in range(4):
                pltpu.make_async_copy(wqkv32.at[_rows(k * 128 + u % 8 * 16, n), _rows(u // 8 * DM, DM)],
                                      wa_raw.at[i % 2, k], sem_wa.at[i % 2]).start()

        @pl.when(u >= 24)
        def _():
            for k in range(4):
                for e in range(n // 8):
                    m = k * 16 + u % 8 * 2 + e
                    pltpu.make_async_copy(woa32.at[:, ((m >> 1) & 3) * 16 + (m & 1) * 8 + (m >> 3), :],
                                          wa_raw.at[i % 2, k, pl.ds(8 * e, 8), :], sem_wa.at[i % 2]).start()

    def wait_slabs(i):
        for raw, sem in ((wo_raw, sem_wo), (wa_raw, sem_wa)):
            pltpu.make_async_copy(raw.at[i % 2], raw.at[i % 2], sem.at[i % 2]).wait()

    def cp_xa(t):
        return pltpu.make_async_copy(xa32.at[_rows(jnp.minimum(t, S // RO - 1) * (RO // 2), RO // 2), :],
                                     xa_raw.at[t % 3], sem_xa.at[t % 3])

    def prep_slabs(pc, u, load, store):
        for half in range(2):
            for c in range(2):
                for i in range(7):
                    z = zero(u, i)
                    x = pc.blocks(lambda k, j: load(z, k, half * 8, 2 * j + c))
                    for n, y in _seven(_rhs_term, [[_f32(w) for w in r] for r in x], i):
                        store(n, half * 16, c, y.astype(BF16))
                    yield

    def prep_wo(pc, u, at):
        def store(n, row, c, y):
            wo[n, c, _rows(u * 32 + row, 16), :] = y
        return prep_slabs(
            pc, u, lambda z, k, row, c: wo_raw[u // sp % 2 + z, k, pl.ds(at + row, 8), c * 128:(c + 1) * 128], store)

    def permute_wa(pc, u, at):
        for i in range(4):
            for half in range(2):
                tie = pc.after(agex)
                raw = [tie(wa_raw[u // sp % 2, i, pl.ds(at + half * 8, 8), c * 128:(c + 1) * 128])
                       for c in range(8)]
                for c, y in enumerate(_swap_lane_and_chunk_bits(raw)):
                    wb32[NP + c, pl.ds(i * 16 + half * 8, 8), :] = jnp.where(u < 24, y, raw[c])
                yield

    def prep_wa(pc, u):
        def store(n, row, c, y):
            wa[u // 8 * NP + n, c, _rows(u % 8 * 32 + row, 16), :] = y
        return prep_slabs(pc, u, lambda z, k, row, c: wb32[NP + c + z, k * 16 + row:k * 16 + row + 8, :], store)

    def heads():
        def cp_w(g):
            return [pltpu.make_async_copy(src.at[:, 2 * g + i, :], dst.at[i], sem_w.at[g % 2, kind, i])
                    for kind, (src, dst) in enumerate(((wk32, wkv_raw.at[g % 2, 0]), (wv32, wkv_raw.at[g % 2, 1]),
                                                       (wq32, wq_raw.at[g % 2])))
                    for i in range(2)]

        def cp_rows(j):
            r = _rows(j * SET, SET)
            return [pltpu.make_async_copy(src.at[r, t * 128:(t + 1) * 128], ctx.at[page + t, r, :], sem_x.at[j])
                    for page, src in ((0, c_hbm), (4, xb_hbm)) for t in range(src.shape[1] // 128)]

        def prep_rows(pc, page, dst, j, a):
            r, tiles = SET // 8, dst.shape[1]
            for t in range(tiles):
                x = [[_f32(ctx32[page + k * tiles + t, _rows(j * (SET // 2) + b * r + a, 8), :])
                      for k in range(4)] for b in range(4)]
                for i in range(7):
                    for n, y in _seven(_lhs_term, x, i):
                        dst[n, t, _rows(2 * (j * r + a), 16), :] = y.astype(BF16)
                    yield

        def prep_w(pc, g, j):
            def unit(raw, depth, a, row):
                for i in range(7):
                    if pc or i == 0:
                        tie, z = (pc.after(), zero(j, i)) if pc else (lambda w: w, 0)
                        x = []
                        for k in range(4):
                            words = [raw[pair + z, _rows(k * (depth // 4) + j * (depth // 16) + a, 16), :]
                                     for pair in range(2)]
                            words = [tie(w) for w in words] if k % 2 == 0 else words
                            x.append([pltpu.bitcast(h, F32) for w in words
                                      for h in (w << 16, w & jnp.uint32(0xFFFF0000))])
                    for n, y in _seven(_rhs_term, x, i):
                        wb[n, _rows(2 * row, 16), :] = y.astype(BF16)
                    yield

            for a in range(0, DM // 16, 16):
                yield from unit(wq_raw.at[g % 2], DM, a, j * (DM // 32) + a // 2)
            for kind in range(2):
                for a in range(0, DC // 16, 16):
                    yield from unit(wkv_raw.at[g % 2, kind], DC, a, (2 + kind) * TILE + j * (DC // 32) + a // 2)

        def project(pc, j):
            r = SET // 8
            rows = _rows(j * r, r)

            def product(lhs, first, last):
                def run(n):
                    y = pc.note(_dot(_wide(lambda t: lhs[n, t, rows, :], last - first), wb32[n + zero(j, 0), first * TILE:last * TILE, :]))
                    yield
                    return y
                return _combine(run)

            parts = dict(q=(ctx, HB, DB ** -0.5 * LOG2E, product(xc32, 0, 2)),
                         k=(ks, 0, None, product(cc32, 2, 3)), v=(vs, 0, None, product(cc32, 3, 4)))
            for dst, page, scale, gen in (parts[c] for c in order):
                y = yield from gen
                for i in range(4):
                    for h in range(GH):
                        dst[page + h, _rows(j * SET + i * 2 * r, 2 * r), :] = (
                            y[i][h] * scale if scale else y[i][h]).astype(BF16)

        def attend(pc, g, first, side, side_steps):
            nb = S // 128
            work = [(first + h, i, t, min(t + ch, i + 1))
                    for h in range(hp) for i in reversed(range(nb)) for t in range(0, i + 1, ch)]
            key = [h * nb + i for h in range(hp) for i in reversed(range(nb)) for t in range(0, i + 1, ch)]
            s, mx, m, l, o, done, ready, due = {}, {}, {}, {}, {}, {}, [], []

            def scores(b, h, i, t0, t1):
                x = pc.note(jax.lax.dot_general(_b16(ctx32[HB + h, i * TILE:(i + 1) * TILE, :]),
                                                _b16(ks32[h, t0 * TILE:t1 * TILE, :]), NT,
                                                preferred_element_type=F32))
                if t1 == i + 1:
                    row, col = (jax.lax.broadcasted_iota(jnp.int32, (128, 128), d) for d in range(2))
                    diag = jnp.where(col <= row, x[:, -128:], NEG)
                    x = jnp.concatenate([x[:, :-128], diag], axis=1) if t1 - t0 > 1 else diag
                s[b, t0] = x
                mx[b] = jnp.maximum(mx[b], _fold(jnp.maximum, x)) if t0 else _fold(jnp.maximum, x)
                if t1 == i + 1:
                    m[b] = jnp.max(mx[b], axis=1, keepdims=True)

            def values(b, h, i, t0, t1):
                p = jnp.exp2(s.pop((b, t0)) - m[b])
                y = pc.note(jnp.dot(p.astype(BF16), _b16(vs32[h, t0 * TILE:t1 * TILE, :]),
                                    preferred_element_type=F32))
                parts = ([l[b]] if t0 else []) + [p[:, c:c + 128] for c in range(0, p.shape[1], 128)]
                l[b] = functools.reduce(jnp.add, [pc.tied(parts[0], pc.recent[-1 - sa])] + parts[1:])
                o[b] = o[b] + y if t0 else y
                if t1 == i + 1:
                    ready.append((h, i, (o[b] * _recip(jnp.sum(l[b], axis=1, keepdims=True))).astype(BF16)))

            def products():
                clock = qi = pi = turn = 0
                while pi < len(work):
                    can = key[pi] in done and clock - done[key[pi]] >= lag
                    if qi < len(work) and (not can or turn == 0):
                        scores(key[qi], *work[qi])
                        clock += work[qi][3] - work[qi][2]
                        if work[qi][3] == work[qi][1] + 1:
                            done[key[qi]] = clock
                        qi, turn = qi + 1, 1
                    else:
                        values(key[pi], *work[pi])
                        clock += work[pi][3] - work[pi][2]
                        if len(due) < len(ready):
                            due.append(clock + pin)
                        pi, turn = pi + 1, 0
                    while due and (due[0] <= clock or pi == len(work)):
                        due.pop(0)
                        h, i, x = ready.pop(0)
                        ctx[g * GH + h, i * 128:(i + 1) * 128, :] = x
                    yield

            main = products()
            _drain(_woven(main, 2 * len(work) - 16, side, side_steps, agea))
            _drain(main)

        for cp in cp_w(0) + cp_rows(0) + cp_rows(1):
            cp.start()
        start_slabs(jnp.int32(0))
        for cp in cp_w(0):
            cp.wait()
        jax.lax.fori_loop(0, GH, lambda j, _: _drain(prep_w(None, 0, j)), None)

        def group(g, _):
            def rows(jj, _):
                @pl.when(g == 0)
                def _():
                    for j in [jj * sp + i for i in range(sp)]:
                        @pl.when(j + 2 < GH)
                        def _():
                            for cp in cp_rows(j + 2):
                                cp.start()
                        for cp in cp_rows(j):
                            cp.wait()

                        @pl.when(j == GH - 1)
                        def _():
                            for cp in cp_w(1):
                                cp.start()

                        def first_rows(a, _):
                            _drain(prep_rows(None, 0, cc, j, a * 8))
                            _drain(prep_rows(None, 4, xc, j, a * 8))
                        jax.lax.fori_loop(0, SET // 64, first_rows, None)


                i = g * (GH // sp) + jj

                @pl.when(i + 1 < HB // sp)
                def _():
                    start_slabs(i + 1)
                wait_slabs(i)
                pc = pace(g, agep)
                for n in range(sp):
                    j = jj * sp + n
                    u = g * GH + j
                    side = _chain(_woven(prep_wo(pc, u, 16 * n), 28, permute_wa(pc, u, 16 * n), 8), prep_wa(pc, u))
                    main = project(pc, j)
                    _drain(_woven(main, 3 * NP - tailp, side, 56, 0 if pc.recent else agex))
                    _drain(main)
            @pl.when((g > 0) & (g + 1 < NG))
            def _():
                for cp in cp_w(g + 1):
                    cp.start()

            @pl.when(g == NG - 1)
            def _():
                cp_xa(0).start()
                cp_xa(1).start()
            if "j" in ph:
                jax.lax.fori_loop(0, GH // sp, rows, None)

            @pl.when(g + 1 < NG)
            def _():
                for cp in cp_w(g + 1):
                    cp.wait()

            def attention(hh, _):
                pc = pace(g, agea)
                nxt = jnp.minimum(g + 1, NG - 1)
                attend(pc, g, hh * hp, _chain(*[prep_w(pc, nxt, hh * hp + i) for i in range(hp)]), 56 * hp)
            if "a" in ph:
                jax.lax.fori_loop(0, GH // hp, attention, None)
            else:
                ctx32[0, 0:8, :] = ks32[0, 0:8, :] | vs32[0, 0:8, :]

        jax.lax.fori_loop(0, NG, group, None)

    heads()

    def rows_phase():
        def cp_out(t, part):
            at = (_rows(t * RO, RO), pl.ds(part * DM, DM))
            return pltpu.make_async_copy(stage.at[at], out_hbm.at[at], sem_out.at[part, t])

        def prep_ctx(pc, t, i):
            for a in range(0, RA, 8):
                for p in range(NG):
                    z = zero(t, i)
                    x = pc.blocks(lambda b, k: ctx32[p * GH + k + z, _rows(t * (RO // 2) + b * RA + a, 8), :])
                    for n, y in _seven(_lhs_term, [[_f32(w) for w in row] for row in x], i):
                        xc[n, p % 2, pl.ds(2 * (p // 2 * RA + a), 16), :] = y.astype(BF16)
                    yield

        def prep_xa(pc, t, i):
            for a in range(0, RA, 8):
                for c in range(2):
                    slot = t % 3 + zero(t, i)
                    x = pc.blocks(lambda b, k: xa_raw[slot, b * RA + a:b * RA + a + 8, (2 * k + c) * 128:(2 * k + c + 1) * 128])
                    for n, y in _seven(_lhs_term, [[_f32(w) for w in row] for row in x], i):
                        xc[n, c, pl.ds(2 * (4 * RA + a), 16), :] = y.astype(BF16)
                    yield

        def window_weights(pc, t):
            lane = jax.lax.broadcasted_iota(jnp.int32, (sm, 128), 1)

            def softmax(a):
                tie = pc.after()
                logits = []
                for w in range(WIN):
                    x = jnp.concatenate([tie(pa[w + zero(t, 1), b:b + 8, :]) for b in range(a, a + sm, 8)], axis=0)
                    for bit in (16, 1):
                        x = x + jnp.where((lane & bit) != 0, pltpu.roll(x, bit, 1), pltpu.roll(x, 128 - bit, 1))
                    if a < DIL * w:
                        pos = jax.lax.broadcasted_iota(jnp.int32, (sm, 128), 0) + (t * RO + a)
                        x = jnp.where(pos >= DIL * w, x, NEG)
                    logits.append(x)
                top = functools.reduce(jnp.maximum, logits)
                es = [jnp.exp2(x - top) for x in logits]
                inv = _recip(functools.reduce(jnp.add, es))
                for w, e in enumerate(es):
                    pa[w, a:a + sm, :] = e * inv

            for a in range(0, RO, 8):
                for w in range(WIN):
                    if w % lw == 0:
                        tie = pc.after()
                        q = [tie(qa[j, a:a + 8, :]) for j in range(8)]
                    b = a + HALO - DIL * w
                    x = q[0] * ka[0, b:b + 8, :]
                    for j in range(1, 8):
                        x = x + q[j] * ka[j, b:b + 8, :]
                    pa[w, a:a + 8, :] = x
                    if w % lw == lw - 1:
                        yield
                if (a + 8) % sm == 0:
                    softmax(a + 8 - sm)
                    yield
            ka[:, 0:HALO, :] = ka[:, RO:, :]

        def window_mix(pc, t):
            for a in range(0, RO, 8):
                for j in range(8):
                    if j % lj == 0:
                        tie = pc.after()
                        ps = [tie(pa[w + zero(t, 0), a:a + 8, :]) for w in range(WIN)]
                    acc = ps[0] * va[j, a + HALO:a + HALO + 8, :]
                    for w in range(1, WIN):
                        b = a + HALO - DIL * w
                        acc = acc + ps[w] * va[j, b:b + 8, :]
                    ya[j, a:a + 8, :] = acc
                    if j % lj == lj - 1:
                        yield
            va[:, 0:HALO, :] = va[:, RO:, :]
            for i in range(7):
                for a in range(0, RA, 8):
                    for c in range(2):
                        z = zero(t, i)
                        x = pc.blocks(lambda b, k: ya[2 * k + c + z, pl.ds(2 * (b * RA + a), 16), :])
                        for n, y in _seven(_lhs_term, x, i):
                            xc[n, c, pl.ds(2 * (5 * RA + a), 16), :] = y.astype(BF16)
                        yield

        def joined(c):
            return jnp.concatenate([jnp.concatenate(row, axis=1) for row in c], axis=0)

        steps = S // RO
        ka[:, 0:HALO, :] = jnp.zeros((8, HALO, 128), F32)
        va[:, 0:HALO, :] = jnp.zeros((8, HALO, 128), F32)

        cp_xa(0).wait()
        if "p" in ph:
            for i in range(7):
                _drain(prep_xa(pace(0, 1), 0, i))

        def step(t, _):
            pc = pace(t, ager)

            cp_xa(t + 2).start()
            cp_xa(t + 1).wait()

            def times(first, w, at):
                def run(n):
                    y = None
                    for k in range(w.shape[2] // 128):
                        z = pc.note(_dot(_wide(lambda c: xc32[n, c, pl.ds((first + k) * RA, RA), :], 2),
                                         _wide(lambda c: w[at + n, c, k * 128:(k + 1) * 128, :], 2)))
                        y = z if y is None else y + z
                        yield
                    return y
                return _combine(run)

            b = times(0, wo32, 0)

            def products():
                y = joined((yield from times(4, wa32, NP)))
                for j in range(8):
                    ka[j, HALO:, :] = y[:, j * 128:(j + 1) * 128]
                y = joined((yield from times(4, wa32, 0))) * (DA ** -0.5 * LOG2E)
                for j in range(8):
                    qa[j] = y[:, j * 128:(j + 1) * 128]
                v = times(4, wa32, 2 * NP)
                for i in range(7):
                    yield from _woven(v, 7, prep_xa(pc, t + 1, i - 1) if i else iter(()), 8 if i else 0)
                y = joined(_drain(v))
                for j in range(8):
                    va[j, HALO:, :] = y[:, j * 128:(j + 1) * 128]
                yield from _woven(b, 28, prep_xa(pc, t + 1, 6), 8)
                return (yield from b)

            rest = products()
            _drain(_woven(rest, n0, _chain(*[prep_ctx(pc, t, i) for i in range(7)]), 224, ager))
            _drain(_woven(rest, n1, window_weights(pc, t), 32 * (WIN // lw) + RO // sm))
            _drain(_woven(rest, 7 * NP - n0 - n1 - n2, window_mix(pc, t), 32 * (8 // lj) + 56))
            stage[_rows(t * RO, RO), DM:] = joined(_drain(rest)).astype(BF16)
            if early:
                cp_out(t, 1).start()
            stage[_rows(t * RO, RO), 0:DM] = joined(_drain(times(5, wa32, 3 * NP))).astype(BF16)
            if not early:
                cp_out(t, 1).start()
            cp_out(t, 0).start()

        if "r" in ph:
            jax.lax.fori_loop(0, steps, step, None)
        else:
            stage[0:16, 0:128] = _b16(ctx32[0, 0:8, :] | wo32[0, 0, 0:8, :] | wa32[0, 0, 0:8, :])
        cp_xa(steps + 1).wait()
        for t in range(steps):
            cp_out(t, 1).wait()
            cp_out(t, 0).wait()

    rows_phase()


def build(pred=8, **cfg):
    flags = {"XLA_TPU_MAX_INSTS_TO_PREDICATE": pred} if pred is not None else None
    vm, dma = pltpu.VMEM, pltpu.SemaphoreType.DMA
    scratch = [
        vm((HB + GH, S, DB), BF16),
        vm((NP, 2, HB * DB // 4, 128), BF16), vm((4 * NP, 2, DM // 4, 128), BF16),
        vm((2, 4, 16 * cfg["sp"], DM), U32), vm((2, 4, 16 * cfg["sp"], DM), U32),
        vm((NP, 2, S // 4, 128), BF16), vm((NP, 1, S // 4, 128), BF16), vm((NP + 8, 4 * 128, DB), BF16),
        vm((2, 2, DM, DB), U32), vm((2, 2, 2, DC, DB), U32),
        vm((GH, S, DB), BF16), vm((GH, S, DB), BF16),
        vm((8, RO, 128), F32), vm((8, HALO + RO, 128), F32), vm((8, HALO + RO, 128), F32),
        vm((8, RO, 128), F32), vm((WIN, RO, 128), F32),
        vm((3, RO // 2, DM), U32), vm((S, 2 * DM), BF16),
        dma((2,)), dma((2,)), dma((2, 3, 2)), dma((GH,)), dma((3,)), dma((2, S // RO)),
    ]

    @jax.jit
    def run(A_x, A_wqkv, A_wo, B_x, B_c_kv, B_w_q, B_w_uk, B_w_uv, B_w_o):
        out = pl.pallas_call(
            functools.partial(_kernel, **cfg),
            out_shape=jax.ShapeDtypeStruct((S, 2 * DM), BF16),
            in_specs=[pl.BlockSpec(memory_space=pl.ANY)] * 9,
            out_specs=pl.BlockSpec(memory_space=pl.ANY),
            scratch_shapes=scratch,
            compiler_params=pltpu.CompilerParams(vmem_limit_bytes=128 * 2**20, flags=flags),
            name="fused",
        )(A_x.reshape(S, DM), A_wqkv, A_wo.reshape(8, DM // 8, DM),
          B_x.reshape(S, DM), B_c_kv.reshape(S, DC), B_w_q, B_w_uk, B_w_uv, B_w_o)
        return out.reshape(1, S, 2 * DM)

    return run


@jax.jit
def pallas_concat_heads__sliding_local_dilated__compressed_kv_cla__prompt_kernel(
    A_x: jax.Array,
    A_wqkv: jax.Array,
    A_wo: jax.Array,
    B_x: jax.Array,
    B_c_kv: jax.Array,
    B_w_q: jax.Array,
    B_w_uk: jax.Array,
    B_w_uv: jax.Array,
    B_w_o: jax.Array,
):
    return build(**CFG)(A_x, A_wqkv, A_wo, B_x, B_c_kv, B_w_q, B_w_uk, B_w_uv, B_w_o)
```

```python
import functools
import math

import jax
import jax.numpy as jnp
from jax.experimental import pallas as pl
from jax.experimental.pallas import tpu as pltpu

S = 2048
DM = 1024
HA, DA = 32, 32
WIN, DIL = 8, 2
HB, DB = 32, 128
DC = 512
NEG = -1e9
LOG2E = math.log2(math.e)

GH = 4
NG = HB // GH
SET = S // GH
RO = 256
HALO = 16
NP = 49
TILE = 64

F32, BF16, U32 = jnp.float32, jnp.bfloat16, jnp.uint32
NT = (((1,), (1,)), ((), ()))

CFG = dict(ph="pjar", ch=4, lag=12, n0=150, early=1, agep=10, agea=3, ager=8, lw=2, lj=2, sa=3, n1=100, n2=20, sm=16,
           hp=2, sp=2, pin=10, agex=15, order='vqk', tailp=4, way='dd', taila=16)

RA = RO // 8


def _b16(x32):
    return pltpu.bitcast(x32, BF16)


def _f32(x32):
    return _b16(x32).astype(F32)


def _wide(load, tiles):
    return jnp.concatenate([load(t) for t in range(tiles)], axis=1) if tiles > 1 else load(0)


def _dot(a32, b32):
    return jnp.dot(_b16(a32), _b16(b32), preferred_element_type=F32)


def _recip(x):
    r = pl.reciprocal(x, approx=True)
    return r * (2.0 - x * r)


def _rows(start, size, align=None):
    return pl.ds(start if isinstance(start, int) else pl.multiple_of(start, align or size), size)


def _fold(f, x):
    return functools.reduce(f, [x[:, c:c + 128] for c in range(0, x.shape[1], 128)])


def _quads(x):
    n = len(x) // 2
    return ([r[:n] for r in x[:n]], [r[n:] for r in x[:n]],
            [r[:n] for r in x[n:]], [r[n:] for r in x[n:]])


def _add(x, y):
    return [[a + b for a, b in zip(r, s)] for r, s in zip(x, y)]


def _sub(x, y):
    return [[a - b for a, b in zip(r, s)] for r, s in zip(x, y)]


def _lhs_term(x, i):
    a11, a12, a21, a22 = _quads(x)
    return (lambda: a11, lambda: _add(a11, a12), lambda: _add(a21, a22), lambda: a22,
            lambda: _add(a11, a22), lambda: _sub(a12, a22), lambda: _sub(a21, a11))[i]()


def _rhs_term(x, i):
    b11, b12, b21, b22 = _quads(x)
    return (lambda: _sub(b12, b22), lambda: b22, lambda: b11, lambda: _sub(b21, b11),
            lambda: _add(b11, b22), lambda: _add(b21, b22), lambda: _add(b11, b12))[i]()


def _seven(term, x, i):
    y = term(x, i)
    return [(7 * i + j, term(y, j)[0][0]) for j in range(7)]


def _combine(product, level=2, base=0):
    if level == 0:
        return [[(yield from product(base))]]
    k = 7 ** (level - 1)
    m3 = yield from _combine(product, level - 1, base)
    m5 = yield from _combine(product, level - 1, base + k)
    c12 = _add(m3, m5)
    m2 = yield from _combine(product, level - 1, base + 2 * k)
    c22 = _sub(m3, m2)
    m4 = yield from _combine(product, level - 1, base + 3 * k)
    c21 = _add(m2, m4)
    c11 = _sub(m4, m5)
    m1 = yield from _combine(product, level - 1, base + 4 * k)
    c11 = _add(c11, m1)
    c22 = _add(c22, m1)
    c11 = _add(c11, (yield from _combine(product, level - 1, base + 5 * k)))
    c22 = _add(c22, (yield from _combine(product, level - 1, base + 6 * k)))
    return [r + s for r, s in zip(c11, c12)] + [r + s for r, s in zip(c21, c22)]


def _drain(gen):
    while True:
        try:
            next(gen)
        except StopIteration as e:
            return e.value


def _chain(*gens):
    for g in gens:
        yield from g


def _woven(main, count, side, side_count, skip=0):
    done = 0
    for _ in range(skip):
        next(main)
        yield
    count -= skip
    for i in range(count):
        while done < side_count and done * count < (i + 1) * side_count:
            next(side)
            done += 1
        next(main)
        yield
    _drain(side)


class _Pace:
    def __init__(self, zero, age):
        self.zero, self.age, self.recent = zero, age, []

    def note(self, y):
        self.recent.append(y[:, -128:])
        return y

    def after(self, age=None):
        age = age or self.age
        if len(self.recent) < age:
            return lambda x: x
        bits = pltpu.bitcast(self.recent[-age][:8], U32) & self.zero
        return lambda x: pltpu.bitcast(
            pltpu.bitcast(x, U32) | jnp.concatenate([bits] * (x.shape[0] // 8), axis=0), x.dtype)

    def tied(self, x, y):
        zero = jnp.concatenate([self.zero] * (x.shape[0] // 8), axis=0)
        return pltpu.bitcast(pltpu.bitcast(x, U32) | (pltpu.bitcast(y, U32) & zero), x.dtype)

    def blocks(self, load):
        tie = self.after()
        return [[tie(load(i, j)) if i % 2 == 0 and j % 2 == 0 else load(i, j) for j in range(4)]
                for i in range(4)]


def _swap_lane_and_chunk_bits(chunks):
    lane = jax.lax.broadcasted_iota(jnp.int32, chunks[0].shape, 1)
    u = (lane >> 1) & 7
    rolled = [x if c == 0 else pltpu.roll(x, 2 * c, 1) for c, x in enumerate(chunks)]
    xs = [rolled[(-i) % 8] for i in range(8)]
    for t in (1, 2, 4):
        m = (u & t) != 0
        xs = [jnp.where(m, xs[(i - t) % 8], xs[i]) for i in range(8)]
    return [x if j == 0 else pltpu.roll(x, 128 - 2 * j, 1) for j, x in enumerate(xs)]


def _kernel(xa_hbm, wqkv_hbm, woa_hbm, xb_hbm, c_hbm, wq_hbm, wuk_hbm, wuv_hbm, wob_hbm,
            out_hbm,
            ctx, wo, wa, wo_raw, wa_raw, xc, cc, wb, wq_raw, wkv_raw, ks, vs,
            qa, ka, va, ya, pa, xa_raw, stage,
            sem_wo, sem_wa, sem_w, sem_x, sem_xa, sem_out, *,
            ph, ch, lag, n0, early, agep, agea, ager, lw, lj, sa, n1, n2, sm, hp, sp, pin, agex, order, tailp, way, taila):
    xa32, wqkv32, woa32 = (r.bitcast(U32) for r in (xa_hbm, wqkv_hbm, woa_hbm))
    wob32 = wob_hbm.bitcast(U32)
    wq32, wk32, wv32 = (r.bitcast(U32) for r in (wq_hbm, wuk_hbm, wuv_hbm))

    ctx32, wo32, wa32, xc32, cc32, wb32, ks32, vs32 = (
        r.bitcast(U32) for r in (ctx, wo, wa, xc, cc, wb, ks, vs))

    def pace(step, age):
        return _Pace(jnp.full((8, 128), step // S, jnp.int32).astype(U32), age)

    def zero(step, salt):
        return step // (S + salt)

    def start_slabs(i):
        u, n = i * sp, 16 * sp
        for k in range(4):
            pltpu.make_async_copy(wob32.at[u // GH * GH + k, _rows(u % GH * 16, n), :],
                                  wo_raw.at[i % 2, k], sem_wo.at[i % 2]).start()

        @pl.when(u < 24)
        def _():
            for k in range(4):
                pltpu.make_async_copy(wqkv32.at[_rows(k * 128 + u % 8 * 16, n), _rows(u // 8 * DM, DM)],
                                      wa_raw.at[i % 2, k], sem_wa.at[i % 2]).start()

        @pl.when(u >= 24)
        def _():
            for k in range(4):
                for e in range(n // 8):
                    m = k * 16 + u % 8 * 2 + e
                    pltpu.make_async_copy(woa32.at[:, ((m >> 1) & 3) * 16 + (m & 1) * 8 + (m >> 3), :],
                                          wa_raw.at[i % 2, k, pl.ds(8 * e, 8), :], sem_wa.at[i % 2]).start()

    def wait_slabs(i):
        for raw, sem in ((wo_raw, sem_wo), (wa_raw, sem_wa)):
            pltpu.make_async_copy(raw.at[i % 2], raw.at[i % 2], sem.at[i % 2]).wait()

    def cp_xa(t):
        return pltpu.make_async_copy(xa32.at[_rows(jnp.minimum(t, S // RO - 1) * (RO // 2), RO // 2), :],
                                     xa_raw.at[t % 3], sem_xa.at[t % 3])

    def prep_slabs(pc, u, load, store):
        for half in range(2):
            for c in range(2):
                for i in range(7):
                    z = zero(u, i)
                    x = pc.blocks(lambda k, j: load(z, k, half * 8, 2 * j + c))
                    for n, y in _seven(_rhs_term, [[_f32(w) for w in r] for r in x], i):
                        store(n, half * 16, c, y.astype(BF16))
                    yield

    def prep_wo(pc, u, at):
        def store(n, row, c, y):
            wo[n, c, _rows(u * 32 + row, 16), :] = y
        return prep_slabs(
            pc, u, lambda z, k, row, c: wo_raw[u // sp % 2 + z, k, pl.ds(at + row, 8), c * 128:(c + 1) * 128], store)

    def permute_wa(pc, u, at):
        for i in range(4):
            for half in range(2):
                tie = pc.after(agex)
                raw = [tie(wa_raw[u // sp % 2, i, pl.ds(at + half * 8, 8), c * 128:(c + 1) * 128])
                       for c in range(8)]
                for c, y in enumerate(_swap_lane_and_chunk_bits(raw)):
                    wb32[NP + c, pl.ds(i * 16 + half * 8, 8), :] = jnp.where(u < 24, y, raw[c])
                yield

    def prep_wa(pc, u):
        def store(n, row, c, y):
            wa[u // 8 * NP + n, c, _rows(u % 8 * 32 + row, 16), :] = y
        return prep_slabs(pc, u, lambda z, k, row, c: wb32[NP + c + z, k * 16 + row:k * 16 + row + 8, :], store)

    def heads():
        def cp_w(g):
            return [pltpu.make_async_copy(src.at[:, 2 * g + i, :], dst.at[i], sem_w.at[g % 2, kind, i])
                    for kind, (src, dst) in enumerate(((wk32, wkv_raw.at[g % 2, 0]), (wv32, wkv_raw.at[g % 2, 1]),
                                                       (wq32, wq_raw.at[g % 2])))
                    for i in range(2)]

        def cp_rows(j):
            r = _rows(j * SET, SET)
            return [pltpu.make_async_copy(src.at[r, t * 128:(t + 1) * 128], ctx.at[page + t, r, :], sem_x.at[j])
                    for page, src in ((0, c_hbm), (4, xb_hbm)) for t in range(src.shape[1] // 128)]

        def prep_rows(pc, page, dst, j, a):
            r, tiles = SET // 8, dst.shape[1]
            for t in range(tiles):
                x = [[_f32(ctx32[page + k * tiles + t, _rows(j * (SET // 2) + b * r + a, 8), :])
                      for k in range(4)] for b in range(4)]
                for i in range(7):
                    for n, y in _seven(_lhs_term, x, i):
                        dst[n, t, _rows(2 * (j * r + a), 16), :] = y.astype(BF16)
                    yield

        def prep_w(pc, g, j):
            def unit(raw, depth, a, row):
                for i in range(7):
                    if pc or i == 0:
                        tie, z = (pc.after(), zero(j, i)) if pc else (lambda w: w, 0)
                        x = []
                        for k in range(4):
                            words = [raw[pair + z, _rows(k * (depth // 4) + j * (depth // 16) + a, 16), :]
                                     for pair in range(2)]
                            words = [tie(w) for w in words] if k % 2 == 0 else words
                            x.append([pltpu.bitcast(h, F32) for w in words
                                      for h in (w << 16, w & jnp.uint32(0xFFFF0000))])
                    for n, y in _seven(_rhs_term, x, i):
                        wb[n, _rows(2 * row, 16), :] = y.astype(BF16)
                    yield

            for a in range(0, DM // 16, 16):
                yield from unit(wq_raw.at[g % 2], DM, a, j * (DM // 32) + a // 2)
            for kind in range(2):
                for a in range(0, DC // 16, 16):
                    yield from unit(wkv_raw.at[g % 2, kind], DC, a, (2 + kind) * TILE + j * (DC // 32) + a // 2)

        def project(pc, j):
            r = SET // 8
            rows = _rows(j * r, r)

            def product(lhs, first, last):
                def run(n):
                    y = pc.note(_dot(_wide(lambda t: lhs[n, t, rows, :], last - first), wb32[n + zero(j, 0), first * TILE:last * TILE, :]))
                    yield
                    return y
                return _combine(run)

            parts = dict(q=(ctx, HB, DB ** -0.5 * LOG2E, product(xc32, 0, 2)),
                         k=(ks, 0, None, product(cc32, 2, 3)), v=(vs, 0, None, product(cc32, 3, 4)))
            for dst, page, scale, gen in (parts[c] for c in order):
                y = yield from gen
                for i in range(4):
                    for h in range(GH):
                        dst[page + h, _rows(j * SET + i * 2 * r, 2 * r), :] = (
                            y[i][h] * scale if scale else y[i][h]).astype(BF16)

        def attend(pc, g, first, side, side_steps):
            nb = S // 128
            ways = dict(d=list(reversed(range(nb))), a=list(range(nb)),
                        z=[i for j in range(nb // 2) for i in (nb - 1 - j, j)],
                        m=[i for j in range(nb // 2) for i in (nb // 2 - 1 - j, nb // 2 + j)],
                        v=list(range(nb - 1, -1, -2)) + list(range(0, nb, 2)))
            blocks = [(h, i) for h in range(hp) for i in ways[way[h]]]
            if way[-1] == "x":
                blocks = [b for pair in zip(blocks[:nb], blocks[nb:]) for b in pair]
            work = [(first + h, i, t, min(t + ch, i + 1)) for h, i in blocks for t in range(0, i + 1, ch)]
            key = [h * nb + i for h, i in blocks for t in range(0, i + 1, ch)]
            s, mx, m, l, o, done, ready, due = {}, {}, {}, {}, {}, {}, [], []

            def scores(b, h, i, t0, t1):
                x = pc.note(jax.lax.dot_general(_b16(ctx32[HB + h, i * TILE:(i + 1) * TILE, :]),
                                                _b16(ks32[h, t0 * TILE:t1 * TILE, :]), NT,
                                                preferred_element_type=F32))
                if t1 == i + 1:
                    row, col = (jax.lax.broadcasted_iota(jnp.int32, (128, 128), d) for d in range(2))
                    diag = jnp.where(col <= row, x[:, -128:], NEG)
                    x = jnp.concatenate([x[:, :-128], diag], axis=1) if t1 - t0 > 1 else diag
                s[b, t0] = x
                mx[b] = jnp.maximum(mx[b], _fold(jnp.maximum, x)) if t0 else _fold(jnp.maximum, x)
                if t1 == i + 1:
                    m[b] = jnp.max(mx[b], axis=1, keepdims=True)

            def values(b, h, i, t0, t1):
                p = jnp.exp2(s.pop((b, t0)) - m[b])
                y = pc.note(jnp.dot(p.astype(BF16), _b16(vs32[h, t0 * TILE:t1 * TILE, :]),
                                    preferred_element_type=F32))
                parts = ([l[b]] if t0 else []) + [p[:, c:c + 128] for c in range(0, p.shape[1], 128)]
                l[b] = functools.reduce(jnp.add, [pc.tied(parts[0], pc.recent[-1 - sa])] + parts[1:])
                o[b] = o[b] + y if t0 else y
                if t1 == i + 1:
                    ready.append((h, i, (o[b] * _recip(jnp.sum(l[b], axis=1, keepdims=True))).astype(BF16)))

            def products():
                clock = qi = pi = turn = 0
                while pi < len(work):
                    can = key[pi] in done and clock - done[key[pi]] >= lag
                    if qi < len(work) and (not can or turn == 0):
                        scores(key[qi], *work[qi])
                        clock += work[qi][3] - work[qi][2]
                        if work[qi][3] == work[qi][1] + 1:
                            done[key[qi]] = clock
                        qi, turn = qi + 1, 1
                    else:
                        values(key[pi], *work[pi])
                        clock += work[pi][3] - work[pi][2]
                        if len(due) < len(ready):
                            due.append(clock + pin)
                        pi, turn = pi + 1, 0
                    while due and (due[0] <= clock or pi == len(work)):
                        due.pop(0)
                        h, i, x = ready.pop(0)
                        ctx[g * GH + h, i * 128:(i + 1) * 128, :] = x
                    yield

            main = products()
            _drain(_woven(main, 2 * len(work) - taila, side, side_steps, agea))
            _drain(main)

        for cp in cp_w(0) + cp_rows(0) + cp_rows(1):
            cp.start()
        start_slabs(jnp.int32(0))
        for cp in cp_w(0):
            cp.wait()
        jax.lax.fori_loop(0, GH, lambda j, _: _drain(prep_w(None, 0, j)), None)

        def group(g, _):
            def rows(jj, _):
                @pl.when(g == 0)
                def _():
                    for j in [jj * sp + i for i in range(sp)]:
                        @pl.when(j + 2 < GH)
                        def _():
                            for cp in cp_rows(j + 2):
                                cp.start()
                        for cp in cp_rows(j):
                            cp.wait()

                        @pl.when(j == GH - 1)
                        def _():
                            for cp in cp_w(1):
                                cp.start()

                        def first_rows(a, _):
                            _drain(prep_rows(None, 0, cc, j, a * 8))
                            _drain(prep_rows(None, 4, xc, j, a * 8))
                        jax.lax.fori_loop(0, SET // 64, first_rows, None)


                i = g * (GH // sp) + jj

                @pl.when(i + 1 < HB // sp)
                def _():
                    start_slabs(i + 1)
                wait_slabs(i)
                pc = pace(g, agep)
                for n in range(sp):
                    j = jj * sp + n
                    u = g * GH + j
                    side = _chain(_woven(prep_wo(pc, u, 16 * n), 28, permute_wa(pc, u, 16 * n), 8), prep_wa(pc, u))
                    main = project(pc, j)
                    _drain(_woven(main, 3 * NP - tailp, side, 56, 0 if pc.recent else agex))
                    _drain(main)
            @pl.when((g > 0) & (g + 1 < NG))
            def _():
                for cp in cp_w(g + 1):
                    cp.start()

            @pl.when(g == NG - 1)
            def _():
                cp_xa(0).start()
                cp_xa(1).start()
            if "j" in ph:
                jax.lax.fori_loop(0, GH // sp, rows, None)

            @pl.when(g + 1 < NG)
            def _():
                for cp in cp_w(g + 1):
                    cp.wait()

            def attention(hh, _):
                pc = pace(g, agea)
                nxt = jnp.minimum(g + 1, NG - 1)
                attend(pc, g, hh * hp, _chain(*[prep_w(pc, nxt, hh * hp + i) for i in range(hp)]), 56 * hp)
            if "a" in ph:
                jax.lax.fori_loop(0, GH // hp, attention, None)
            else:
                ctx32[0, 0:8, :] = ks32[0, 0:8, :] | vs32[0, 0:8, :]

        jax.lax.fori_loop(0, NG, group, None)

    heads()

    def rows_phase():
        def cp_out(t, part):
            at = (_rows(t * RO, RO), pl.ds(part * DM, DM))
            return pltpu.make_async_copy(stage.at[at], out_hbm.at[at], sem_out.at[part, t])

        def prep_ctx(pc, t, i):
            for a in range(0, RA, 8):
                for p in range(NG):
                    z = zero(t, i)
                    x = pc.blocks(lambda b, k: ctx32[p * GH + k + z, _rows(t * (RO // 2) + b * RA + a, 8), :])
                    for n, y in _seven(_lhs_term, [[_f32(w) for w in row] for row in x], i):
                        xc[n, p % 2, pl.ds(2 * (p // 2 * RA + a), 16), :] = y.astype(BF16)
                    yield

        def prep_xa(pc, t, i):
            for a in range(0, RA, 8):
                for c in range(2):
                    slot = t % 3 + zero(t, i)
                    x = pc.blocks(lambda b, k: xa_raw[slot, b * RA + a:b * RA + a + 8, (2 * k + c) * 128:(2 * k + c + 1) * 128])
                    for n, y in _seven(_lhs_term, [[_f32(w) for w in row] for row in x], i):
                        xc[n, c, pl.ds(2 * (4 * RA + a), 16), :] = y.astype(BF16)
                    yield

        def window_weights(pc, t):
            lane = jax.lax.broadcasted_iota(jnp.int32, (sm, 128), 1)

            def softmax(a):
                tie = pc.after()
                logits = []
                for w in range(WIN):
                    x = jnp.concatenate([tie(pa[w + zero(t, 1), b:b + 8, :]) for b in range(a, a + sm, 8)], axis=0)
                    for bit in (16, 1):
                        x = x + jnp.where((lane & bit) != 0, pltpu.roll(x, bit, 1), pltpu.roll(x, 128 - bit, 1))
                    if a < DIL * w:
                        pos = jax.lax.broadcasted_iota(jnp.int32, (sm, 128), 0) + (t * RO + a)
                        x = jnp.where(pos >= DIL * w, x, NEG)
                    logits.append(x)
                top = functools.reduce(jnp.maximum, logits)
                es = [jnp.exp2(x - top) for x in logits]
                inv = _recip(functools.reduce(jnp.add, es))
                for w, e in enumerate(es):
                    pa[w, a:a + sm, :] = e * inv

            for a in range(0, RO, 8):
                for w in range(WIN):
                    if w % lw == 0:
                        tie = pc.after()
                        q = [tie(qa[j, a:a + 8, :]) for j in range(8)]
                    b = a + HALO - DIL * w
                    x = q[0] * ka[0, b:b + 8, :]
                    for j in range(1, 8):
                        x = x + q[j] * ka[j, b:b + 8, :]
                    pa[w, a:a + 8, :] = x
                    if w % lw == lw - 1:
                        yield
                if (a + 8) % sm == 0:
                    softmax(a + 8 - sm)
                    yield
            ka[:, 0:HALO, :] = ka[:, RO:, :]

        def window_mix(pc, t):
            for a in range(0, RO, 8):
                for j in range(8):
                    if j % lj == 0:
                        tie = pc.after()
                        ps = [tie(pa[w + zero(t, 0), a:a + 8, :]) for w in range(WIN)]
                    acc = ps[0] * va[j, a + HALO:a + HALO + 8, :]
                    for w in range(1, WIN):
                        b = a + HALO - DIL * w
                        acc = acc + ps[w] * va[j, b:b + 8, :]
                    ya[j, a:a + 8, :] = acc
                    if j % lj == lj - 1:
                        yield
            va[:, 0:HALO, :] = va[:, RO:, :]
            for i in range(7):
                for a in range(0, RA, 8):
                    for c in range(2):
                        z = zero(t, i)
                        x = pc.blocks(lambda b, k: ya[2 * k + c + z, pl.ds(2 * (b * RA + a), 16), :])
                        for n, y in _seven(_lhs_term, x, i):
                            xc[n, c, pl.ds(2 * (5 * RA + a), 16), :] = y.astype(BF16)
                        yield

        def joined(c):
            return jnp.concatenate([jnp.concatenate(row, axis=1) for row in c], axis=0)

        steps = S // RO
        ka[:, 0:HALO, :] = jnp.zeros((8, HALO, 128), F32)
        va[:, 0:HALO, :] = jnp.zeros((8, HALO, 128), F32)

        cp_xa(0).wait()
        if "p" in ph:
            for i in range(7):
                _drain(prep_xa(pace(0, 1), 0, i))

        def step(t, _):
            pc = pace(t, ager)

            cp_xa(t + 2).start()
            cp_xa(t + 1).wait()

            def times(first, w, at):
                def run(n):
                    y = None
                    for k in range(w.shape[2] // 128):
                        z = pc.note(_dot(_wide(lambda c: xc32[n, c, pl.ds((first + k) * RA, RA), :], 2),
                                         _wide(lambda c: w[at + n, c, k * 128:(k + 1) * 128, :], 2)))
                        y = z if y is None else y + z
                        yield
                    return y
                return _combine(run)

            b = times(0, wo32, 0)

            def products():
                y = joined((yield from times(4, wa32, NP)))
                for j in range(8):
                    ka[j, HALO:, :] = y[:, j * 128:(j + 1) * 128]
                y = joined((yield from times(4, wa32, 0))) * (DA ** -0.5 * LOG2E)
                for j in range(8):
                    qa[j] = y[:, j * 128:(j + 1) * 128]
                v = times(4, wa32, 2 * NP)
                for i in range(7):
                    yield from _woven(v, 7, prep_xa(pc, t + 1, i - 1) if i else iter(()), 8 if i else 0)
                y = joined(_drain(v))
                for j in range(8):
                    va[j, HALO:, :] = y[:, j * 128:(j + 1) * 128]
                yield from _woven(b, 28, prep_xa(pc, t + 1, 6), 8)
                return (yield from b)

            rest = products()
            _drain(_woven(rest, n0, _chain(*[prep_ctx(pc, t, i) for i in range(7)]), 224, ager))
            _drain(_woven(rest, n1, window_weights(pc, t), 32 * (WIN // lw) + RO // sm))
            _drain(_woven(rest, 7 * NP - n0 - n1 - n2, window_mix(pc, t), 32 * (8 // lj) + 56))
            stage[_rows(t * RO, RO), DM:] = joined(_drain(rest)).astype(BF16)
            if early:
                cp_out(t, 1).start()
            stage[_rows(t * RO, RO), 0:DM] = joined(_drain(times(5, wa32, 3 * NP))).astype(BF16)
            if not early:
                cp_out(t, 1).start()
            cp_out(t, 0).start()

        if "r" in ph:
            jax.lax.fori_loop(0, steps, step, None)
        else:
            stage[0:16, 0:128] = _b16(ctx32[0, 0:8, :] | wo32[0, 0, 0:8, :] | wa32[0, 0, 0:8, :])
        cp_xa(steps + 1).wait()
        for t in range(steps):
            cp_out(t, 1).wait()
            cp_out(t, 0).wait()

    rows_phase()


def build(pred=8, fl="", **cfg):
    flags = {"XLA_TPU_MAX_INSTS_TO_PREDICATE": pred} if pred is not None else None
    names = {"L": "XLA_TPU_FORCE_LP_LLO_SCHEDULER", "E": "XLA_TPU_EVENLY_DISTRIBUTE_CRITICAL_NODES",
             "F": "XLA_TPU_ENABLE_LLO_SMALL_LOOP_FLATTENING", "R": "XLA_TPU_RESCHEDULE_DMA_DONES"}
    flags.update({names[c]: True for c in fl})
    vm, dma = pltpu.VMEM, pltpu.SemaphoreType.DMA
    scratch = [
        vm((HB + GH, S, DB), BF16),
        vm((NP, 2, HB * DB // 4, 128), BF16), vm((4 * NP, 2, DM // 4, 128), BF16),
        vm((2, 4, 16 * cfg["sp"], DM), U32), vm((2, 4, 16 * cfg["sp"], DM), U32),
        vm((NP, 2, S // 4, 128), BF16), vm((NP, 1, S // 4, 128), BF16), vm((NP + 8, 4 * 128, DB), BF16),
        vm((2, 2, DM, DB), U32), vm((2, 2, 2, DC, DB), U32),
        vm((GH, S, DB), BF16), vm((GH, S, DB), BF16),
        vm((8, RO, 128), F32), vm((8, HALO + RO, 128), F32), vm((8, HALO + RO, 128), F32),
        vm((8, RO, 128), F32), vm((WIN, RO, 128), F32),
        vm((3, RO // 2, DM), U32), vm((S, 2 * DM), BF16),
        dma((2,)), dma((2,)), dma((2, 3, 2)), dma((GH,)), dma((3,)), dma((2, S // RO)),
    ]

    @jax.jit
    def run(A_x, A_wqkv, A_wo, B_x, B_c_kv, B_w_q, B_w_uk, B_w_uv, B_w_o):
        out = pl.pallas_call(
            functools.partial(_kernel, **cfg),
            out_shape=jax.ShapeDtypeStruct((S, 2 * DM), BF16),
            in_specs=[pl.BlockSpec(memory_space=pl.ANY)] * 9,
            out_specs=pl.BlockSpec(memory_space=pl.ANY),
            scratch_shapes=scratch,
            compiler_params=pltpu.CompilerParams(vmem_limit_bytes=128 * 2**20, flags=flags),
            name="fused",
        )(A_x.reshape(S, DM), A_wqkv, A_wo.reshape(8, DM // 8, DM),
          B_x.reshape(S, DM), B_c_kv.reshape(S, DC), B_w_q, B_w_uk, B_w_uv, B_w_o)
        return out.reshape(1, S, 2 * DM)

    return run


@jax.jit
def pallas_concat_heads__sliding_local_dilated__compressed_kv_cla__prompt_kernel(
    A_x: jax.Array,
    A_wqkv: jax.Array,
    A_wo: jax.Array,
    B_x: jax.Array,
    B_c_kv: jax.Array,
    B_w_q: jax.Array,
    B_w_uk: jax.Array,
    B_w_uv: jax.Array,
    B_w_o: jax.Array,
):
    return build(**CFG)(A_x, A_wqkv, A_wo, B_x, B_c_kv, B_w_q, B_w_uk, B_w_uv, B_w_o)
```

```python
import functools
import math

import jax
import jax.numpy as jnp
from jax.experimental import pallas as pl
from jax.experimental.pallas import tpu as pltpu

S = 2048
DM = 1024
HA, DA = 32, 32
WIN, DIL = 8, 2
HB, DB = 32, 128
DC = 512
NEG = -1e9
LOG2E = math.log2(math.e)

GH = 4
NG = HB // GH
SET = S // GH
RO = 256
HALO = 16
NP = 49
TILE = 64

F32, BF16, U32 = jnp.float32, jnp.bfloat16, jnp.uint32
NT = (((1,), (1,)), ((), ()))

CFG = dict(ph="pjar", ch=4, lag=12, n0=150, early=1, agep=10, agea=3, ager=8, lw=2, lj=2, sa=3, n1=100, n2=6, sm=16,
           hp=2, sp=2, pin=10, agex=15, order='vqk', tailp=4, way='dd', taila=8, n3=44)

RA = RO // 8


def _b16(x32):
    return pltpu.bitcast(x32, BF16)


def _f32(x32):
    return _b16(x32).astype(F32)


def _wide(load, tiles):
    return jnp.concatenate([load(t) for t in range(tiles)], axis=1) if tiles > 1 else load(0)


def _dot(a32, b32):
    return jnp.dot(_b16(a32), _b16(b32), preferred_element_type=F32)


def _recip(x):
    r = pl.reciprocal(x, approx=True)
    return r * (2.0 - x * r)


def _rows(start, size, align=None):
    return pl.ds(start if isinstance(start, int) else pl.multiple_of(start, align or size), size)


def _fold(f, x):
    return functools.reduce(f, [x[:, c:c + 128] for c in range(0, x.shape[1], 128)])


def _quads(x):
    n = len(x) // 2
    return ([r[:n] for r in x[:n]], [r[n:] for r in x[:n]],
            [r[:n] for r in x[n:]], [r[n:] for r in x[n:]])


def _add(x, y):
    return [[a + b for a, b in zip(r, s)] for r, s in zip(x, y)]


def _sub(x, y):
    return [[a - b for a, b in zip(r, s)] for r, s in zip(x, y)]


def _lhs_term(x, i):
    a11, a12, a21, a22 = _quads(x)
    return (lambda: a11, lambda: _add(a11, a12), lambda: _add(a21, a22), lambda: a22,
            lambda: _add(a11, a22), lambda: _sub(a12, a22), lambda: _sub(a21, a11))[i]()


def _rhs_term(x, i):
    b11, b12, b21, b22 = _quads(x)
    return (lambda: _sub(b12, b22), lambda: b22, lambda: b11, lambda: _sub(b21, b11),
            lambda: _add(b11, b22), lambda: _add(b21, b22), lambda: _add(b11, b12))[i]()


def _seven(term, x, i):
    y = term(x, i)
    return [(7 * i + j, term(y, j)[0][0]) for j in range(7)]


def _combine(product, level=2, base=0):
    if level == 0:
        return [[(yield from product(base))]]
    k = 7 ** (level - 1)
    m3 = yield from _combine(product, level - 1, base)
    m5 = yield from _combine(product, level - 1, base + k)
    c12 = _add(m3, m5)
    m2 = yield from _combine(product, level - 1, base + 2 * k)
    c22 = _sub(m3, m2)
    m4 = yield from _combine(product, level - 1, base + 3 * k)
    c21 = _add(m2, m4)
    c11 = _sub(m4, m5)
    m1 = yield from _combine(product, level - 1, base + 4 * k)
    c11 = _add(c11, m1)
    c22 = _add(c22, m1)
    c11 = _add(c11, (yield from _combine(product, level - 1, base + 5 * k)))
    c22 = _add(c22, (yield from _combine(product, level - 1, base + 6 * k)))
    return [r + s for r, s in zip(c11, c12)] + [r + s for r, s in zip(c21, c22)]


def _drain(gen):
    while True:
        try:
            next(gen)
        except StopIteration as e:
            return e.value


def _chain(*gens):
    for g in gens:
        yield from g


def _woven(main, count, side, side_count, skip=0):
    done = 0
    for _ in range(skip):
        next(main)
        yield
    count -= skip
    for i in range(count):
        while done < side_count and done * count < (i + 1) * side_count:
            next(side)
            done += 1
        next(main)
        yield
    _drain(side)


class _Pace:
    def __init__(self, zero, age):
        self.zero, self.age, self.recent = zero, age, []

    def note(self, y):
        self.recent.append(y[:, -128:])
        return y

    def after(self, age=None):
        age = age or self.age
        if len(self.recent) < age:
            return lambda x: x
        bits = pltpu.bitcast(self.recent[-age][:8], U32) & self.zero
        return lambda x: pltpu.bitcast(
            pltpu.bitcast(x, U32) | jnp.concatenate([bits] * (x.shape[0] // 8), axis=0), x.dtype)

    def tied(self, x, y):
        zero = jnp.concatenate([self.zero] * (x.shape[0] // 8), axis=0)
        return pltpu.bitcast(pltpu.bitcast(x, U32) | (pltpu.bitcast(y, U32) & zero), x.dtype)

    def blocks(self, load):
        tie = self.after()
        return [[tie(load(i, j)) if i % 2 == 0 and j % 2 == 0 else load(i, j) for j in range(4)]
                for i in range(4)]


def _swap_lane_and_chunk_bits(chunks):
    lane = jax.lax.broadcasted_iota(jnp.int32, chunks[0].shape, 1)
    u = (lane >> 1) & 7
    rolled = [x if c == 0 else pltpu.roll(x, 2 * c, 1) for c, x in enumerate(chunks)]
    xs = [rolled[(-i) % 8] for i in range(8)]
    for t in (1, 2, 4):
        m = (u & t) != 0
        xs = [jnp.where(m, xs[(i - t) % 8], xs[i]) for i in range(8)]
    return [x if j == 0 else pltpu.roll(x, 128 - 2 * j, 1) for j, x in enumerate(xs)]


def _kernel(xa_hbm, wqkv_hbm, woa_hbm, xb_hbm, c_hbm, wq_hbm, wuk_hbm, wuv_hbm, wob_hbm,
            out_hbm,
            ctx, wo, wa, wo_raw, wa_raw, xc, cc, wb, wq_raw, wkv_raw, ks, vs,
            qa, ka, va, ya, pa, xa_raw, stage,
            sem_wo, sem_wa, sem_w, sem_x, sem_xa, sem_out, *,
            ph, ch, lag, n0, early, agep, agea, ager, lw, lj, sa, n1, n2, sm, hp, sp, pin, agex, order, tailp, way, taila, n3):
    xa32, wqkv32, woa32 = (r.bitcast(U32) for r in (xa_hbm, wqkv_hbm, woa_hbm))
    wob32 = wob_hbm.bitcast(U32)
    wq32, wk32, wv32 = (r.bitcast(U32) for r in (wq_hbm, wuk_hbm, wuv_hbm))

    ctx32, wo32, wa32, xc32, cc32, wb32, ks32, vs32 = (
        r.bitcast(U32) for r in (ctx, wo, wa, xc, cc, wb, ks, vs))

    def pace(step, age):
        return _Pace(jnp.full((8, 128), step // S, jnp.int32).astype(U32), age)

    def zero(step, salt):
        return step // (S + salt)

    def start_slabs(i):
        u = jnp.minimum(i * sp, HB - sp)
        v = jnp.minimum(u, 24 - sp)
        slot = i % 2 + jnp.where(i * sp < 24, 0, 2)
        for k in range(4):
            pltpu.make_async_copy(wob32.at[u // GH * GH + k, _rows(u % GH * 16, 16 * sp), :],
                                  wo_raw.at[i % 2, k], sem_wo.at[i % 2]).start()
            pltpu.make_async_copy(wqkv32.at[_rows(k * 128 + v % 8 * 16, 16 * sp), _rows(v // 8 * DM, DM)],
                                  wa_raw.at[slot, k], sem_wa.at[slot]).start()

    def start_output_slabs(i):
        for k in range(4):
            for e in range(2 * sp):
                m = k * 16 + i * sp % 8 * 2 + e
                pltpu.make_async_copy(woa32.at[:, ((m >> 1) & 3) * 16 + (m & 1) * 8 + (m >> 3), :],
                                      wa_raw.at[i % 2, k, pl.ds(8 * e, 8), :], sem_wa.at[i % 2]).start()

    def wait_slot(raw, sem, slot):
        pltpu.make_async_copy(raw.at[slot], raw.at[slot], sem.at[slot]).wait()

    def cp_xa(t):
        return pltpu.make_async_copy(xa32.at[_rows(jnp.minimum(t, S // RO - 1) * (RO // 2), RO // 2), :],
                                     xa_raw.at[t % 3], sem_xa.at[t % 3])

    def prep_slabs(pc, u, load, store):
        for half in range(2):
            for c in range(2):
                for i in range(7):
                    z = zero(u, i)
                    x = pc.blocks(lambda k, j: load(z, k, half * 8, 2 * j + c))
                    for n, y in _seven(_rhs_term, [[_f32(w) for w in r] for r in x], i):
                        store(n, half * 16, c, y.astype(BF16))
                    yield

    def prep_wo(pc, u, at):
        def store(n, row, c, y):
            wo[n, c, _rows(u * 32 + row, 16), :] = y
        return prep_slabs(
            pc, u, lambda z, k, row, c: wo_raw[u // sp % 2 + z, k, pl.ds(at + row, 8), c * 128:(c + 1) * 128], store)

    def permute_wa(pc, u, at):
        for i in range(4):
            for half in range(2):
                tie = pc.after(agex)
                raw = [tie(wa_raw[u // sp % 2, i, pl.ds(at + half * 8, 8), c * 128:(c + 1) * 128])
                       for c in range(8)]
                for c, y in enumerate(_swap_lane_and_chunk_bits(raw)):
                    wb32[NP + c, pl.ds(i * 16 + half * 8, 8), :] = jnp.where(u < 24, y, raw[c])
                yield

    def prep_wa(pc, u):
        def store(n, row, c, y):
            wa[u // 8 * NP + n, c, _rows(u % 8 * 32 + row, 16), :] = y
        return prep_slabs(pc, u, lambda z, k, row, c: wb32[NP + c + z, k * 16 + row:k * 16 + row + 8, :], store)

    def heads():
        def cp_w(g):
            return [pltpu.make_async_copy(src.at[:, 2 * g + i, :], dst.at[i], sem_w.at[g % 2, kind, i])
                    for kind, (src, dst) in enumerate(((wk32, wkv_raw.at[g % 2, 0]), (wv32, wkv_raw.at[g % 2, 1]),
                                                       (wq32, wq_raw.at[g % 2])))
                    for i in range(2)]

        def cp_rows(j):
            r = _rows(j * SET, SET)
            return [pltpu.make_async_copy(src.at[r, t * 128:(t + 1) * 128], ctx.at[page + t, r, :], sem_x.at[j])
                    for page, src in ((0, c_hbm), (4, xb_hbm)) for t in range(src.shape[1] // 128)]

        def prep_rows(pc, page, dst, j, a):
            r, tiles = SET // 8, dst.shape[1]
            for t in range(tiles):
                x = [[_f32(ctx32[page + k * tiles + t, _rows(j * (SET // 2) + b * r + a, 8), :])
                      for k in range(4)] for b in range(4)]
                for i in range(7):
                    for n, y in _seven(_lhs_term, x, i):
                        dst[n, t, _rows(2 * (j * r + a), 16), :] = y.astype(BF16)
                    yield

        def prep_w(pc, g, j):
            def unit(raw, depth, a, row):
                for i in range(7):
                    if pc or i == 0:
                        tie, z = (pc.after(), zero(j, i)) if pc else (lambda w: w, 0)
                        x = []
                        for k in range(4):
                            words = [raw[pair + z, _rows(k * (depth // 4) + j * (depth // 16) + a, 16), :]
                                     for pair in range(2)]
                            words = [tie(w) for w in words] if k % 2 == 0 else words
                            x.append([pltpu.bitcast(h, F32) for w in words
                                      for h in (w << 16, w & jnp.uint32(0xFFFF0000))])
                    for n, y in _seven(_rhs_term, x, i):
                        wb[n, _rows(2 * row, 16), :] = y.astype(BF16)
                    yield

            for a in range(0, DM // 16, 16):
                yield from unit(wq_raw.at[g % 2], DM, a, j * (DM // 32) + a // 2)
            for kind in range(2):
                for a in range(0, DC // 16, 16):
                    yield from unit(wkv_raw.at[g % 2, kind], DC, a, (2 + kind) * TILE + j * (DC // 32) + a // 2)

        def project(pc, j):
            r = SET // 8
            rows = _rows(j * r, r)

            def product(lhs, first, last):
                def run(n):
                    y = pc.note(_dot(_wide(lambda t: lhs[n, t, rows, :], last - first), wb32[n + zero(j, 0), first * TILE:last * TILE, :]))
                    yield
                    return y
                return _combine(run)

            parts = dict(q=(ctx, HB, DB ** -0.5 * LOG2E, product(xc32, 0, 2)),
                         k=(ks, 0, None, product(cc32, 2, 3)), v=(vs, 0, None, product(cc32, 3, 4)))
            for dst, page, scale, gen in (parts[c] for c in order):
                y = yield from gen
                for i in range(4):
                    for h in range(GH):
                        dst[page + h, _rows(j * SET + i * 2 * r, 2 * r), :] = (
                            y[i][h] * scale if scale else y[i][h]).astype(BF16)

        def attend(pc, g, first, side, side_steps):
            nb = S // 128
            ways = dict(d=list(reversed(range(nb))), a=list(range(nb)),
                        z=[i for j in range(nb // 2) for i in (nb - 1 - j, j)],
                        m=[i for j in range(nb // 2) for i in (nb // 2 - 1 - j, nb // 2 + j)],
                        v=list(range(nb - 1, -1, -2)) + list(range(0, nb, 2)))
            blocks = [(h, i) for h in range(hp) for i in ways[way[h]]]
            if way[-1] == "x":
                blocks = [b for pair in zip(blocks[:nb], blocks[nb:]) for b in pair]
            work = [(first + h, i, t, min(t + ch, i + 1)) for h, i in blocks for t in range(0, i + 1, ch)]
            key = [h * nb + i for h, i in blocks for t in range(0, i + 1, ch)]
            s, mx, m, l, o, done, ready, due = {}, {}, {}, {}, {}, {}, [], []

            def scores(b, h, i, t0, t1):
                x = pc.note(jax.lax.dot_general(_b16(ctx32[HB + h, i * TILE:(i + 1) * TILE, :]),
                                                _b16(ks32[h, t0 * TILE:t1 * TILE, :]), NT,
                                                preferred_element_type=F32))
                if t1 == i + 1:
                    row, col = (jax.lax.broadcasted_iota(jnp.int32, (128, 128), d) for d in range(2))
                    diag = jnp.where(col <= row, x[:, -128:], NEG)
                    x = jnp.concatenate([x[:, :-128], diag], axis=1) if t1 - t0 > 1 else diag
                s[b, t0] = x
                mx[b] = jnp.maximum(mx[b], _fold(jnp.maximum, x)) if t0 else _fold(jnp.maximum, x)
                if t1 == i + 1:
                    m[b] = jnp.max(mx[b], axis=1, keepdims=True)

            def values(b, h, i, t0, t1):
                p = jnp.exp2(s.pop((b, t0)) - m[b])
                y = pc.note(jnp.dot(p.astype(BF16), _b16(vs32[h, t0 * TILE:t1 * TILE, :]),
                                    preferred_element_type=F32))
                parts = ([l[b]] if t0 else []) + [p[:, c:c + 128] for c in range(0, p.shape[1], 128)]
                l[b] = functools.reduce(jnp.add, [pc.tied(parts[0], pc.recent[-1 - sa])] + parts[1:])
                o[b] = o[b] + y if t0 else y
                if t1 == i + 1:
                    ready.append((h, i, (o[b] * _recip(jnp.sum(l[b], axis=1, keepdims=True))).astype(BF16)))

            def products():
                clock = qi = pi = turn = 0
                while pi < len(work):
                    can = key[pi] in done and clock - done[key[pi]] >= lag
                    if qi < len(work) and (not can or turn == 0):
                        scores(key[qi], *work[qi])
                        clock += work[qi][3] - work[qi][2]
                        if work[qi][3] == work[qi][1] + 1:
                            done[key[qi]] = clock
                        qi, turn = qi + 1, 1
                    else:
                        values(key[pi], *work[pi])
                        clock += work[pi][3] - work[pi][2]
                        if len(due) < len(ready):
                            due.append(clock + pin)
                        pi, turn = pi + 1, 0
                    while due and (due[0] <= clock or pi == len(work)):
                        due.pop(0)
                        h, i, x = ready.pop(0)
                        ctx[g * GH + h, i * 128:(i + 1) * 128, :] = x
                    yield

            main = products()
            _drain(_woven(main, 2 * len(work) - taila, side, side_steps, agea))
            _drain(main)

        for cp in cp_w(0) + cp_rows(0) + cp_rows(1):
            cp.start()
        start_slabs(jnp.int32(0))
        for cp in cp_w(0):
            cp.wait()
        jax.lax.fori_loop(0, GH, lambda j, _: _drain(prep_w(None, 0, j)), None)

        def group(g, _):
            def rows(jj, _):
                @pl.when(g == 0)
                def _():
                    for j in [jj * sp + i for i in range(sp)]:
                        @pl.when(j + 2 < GH)
                        def _():
                            for cp in cp_rows(j + 2):
                                cp.start()
                        for cp in cp_rows(j):
                            cp.wait()

                        @pl.when(j == 1)
                        def _():
                            start_slabs(j)

                        @pl.when(j == GH - 1)
                        def _():
                            for cp in cp_w(1):
                                cp.start()

                        def first_rows(a, _):
                            _drain(prep_rows(None, 0, cc, j, a * 8))
                            _drain(prep_rows(None, 4, xc, j, a * 8))
                        jax.lax.fori_loop(0, SET // 64, first_rows, None)


                i = g * (GH // sp) + jj

                @pl.when((i + 1) * sp >= 24)
                def _():
                    @pl.when(i * sp >= 24)
                    def _():
                        wait_slot(wa_raw, sem_wa, 2 + i % 2)

                    @pl.when((i + 1) * sp < HB)
                    def _():
                        start_output_slabs(i + 1)
                wait_slot(wo_raw, sem_wo, i % 2)
                wait_slot(wa_raw, sem_wa, i % 2)
                pc = pace(g, agep)
                for n in range(sp):
                    j = jj * sp + n
                    u = g * GH + j
                    side = _chain(_woven(prep_wo(pc, u, 16 * n), 28, permute_wa(pc, u, 16 * n), 8), prep_wa(pc, u))
                    main = project(pc, j)
                    _drain(_woven(main, 3 * NP - tailp, side, 56, 0 if pc.recent else agex))
                    _drain(main)
                start_slabs(i + 2)

            @pl.when((g > 0) & (g + 1 < NG))
            def _():
                for cp in cp_w(g + 1):
                    cp.start()

            @pl.when(g == NG - 1)
            def _():
                cp_xa(0).start()
                cp_xa(1).start()
            if "j" in ph:
                jax.lax.fori_loop(0, GH // sp, rows, None)

            @pl.when(g + 1 < NG)
            def _():
                for cp in cp_w(g + 1):
                    cp.wait()

            def attention(hh, _):
                pc = pace(g, agea)
                nxt = jnp.minimum(g + 1, NG - 1)
                attend(pc, g, hh * hp, _chain(*[prep_w(pc, nxt, hh * hp + i) for i in range(hp)]), 56 * hp)
            if "a" in ph:
                jax.lax.fori_loop(0, GH // hp, attention, None)
            else:
                ctx32[0, 0:8, :] = ks32[0, 0:8, :] | vs32[0, 0:8, :]

        jax.lax.fori_loop(0, NG, group, None)
        wait_slot(wo_raw, sem_wo, 0)
        wait_slot(wo_raw, sem_wo, 1)
        wait_slot(wa_raw, sem_wa, 2)
        wait_slot(wa_raw, sem_wa, 3)

    heads()

    def rows_phase():
        def cp_out(t, part):
            at = (_rows(t * RO, RO), pl.ds(part * DM, DM))
            return pltpu.make_async_copy(stage.at[at], out_hbm.at[at], sem_out.at[part, t])

        def prep_ctx(pc, t, i):
            for a in range(0, RA, 8):
                for p in range(NG):
                    z = zero(t, i)
                    x = pc.blocks(lambda b, k: ctx32[p * GH + k + z, _rows(t * (RO // 2) + b * RA + a, 8), :])
                    for n, y in _seven(_lhs_term, [[_f32(w) for w in row] for row in x], i):
                        xc[n, p % 2, pl.ds(2 * (p // 2 * RA + a), 16), :] = y.astype(BF16)
                    yield

        def prep_xa(pc, t, i):
            for a in range(0, RA, 8):
                for c in range(2):
                    slot = t % 3 + zero(t, i)
                    x = pc.blocks(lambda b, k: xa_raw[slot, b * RA + a:b * RA + a + 8, (2 * k + c) * 128:(2 * k + c + 1) * 128])
                    for n, y in _seven(_lhs_term, [[_f32(w) for w in row] for row in x], i):
                        xc[n, c, pl.ds(2 * (4 * RA + a), 16), :] = y.astype(BF16)
                    yield

        def window_weights(pc, t):
            lane = jax.lax.broadcasted_iota(jnp.int32, (sm, 128), 1)

            def softmax(a):
                tie = pc.after()
                logits = []
                for w in range(WIN):
                    x = jnp.concatenate([tie(pa[w + zero(t, 1), b:b + 8, :]) for b in range(a, a + sm, 8)], axis=0)
                    for bit in (16, 1):
                        x = x + jnp.where((lane & bit) != 0, pltpu.roll(x, bit, 1), pltpu.roll(x, 128 - bit, 1))
                    if a < DIL * w:
                        pos = jax.lax.broadcasted_iota(jnp.int32, (sm, 128), 0) + (t * RO + a)
                        x = jnp.where(pos >= DIL * w, x, NEG)
                    logits.append(x)
                top = functools.reduce(jnp.maximum, logits)
                es = [jnp.exp2(x - top) for x in logits]
                inv = _recip(functools.reduce(jnp.add, es))
                for w, e in enumerate(es):
                    pa[w, a:a + sm, :] = e * inv

            for a in range(0, RO, 8):
                for w in range(WIN):
                    if w % lw == 0:
                        tie = pc.after()
                        q = [tie(qa[j, a:a + 8, :]) for j in range(8)]
                    b = a + HALO - DIL * w
                    x = q[0] * ka[0, b:b + 8, :]
                    for j in range(1, 8):
                        x = x + q[j] * ka[j, b:b + 8, :]
                    pa[w, a:a + 8, :] = x
                    if w % lw == lw - 1:
                        yield
                if (a + 8) % sm == 0:
                    softmax(a + 8 - sm)
                    yield
            ka[:, 0:HALO, :] = ka[:, RO:, :]

        def window_mix(pc, t):
            for a in range(0, RO, 8):
                for j in range(8):
                    if j % lj == 0:
                        tie = pc.after()
                        ps = [tie(pa[w + zero(t, 0), a:a + 8, :]) for w in range(WIN)]
                    acc = ps[0] * va[j, a + HALO:a + HALO + 8, :]
                    for w in range(1, WIN):
                        b = a + HALO - DIL * w
                        acc = acc + ps[w] * va[j, b:b + 8, :]
                    ya[j, a:a + 8, :] = acc
                    if j % lj == lj - 1:
                        yield
            va[:, 0:HALO, :] = va[:, RO:, :]

        def prep_mixed(pc, t):
            for i in range(7):
                for a in range(0, RA, 8):
                    for c in range(2):
                        z = zero(t, i)
                        x = pc.blocks(lambda b, k: ya[2 * k + c + z, pl.ds(2 * (b * RA + a), 16), :])
                        for n, y in _seven(_lhs_term, x, i):
                            xc[n, c, pl.ds(2 * (5 * RA + a), 16), :] = y.astype(BF16)
                        yield

        def joined(c):
            return jnp.concatenate([jnp.concatenate(row, axis=1) for row in c], axis=0)

        steps = S // RO
        ka[:, 0:HALO, :] = jnp.zeros((8, HALO, 128), F32)
        va[:, 0:HALO, :] = jnp.zeros((8, HALO, 128), F32)

        cp_xa(0).wait()
        if "p" in ph:
            for i in range(7):
                _drain(prep_xa(pace(0, 1), 0, i))

        def step(t, _):
            pc = pace(t, ager)

            cp_xa(t + 2).start()
            cp_xa(t + 1).wait()

            def times(first, w, at):
                def run(n):
                    y = None
                    for k in range(w.shape[2] // 128):
                        z = pc.note(_dot(_wide(lambda c: xc32[n, c, pl.ds((first + k) * RA, RA), :], 2),
                                         _wide(lambda c: w[at + n, c, k * 128:(k + 1) * 128, :], 2)))
                        y = z if y is None else y + z
                        yield
                    return y
                return _combine(run)

            b = times(0, wo32, 0)

            def products():
                y = joined((yield from times(4, wa32, NP)))
                for j in range(8):
                    ka[j, HALO:, :] = y[:, j * 128:(j + 1) * 128]
                y = joined((yield from times(4, wa32, 0))) * (DA ** -0.5 * LOG2E)
                for j in range(8):
                    qa[j] = y[:, j * 128:(j + 1) * 128]
                v = times(4, wa32, 2 * NP)
                for i in range(7):
                    yield from _woven(v, 7, prep_xa(pc, t + 1, i - 1) if i else iter(()), 8 if i else 0)
                y = joined(_drain(v))
                for j in range(8):
                    va[j, HALO:, :] = y[:, j * 128:(j + 1) * 128]
                yield from _woven(b, 28, prep_xa(pc, t + 1, 6), 8)
                return (yield from b)

            rest = products()
            _drain(_woven(rest, n0, _chain(*[prep_ctx(pc, t, i) for i in range(7)]), 224, ager))
            _drain(_woven(rest, n1, window_weights(pc, t), 32 * (WIN // lw) + RO // sm))
            _drain(_woven(rest, 7 * NP - n0 - n1 - n2 - n3, window_mix(pc, t), 32 * (8 // lj)))
            _drain(_woven(rest, n3, prep_mixed(pc, t), 56))
            stage[_rows(t * RO, RO), DM:] = joined(_drain(rest)).astype(BF16)
            if early:
                cp_out(t, 1).start()
            stage[_rows(t * RO, RO), 0:DM] = joined(_drain(times(5, wa32, 3 * NP))).astype(BF16)
            if not early:
                cp_out(t, 1).start()
            cp_out(t, 0).start()

        if "r" in ph:
            jax.lax.fori_loop(0, steps, step, None)
        else:
            stage[0:16, 0:128] = _b16(ctx32[0, 0:8, :] | wo32[0, 0, 0:8, :] | wa32[0, 0, 0:8, :])
        cp_xa(steps + 1).wait()
        for t in range(steps):
            cp_out(t, 1).wait()
            cp_out(t, 0).wait()

    rows_phase()


def build(pred=8, fl="", **cfg):
    flags = {"XLA_TPU_MAX_INSTS_TO_PREDICATE": pred} if pred is not None else None
    names = {"L": "XLA_TPU_FORCE_LP_LLO_SCHEDULER", "E": "XLA_TPU_EVENLY_DISTRIBUTE_CRITICAL_NODES",
             "F": "XLA_TPU_ENABLE_LLO_SMALL_LOOP_FLATTENING", "R": "XLA_TPU_RESCHEDULE_DMA_DONES"}
    flags.update({names[c]: True for c in fl})
    vm, dma = pltpu.VMEM, pltpu.SemaphoreType.DMA
    scratch = [
        vm((HB + GH, S, DB), BF16),
        vm((NP, 2, HB * DB // 4, 128), BF16), vm((4 * NP, 2, DM // 4, 128), BF16),
        vm((2, 4, 16 * cfg["sp"], DM), U32), vm((4, 4, 16 * cfg["sp"], DM), U32),
        vm((NP, 2, S // 4, 128), BF16), vm((NP, 1, S // 4, 128), BF16), vm((NP + 8, 4 * 128, DB), BF16),
        vm((2, 2, DM, DB), U32), vm((2, 2, 2, DC, DB), U32),
        vm((GH, S, DB), BF16), vm((GH, S, DB), BF16),
        vm((8, RO, 128), F32), vm((8, HALO + RO, 128), F32), vm((8, HALO + RO, 128), F32),
        vm((8, RO, 128), F32), vm((WIN, RO, 128), F32),
        vm((3, RO // 2, DM), U32), vm((S, 2 * DM), BF16),
        dma((2,)), dma((4,)), dma((2, 3, 2)), dma((GH,)), dma((3,)), dma((2, S // RO)),
    ]

    @jax.jit
    def run(A_x, A_wqkv, A_wo, B_x, B_c_kv, B_w_q, B_w_uk, B_w_uv, B_w_o):
        out = pl.pallas_call(
            functools.partial(_kernel, **cfg),
            out_shape=jax.ShapeDtypeStruct((S, 2 * DM), BF16),
            in_specs=[pl.BlockSpec(memory_space=pl.ANY)] * 9,
            out_specs=pl.BlockSpec(memory_space=pl.ANY),
            scratch_shapes=scratch,
            compiler_params=pltpu.CompilerParams(vmem_limit_bytes=128 * 2**20, flags=flags),
            name="fused",
        )(A_x.reshape(S, DM), A_wqkv, A_wo.reshape(8, DM // 8, DM),
          B_x.reshape(S, DM), B_c_kv.reshape(S, DC), B_w_q, B_w_uk, B_w_uv, B_w_o)
        return out.reshape(1, S, 2 * DM)

    return run


@jax.jit
def pallas_concat_heads__sliding_local_dilated__compressed_kv_cla__prompt_kernel(
    A_x: jax.Array,
    A_wqkv: jax.Array,
    A_wo: jax.Array,
    B_x: jax.Array,
    B_c_kv: jax.Array,
    B_w_q: jax.Array,
    B_w_uk: jax.Array,
    B_w_uv: jax.Array,
    B_w_o: jax.Array,
):
    return build(**CFG)(A_x, A_wqkv, A_wo, B_x, B_c_kv, B_w_q, B_w_uk, B_w_uv, B_w_o)
```

```python
import functools
import math

import jax
import jax.numpy as jnp
from jax.experimental import pallas as pl
from jax.experimental.pallas import tpu as pltpu

S = 2048
DM = 1024
DA = 32
WIN, DIL = 8, 2
HB, DB = 32, 128
DC = 512
NEG = -1e9
LOG2E = math.log2(math.e)

NP = 49
GH = 4
NG = HB // GH
SET = S // GH
TILE = 64
RO = 256
RA = RO // 8
HALO = 16

F32, BF16, U32 = jnp.float32, jnp.bfloat16, jnp.uint32


def _b16(words):
    return pltpu.bitcast(words, BF16)


def _f32(words):
    return _b16(words).astype(F32)


def _dot(a, b):
    return jnp.dot(_b16(a), _b16(b), preferred_element_type=F32)


def _wide(load, tiles):
    return jnp.concatenate([load(t) for t in range(tiles)], axis=1) if tiles > 1 else load(0)


def _lane_tiles(x):
    return [x[:, c:c + 128] for c in range(0, x.shape[1], 128)]


def _rows(start, size):
    return pl.ds(start if isinstance(start, int) else pl.multiple_of(start, size), size)


def _recip(x):
    r = pl.reciprocal(x, approx=True)
    return r * (2.0 - x * r)


def _zero(step, salt):
    return step // (S + salt)


def _quads(x):
    n = len(x) // 2
    return ([r[:n] for r in x[:n]], [r[n:] for r in x[:n]],
            [r[:n] for r in x[n:]], [r[n:] for r in x[n:]])


def _add(x, y):
    return [[a + b for a, b in zip(r, s)] for r, s in zip(x, y)]


def _sub(x, y):
    return [[a - b for a, b in zip(r, s)] for r, s in zip(x, y)]


def _lhs_term(x, i):
    a11, a12, a21, a22 = _quads(x)
    return (lambda: a11, lambda: _add(a11, a12), lambda: _add(a21, a22), lambda: a22,
            lambda: _add(a11, a22), lambda: _sub(a12, a22), lambda: _sub(a21, a11))[i]()


def _rhs_term(x, i):
    b11, b12, b21, b22 = _quads(x)
    return (lambda: _sub(b12, b22), lambda: b22, lambda: b11, lambda: _sub(b21, b11),
            lambda: _add(b11, b22), lambda: _add(b21, b22), lambda: _add(b11, b12))[i]()


def _seven(term, x, i):
    y = term(x, i)
    return [(7 * i + j, term(y, j)[0][0]) for j in range(7)]


def _combine(product, level=2, base=0):
    if level == 0:
        return [[(yield from product(base))]]
    k = 7 ** (level - 1)
    m3 = yield from _combine(product, level - 1, base)
    m5 = yield from _combine(product, level - 1, base + k)
    c12 = _add(m3, m5)
    m2 = yield from _combine(product, level - 1, base + 2 * k)
    c22 = _sub(m3, m2)
    m4 = yield from _combine(product, level - 1, base + 3 * k)
    c21 = _add(m2, m4)
    c11 = _sub(m4, m5)
    m1 = yield from _combine(product, level - 1, base + 4 * k)
    c11 = _add(c11, m1)
    c22 = _add(c22, m1)
    c11 = _add(c11, (yield from _combine(product, level - 1, base + 5 * k)))
    c22 = _add(c22, (yield from _combine(product, level - 1, base + 6 * k)))
    return [r + s for r, s in zip(c11, c12)] + [r + s for r, s in zip(c21, c22)]


def _drain(gen):
    while True:
        try:
            next(gen)
        except StopIteration as e:
            return e.value


def _chain(*gens):
    for g in gens:
        yield from g


def _woven(main, count, side, side_count, skip=0):
    for _ in range(skip):
        next(main)
        yield
    count, done = count - skip, 0
    for i in range(count):
        while done < side_count and done * count < (i + 1) * side_count:
            next(side)
            done += 1
        next(main)
        yield
    _drain(side)


class _Pace:
    def __init__(self, step, age):
        self.zero = jnp.full((8, 128), step // S, jnp.int32).astype(U32)
        self.age, self.recent = age, []

    def note(self, y):
        self.recent.append(y[:, -128:])
        return y

    def after(self, age=None):
        age = age or self.age
        if len(self.recent) < age:
            return lambda x: x
        bits = pltpu.bitcast(self.recent[-age][:8], U32) & self.zero
        return lambda x: pltpu.bitcast(
            pltpu.bitcast(x, U32) | jnp.concatenate([bits] * (x.shape[0] // 8), axis=0), x.dtype)

    def tied(self, x, age):
        zero = jnp.concatenate([self.zero] * (x.shape[0] // 8), axis=0)
        return pltpu.bitcast(
            pltpu.bitcast(x, U32) | (pltpu.bitcast(self.recent[-age], U32) & zero), x.dtype)

    def blocks(self, load):
        tie = self.after()
        return [[tie(load(i, j)) if i % 2 == 0 and j % 2 == 0 else load(i, j) for j in range(4)]
                for i in range(4)]


def _swap_lane_and_tile_bits(tiles):
    lane = jax.lax.broadcasted_iota(jnp.int32, tiles[0].shape, 1)
    u = (lane >> 1) & 7
    rolled = [x if c == 0 else pltpu.roll(x, 2 * c, 1) for c, x in enumerate(tiles)]
    xs = [rolled[(-i) % 8] for i in range(8)]
    for t in (1, 2, 4):
        m = (u & t) != 0
        xs = [jnp.where(m, xs[(i - t) % 8], xs[i]) for i in range(8)]
    return [x if j == 0 else pltpu.roll(x, 128 - 2 * j, 1) for j, x in enumerate(xs)]


def _kernel(xa_hbm, wqkv_hbm, woa_hbm, xb_hbm, c_hbm, wq_hbm, wuk_hbm, wuv_hbm, wob_hbm,
            out_hbm,
            ctx, wo, wa, wo_raw, wa_raw, xc, cc, wb, wq_raw, wkv_raw, ks, vs,
            qa, ka, va, ya, pa, xa_raw, stage,
            sem_wo, sem_wa, sem_w, sem_x, sem_xa, sem_out):
    xa32, wqkv32, woa32 = (r.bitcast(U32) for r in (xa_hbm, wqkv_hbm, woa_hbm))
    wob32 = wob_hbm.bitcast(U32)
    wq32, wk32, wv32 = (r.bitcast(U32) for r in (wq_hbm, wuk_hbm, wuv_hbm))
    ctx32, wo32, wa32, xc32, cc32, wb32, ks32, vs32 = (
        r.bitcast(U32) for r in (ctx, wo, wa, xc, cc, wb, ks, vs))

    def start_slabs(i):
        u = jnp.minimum(i * 2, HB - 2)
        v = jnp.minimum(u, 22)
        slot = i % 2 + jnp.where(i * 2 < 24, 0, 2)
        for k in range(4):
            pltpu.make_async_copy(wob32.at[u // GH * GH + k, _rows(u % GH * 16, 32), :],
                                  wo_raw.at[i % 2, k], sem_wo.at[i % 2]).start()
            pltpu.make_async_copy(wqkv32.at[_rows(k * 128 + v % 8 * 16, 32), _rows(v // 8 * DM, DM)],
                                  wa_raw.at[slot, k], sem_wa.at[slot]).start()

    def start_output_slabs(i):
        for k in range(4):
            for e in range(4):
                m = k * 16 + i * 2 % 8 * 2 + e
                pltpu.make_async_copy(woa32.at[:, ((m >> 1) & 3) * 16 + (m & 1) * 8 + (m >> 3), :],
                                      wa_raw.at[i % 2, k, pl.ds(8 * e, 8), :], sem_wa.at[i % 2]).start()

    def wait_slot(raw, sem, slot):
        pltpu.make_async_copy(raw.at[slot], raw.at[slot], sem.at[slot]).wait()

    def cp_xa(t):
        return pltpu.make_async_copy(xa32.at[_rows(jnp.minimum(t, S // RO - 1) * (RO // 2), RO // 2), :],
                                     xa_raw.at[t % 3], sem_xa.at[t % 3])

    def prep_slabs(pc, u, load, store):
        for half in range(2):
            for c in range(2):
                for i in range(7):
                    z = _zero(u, i)
                    x = pc.blocks(lambda k, j: load(z, k, half * 8, 2 * j + c))
                    for n, y in _seven(_rhs_term, [[_f32(w) for w in r] for r in x], i):
                        store(n, half * 16, c, y.astype(BF16))
                    yield

    def prep_wo(pc, u, at):
        def store(n, row, c, y):
            wo[n, c, _rows(u * 32 + row, 16), :] = y
        return prep_slabs(
            pc, u, lambda z, k, row, c: wo_raw[u // 2 % 2 + z, k, pl.ds(at + row, 8), c * 128:(c + 1) * 128],
            store)

    def reorder_wa(pc, u, at):
        for i in range(4):
            for half in range(2):
                tie = pc.after(15)
                raw = [tie(wa_raw[u // 2 % 2, i, pl.ds(at + half * 8, 8), c * 128:(c + 1) * 128])
                       for c in range(8)]
                for c, y in enumerate(_swap_lane_and_tile_bits(raw)):
                    wb32[NP + c, pl.ds(i * 16 + half * 8, 8), :] = jnp.where(u < 24, y, raw[c])
                yield

    def prep_wa(pc, u):
        def store(n, row, c, y):
            wa[u // 8 * NP + n, c, _rows(u % 8 * 32 + row, 16), :] = y
        return prep_slabs(
            pc, u, lambda z, k, row, c: wb32[NP + c + z, k * 16 + row:k * 16 + row + 8, :], store)

    def cp_w(g):
        return [pltpu.make_async_copy(src.at[:, 2 * g + i, :], dst.at[i], sem_w.at[g % 2, kind, i])
                for kind, (src, dst) in enumerate(((wk32, wkv_raw.at[g % 2, 0]),
                                                   (wv32, wkv_raw.at[g % 2, 1]),
                                                   (wq32, wq_raw.at[g % 2])))
                for i in range(2)]

    def cp_rows(j):
        r = _rows(j * SET, SET)
        return [pltpu.make_async_copy(src.at[r, t * 128:(t + 1) * 128], ctx.at[page + t, r, :], sem_x.at[j])
                for page, src in ((0, c_hbm), (4, xb_hbm)) for t in range(src.shape[1] // 128)]

    def prep_rows(page, dst, j, a):
        r, tiles = SET // 8, dst.shape[1]
        for t in range(tiles):
            x = [[_f32(ctx32[page + k * tiles + t, _rows(j * (SET // 2) + b * r + a, 8), :])
                  for k in range(4)] for b in range(4)]
            for i in range(7):
                for n, y in _seven(_lhs_term, x, i):
                    dst[n, t, _rows(2 * (j * r + a), 16), :] = y.astype(BF16)

    def prep_w(pc, g, j):
        def unit(raw, depth, a, row):
            for i in range(7):
                if pc or i == 0:
                    tie, z = (pc.after(), _zero(j, i)) if pc else (lambda w: w, 0)
                    x = []
                    for k in range(4):
                        words = [raw[pair + z, _rows(k * (depth // 4) + j * (depth // 16) + a, 16), :]
                                 for pair in range(2)]
                        words = [tie(w) for w in words] if k % 2 == 0 else words
                        x.append([pltpu.bitcast(h, F32) for w in words
                                  for h in (w << 16, w & jnp.uint32(0xFFFF0000))])
                for n, y in _seven(_rhs_term, x, i):
                    wb[n, _rows(2 * row, 16), :] = y.astype(BF16)
                yield

        for a in range(0, DM // 16, 16):
            yield from unit(wq_raw.at[g % 2], DM, a, j * (DM // 32) + a // 2)
        for kind in range(2):
            for a in range(0, DC // 16, 16):
                yield from unit(wkv_raw.at[g % 2, kind], DC, a, (2 + kind) * TILE + j * (DC // 32) + a // 2)

    def project(pc, j):
        r = SET // 8
        rows = _rows(j * r, r)

        def product(lhs, first, last):
            def run(n):
                y = pc.note(_dot(_wide(lambda t: lhs[n, t, rows, :], last - first),
                                 wb32[n + _zero(j, 0), first * TILE:last * TILE, :]))
                yield
                return y
            return _combine(run)

        for dst, page, scale, gen in ((vs, 0, None, product(cc32, 3, 4)),
                                      (ctx, HB, DB ** -0.5 * LOG2E, product(xc32, 0, 2)),
                                      (ks, 0, None, product(cc32, 2, 3))):
            y = yield from gen
            for i in range(4):
                for h in range(GH):
                    dst[page + h, _rows(j * SET + i * 2 * r, 2 * r), :] = (
                        y[i][h] * scale if scale else y[i][h]).astype(BF16)

    def attend(pc, g, first, side, side_steps):
        nb = S // 128
        work = [(h * nb + i, first + h, i, t, min(t + 4, i + 1))
                for h in range(2) for i in reversed(range(nb)) for t in range(0, i + 1, 4)]
        s, mx, m, l, o, done, ready, due = {}, {}, {}, {}, {}, {}, [], []

        def scores(b, h, i, t0, t1):
            x = pc.note(jax.lax.dot_general(
                _b16(ctx32[HB + h, i * TILE:(i + 1) * TILE, :]), _b16(ks32[h, t0 * TILE:t1 * TILE, :]),
                (((1,), (1,)), ((), ())), preferred_element_type=F32))
            if t1 == i + 1:
                row, col = (jax.lax.broadcasted_iota(jnp.int32, (128, 128), d) for d in range(2))
                diag = jnp.where(col <= row, x[:, -128:], NEG)
                x = jnp.concatenate([x[:, :-128], diag], axis=1) if t1 - t0 > 1 else diag
            s[b, t0] = x
            top = functools.reduce(jnp.maximum, _lane_tiles(x))
            mx[b] = jnp.maximum(mx[b], top) if t0 else top
            if t1 == i + 1:
                m[b] = jnp.max(mx[b], axis=1, keepdims=True)

        def values(b, h, i, t0, t1):
            p = jnp.exp2(s.pop((b, t0)) - m[b])
            y = pc.note(jnp.dot(p.astype(BF16), _b16(vs32[h, t0 * TILE:t1 * TILE, :]),
                                preferred_element_type=F32))
            parts = ([l[b]] if t0 else []) + _lane_tiles(p)
            l[b] = functools.reduce(jnp.add, [pc.tied(parts[0], 4)] + parts[1:])
            o[b] = o[b] + y if t0 else y
            if t1 == i + 1:
                ready.append((h, i, (o[b] * _recip(jnp.sum(l[b], axis=1, keepdims=True))).astype(BF16)))

        def products():
            clock = qi = pi = turn = 0
            while pi < len(work):
                can = work[pi][0] in done and clock - done[work[pi][0]] >= 12
                if qi < len(work) and (not can or turn == 0):
                    b, _, i, t0, t1 = work[qi]
                    scores(*work[qi])
                    clock += t1 - t0
                    if t1 == i + 1:
                        done[b] = clock
                    qi, turn = qi + 1, 1
                else:
                    values(*work[pi])
                    clock += work[pi][4] - work[pi][3]
                    if len(due) < len(ready):
                        due.append(clock + 8)
                    pi, turn = pi + 1, 0
                while due and (due[0] <= clock or pi == len(work)):
                    due.pop(0)
                    h, i, x = ready.pop(0)
                    ctx[g * GH + h, i * 128:(i + 1) * 128, :] = x
                yield

        main = products()
        _drain(_woven(main, 2 * len(work) - 8, side, side_steps, 3))
        _drain(main)

    for cp in cp_w(0) + cp_rows(0) + cp_rows(1):
        cp.start()
    start_slabs(jnp.int32(0))
    for cp in cp_w(0):
        cp.wait()
    jax.lax.fori_loop(0, GH, lambda j, _: _drain(prep_w(None, 0, j)), None)

    def group(g, _):
        def projections(jj, _):
            @pl.when(g == 0)
            def _():
                for j in (jj * 2, jj * 2 + 1):
                    @pl.when(j + 2 < GH)
                    def _():
                        for cp in cp_rows(j + 2):
                            cp.start()
                    for cp in cp_rows(j):
                        cp.wait()

                    @pl.when(j == 1)
                    def _():
                        start_slabs(j)

                    @pl.when(j == GH - 1)
                    def _():
                        for cp in cp_w(1):
                            cp.start()

                    def first_rows(a, _):
                        prep_rows(0, cc, j, a * 8)
                        prep_rows(4, xc, j, a * 8)
                    jax.lax.fori_loop(0, SET // 64, first_rows, None)

            i = g * 2 + jj

            @pl.when((i + 1) * 2 >= 24)
            def _():
                @pl.when(i * 2 >= 24)
                def _():
                    wait_slot(wa_raw, sem_wa, 2 + i % 2)

                @pl.when((i + 1) * 2 < HB)
                def _():
                    start_output_slabs(i + 1)
            wait_slot(wo_raw, sem_wo, i % 2)
            wait_slot(wa_raw, sem_wa, i % 2)
            pc = _Pace(g, 10)
            for n in range(2):
                j = jj * 2 + n
                u = g * GH + j
                first = prep_wo(pc, u, 16 * n)
                side = _chain(_woven(first, 20, reorder_wa(pc, u, 16 * n), 8), first, prep_wa(pc, u))
                main = project(pc, j)
                _drain(_woven(main, 3 * NP - 4, side, 56, 8 if n else 15))
                _drain(main)
            start_slabs(i + 2)

        @pl.when((g > 0) & (g + 1 < NG))
        def _():
            for cp in cp_w(g + 1):
                cp.start()

        @pl.when(g == NG - 1)
        def _():
            cp_xa(0).start()
            cp_xa(1).start()
        jax.lax.fori_loop(0, 2, projections, None)

        @pl.when(g + 1 < NG)
        def _():
            for cp in cp_w(g + 1):
                cp.wait()

        def attention(hh, _):
            pc = _Pace(g, 3)
            following = jnp.minimum(g + 1, NG - 1)
            attend(pc, g, hh * 2, _chain(*[prep_w(pc, following, hh * 2 + i) for i in range(2)]), 112)
        jax.lax.fori_loop(0, 2, attention, None)

    jax.lax.fori_loop(0, NG, group, None)
    wait_slot(wo_raw, sem_wo, 0)
    wait_slot(wo_raw, sem_wo, 1)
    wait_slot(wa_raw, sem_wa, 2)
    wait_slot(wa_raw, sem_wa, 3)

    def cp_out(t, part):
        at = (_rows(t * RO, RO), pl.ds(part * DM, DM))
        return pltpu.make_async_copy(stage.at[at], out_hbm.at[at], sem_out.at[part, t])

    def prep_ctx(pc, t, i):
        for a in range(0, RA, 8):
            for p in range(NG):
                z = _zero(t, i)
                x = pc.blocks(lambda b, k: ctx32[p * GH + k + z, _rows(t * (RO // 2) + b * RA + a, 8), :])
                for n, y in _seven(_lhs_term, [[_f32(w) for w in row] for row in x], i):
                    xc[n, p % 2, pl.ds(2 * (p // 2 * RA + a), 16), :] = y.astype(BF16)
                yield

    def prep_xa(pc, t, i):
        for a in range(0, RA, 8):
            for c in range(2):
                slot = t % 3 + _zero(t, i)
                x = pc.blocks(lambda b, k: xa_raw[slot, b * RA + a:b * RA + a + 8,
                                                  (2 * k + c) * 128:(2 * k + c + 1) * 128])
                for n, y in _seven(_lhs_term, [[_f32(w) for w in row] for row in x], i):
                    xc[n, c, pl.ds(2 * (4 * RA + a), 16), :] = y.astype(BF16)
                yield

    def window_weights(pc, t):
        lane = jax.lax.broadcasted_iota(jnp.int32, (16, 128), 1)

        def softmax(a):
            tie = pc.after()
            logits = []
            for w in range(WIN):
                x = jnp.concatenate([tie(pa[w + _zero(t, 1), b:b + 8, :]) for b in (a, a + 8)], axis=0)
                for bit in (16, 1):
                    x = x + jnp.where((lane & bit) != 0, pltpu.roll(x, bit, 1), pltpu.roll(x, 128 - bit, 1))
                if a < DIL * w:
                    pos = jax.lax.broadcasted_iota(jnp.int32, (16, 128), 0) + (t * RO + a)
                    x = jnp.where(pos >= DIL * w, x, NEG)
                logits.append(x)
            top = functools.reduce(jnp.maximum, logits)
            es = [jnp.exp2(x - top) for x in logits]
            inv = _recip(functools.reduce(jnp.add, es))
            for w, e in enumerate(es):
                pa[w, a:a + 16, :] = e * inv

        for a in range(0, RO, 8):
            for w in range(WIN):
                if w % 2 == 0:
                    tie = pc.after()
                    q = [tie(qa[j, a:a + 8, :]) for j in range(8)]
                b = a + HALO - DIL * w
                x = q[0] * ka[0, b:b + 8, :]
                for j in range(1, 8):
                    x = x + q[j] * ka[j, b:b + 8, :]
                pa[w, a:a + 8, :] = x
                if w % 2 == 1:
                    yield
            if a % 16 == 8:
                softmax(a - 8)
                yield
        ka[:, 0:HALO, :] = ka[:, RO:, :]

    def window_mix(pc, t):
        for a in range(0, RO, 8):
            for j in range(8):
                if j % 2 == 0:
                    tie = pc.after()
                    ps = [tie(pa[w + _zero(t, 0), a:a + 8, :]) for w in range(WIN)]
                acc = ps[0] * va[j, a + HALO:a + HALO + 8, :]
                for w in range(1, WIN):
                    b = a + HALO - DIL * w
                    acc = acc + ps[w] * va[j, b:b + 8, :]
                ya[j, a:a + 8, :] = acc
                if j % 2 == 1:
                    yield
        va[:, 0:HALO, :] = va[:, RO:, :]

    def prep_mixed(pc, t):
        for i in range(7):
            for a in range(0, RA, 8):
                for c in range(2):
                    z = _zero(t, i)
                    x = pc.blocks(lambda b, k: ya[2 * k + c + z, pl.ds(2 * (b * RA + a), 16), :])
                    for n, y in _seven(_lhs_term, x, i):
                        xc[n, c, pl.ds(2 * (5 * RA + a), 16), :] = y.astype(BF16)
                    yield

    def joined(blocks):
        return jnp.concatenate([jnp.concatenate(row, axis=1) for row in blocks], axis=0)

    ka[:, 0:HALO, :] = jnp.zeros((8, HALO, 128), F32)
    va[:, 0:HALO, :] = jnp.zeros((8, HALO, 128), F32)
    cp_xa(0).wait()
    for i in range(7):
        _drain(prep_xa(_Pace(0, 1), 0, i))

    def step(t, _):
        pc = _Pace(t, 8)
        cp_xa(t + 2).start()
        cp_xa(t + 1).wait()

        def times(first, w, at):
            def run(n):
                y = None
                for k in range(w.shape[2] // 128):
                    z = pc.note(_dot(_wide(lambda c: xc32[n, c, pl.ds((first + k) * RA, RA), :], 2),
                                     _wide(lambda c: w[at + n, c, k * 128:(k + 1) * 128, :], 2)))
                    y = z if y is None else y + z
                    yield
                return y
            return _combine(run)

        def products():
            y = joined((yield from times(4, wa32, NP)))
            for j in range(8):
                ka[j, HALO:, :] = y[:, j * 128:(j + 1) * 128]
            y = joined((yield from times(4, wa32, 0))) * (DA ** -0.5 * LOG2E)
            for j in range(8):
                qa[j] = y[:, j * 128:(j + 1) * 128]
            v, b = times(4, wa32, 2 * NP), times(0, wo32, 0)
            for i in range(7):
                yield from _woven(v, 7, prep_xa(pc, t + 1, i - 1) if i else iter(()), 8 if i else 0)
            y = joined(_drain(v))
            for j in range(8):
                va[j, HALO:, :] = y[:, j * 128:(j + 1) * 128]
            yield from _woven(b, 28, prep_xa(pc, t + 1, 6), 8)
            return (yield from b)

        main = products()
        _drain(_woven(main, 150, _chain(*[prep_ctx(pc, t, i) for i in range(7)]), 224, 8))
        _drain(_woven(main, 100, window_weights(pc, t), 144))
        _drain(_woven(main, 43, window_mix(pc, t), 128))
        _drain(_woven(main, 44, prep_mixed(pc, t), 56))
        stage[_rows(t * RO, RO), DM:] = joined(_drain(main)).astype(BF16)
        cp_out(t, 1).start()
        stage[_rows(t * RO, RO), 0:DM] = joined(_drain(times(5, wa32, 3 * NP))).astype(BF16)
        cp_out(t, 0).start()

    jax.lax.fori_loop(0, S // RO, step, None)
    cp_xa(S // RO + 1).wait()
    for t in range(S // RO):
        cp_out(t, 1).wait()
        cp_out(t, 0).wait()


@jax.jit
def pallas_concat_heads__sliding_local_dilated__compressed_kv_cla__prompt_kernel(
    A_x: jax.Array,
    A_wqkv: jax.Array,
    A_wo: jax.Array,
    B_x: jax.Array,
    B_c_kv: jax.Array,
    B_w_q: jax.Array,
    B_w_uk: jax.Array,
    B_w_uv: jax.Array,
    B_w_o: jax.Array,
):
    vmem, dma = pltpu.VMEM, pltpu.SemaphoreType.DMA
    scratch = [
        vmem((HB + GH, S, DB), BF16),
        vmem((NP, 2, HB * DB // 4, 128), BF16),
        vmem((4 * NP, 2, DM // 4, 128), BF16),
        vmem((2, 4, 32, DM), U32),
        vmem((4, 4, 32, DM), U32),
        vmem((NP, 2, S // 4, 128), BF16),
        vmem((NP, 1, S // 4, 128), BF16),
        vmem((NP + 8, 4 * 128, DB), BF16),
        vmem((2, 2, DM, DB), U32),
        vmem((2, 2, 2, DC, DB), U32),
        vmem((GH, S, DB), BF16),
        vmem((GH, S, DB), BF16),
        vmem((8, RO, 128), F32),
        vmem((8, HALO + RO, 128), F32),
        vmem((8, HALO + RO, 128), F32),
        vmem((8, RO, 128), F32),
        vmem((WIN, RO, 128), F32),
        vmem((3, RO // 2, DM), U32),
        vmem((S, 2 * DM), BF16),
        dma((2,)), dma((4,)), dma((2, 3, 2)), dma((GH,)), dma((3,)), dma((2, S // RO)),
    ]
    out = pl.pallas_call(
        _kernel,
        out_shape=jax.ShapeDtypeStruct((S, 2 * DM), BF16),
        in_specs=[pl.BlockSpec(memory_space=pl.ANY)] * 9,
        out_specs=pl.BlockSpec(memory_space=pl.ANY),
        scratch_shapes=scratch,
        compiler_params=pltpu.CompilerParams(
            vmem_limit_bytes=128 * 2**20,
            flags={"XLA_TPU_MAX_INSTS_TO_PREDICATE": 8}),
        name="fused",
    )(A_x.reshape(S, DM), A_wqkv, A_wo.reshape(8, DM // 8, DM),
      B_x.reshape(S, DM), B_c_kv.reshape(S, DC), B_w_q, B_w_uk, B_w_uv, B_w_o)
    return out.reshape(1, S, 2 * DM)
```
